```python
import jax
import jax.numpy as jnp

def _softmax(x, axis=-1):
    return jax.nn.softmax(x, axis=axis)
def _gelu(x):
    return jax.nn.gelu(x, approximate=True)
def _silu(x):
    return jax.nn.silu(x)
def _sigmoid(x):
    return jax.nn.sigmoid(x)
def _layernorm(x, axis=-1, eps=1e-5):
    m = jnp.mean(x, axis=axis, keepdims=True)
    v = jnp.var(x, axis=axis, keepdims=True)
    return (x - m) / jnp.sqrt(v + eps)
def _scatter_add(tgt, idx, src, axis=0):
    return tgt.at[idx].add(src)
def _segment_sum(src, seg, n):
    return jax.ops.segment_sum(src, seg, n)
class _Rng:
    def __init__(self, key):
        self._k = key
    def _next(self):
        self._k, sub = jax.random.split(self._k)
        return sub
    def normal(self, shape):
        return jax.random.normal(self._next(), shape, dtype=jnp.bfloat16)
    def randint(self, lo, hi, shape):
        return jax.random.randint(self._next(), shape, lo, hi, dtype=jnp.int32)
    def uniform(self, shape, lo=0.0, hi=1.0):
        return jax.random.uniform(self._next(), shape, jnp.bfloat16, lo, hi)
    def permutation(self, n):
        return jax.random.permutation(self._next(), n)


kernel_name = 'interleave_layers__sliding_local_dilated__linear_kernel_hedgehog__prompt'

def setup_inputs():
    _rng = _Rng(jax.random.key(int.from_bytes(__import__("os").urandom(4), "little")))
    _w = (lambda a: (lambda t: t.astype(jnp.bfloat16) if jnp.issubdtype(t.dtype, jnp.floating) else t)(jnp.asarray(a)))
    def _A_setup():
        B, S, D = 1, 2048, 1024
        return {
            "x": _w((lambda *s: _rng.normal(s) * 0.05)(B, S, D)),
            "wqkv": _w((lambda *s: _rng.normal(s) * 0.05)(D, 3 * D)),
            "wo": _w((lambda *s: _rng.normal(s) * 0.05)(D, D)),
        }
    _A_in = _A_setup()

    def _B_setup():
        B, S, D, H = 1, 2048, 1024, 32
        Dh = D // H
        return {
            "x": _w((lambda *s: _rng.normal(s) * 0.05)(B, S, D)),
            "wqkv": _w((lambda *s: _rng.normal(s) * 0.05)(D, 3 * D)),
            "w_phi": _w((lambda *s: _rng.normal(s) * 0.05)(H, Dh, Dh) * (Dh ** -0.5)),
            "wo": _w((lambda *s: _rng.normal(s) * 0.05)(D, D)),
        }
    _B_in = _B_setup()

    return {
        "A_x": _A_in["x"],
        "A_wqkv": _A_in["wqkv"],
        "A_wo": _A_in["wo"],
        "B_x": _B_in["x"],
        "B_wqkv": _B_in["wqkv"],
        "B_w_phi": _B_in["w_phi"],
        "B_wo": _B_in["wo"],
    }

def reference(A_x, A_wqkv, A_wo, B_x, B_wqkv, B_w_phi, B_wo):
    def _A_ref(x, wqkv, wo):
        B, S, D = x.shape
        H = 32; Dh = D // H
        W, dil = 8, 2
        qkv = (lambda x, *d: x.transpose(*d))((x @ wqkv).reshape(B, S, 3, H, Dh), 2, 0, 3, 1, 4)
        q, k, v = qkv[0], qkv[1], qkv[2]
        scale = Dh ** -0.5
        pos = jnp.arange(S)
        off = jnp.arange(W) * dil
        idx = pos[:, None] - off[None, :]
        mask = idx >= 0
        idx_c = jnp.where(mask, idx, 0).reshape(-1)
        kg = k[:, :, idx_c, :].reshape(B, H, S, W, Dh)
        vg = v[:, :, idx_c, :].reshape(B, H, S, W, Dh)
        logits = jnp.einsum("bhsd,bhswd->bhsw", q, kg) * scale
        logits = jnp.where(mask[None, None, :, :], logits, -1e9)
        attn = _softmax(logits, axis=-1)
        o = jnp.einsum("bhsw,bhswd->bhsd", attn, vg)
        return (lambda x, *d: x.transpose(*d))(o, 0, 2, 1, 3).reshape(B, S, D) @ wo

    def _B_ref(x, wqkv, w_phi, wo):
        B, S, D = x.shape
        H = 32; Dh = D // H
        qkv = (lambda x, *d: x.transpose(*d))((x @ wqkv).reshape(B, S, 3, H, Dh), 2, 0, 3, 1, 4)
        q, k, v = qkv[0], qkv[1], qkv[2]
        pq = jnp.einsum("bhsd,hdf->bhsf", q, w_phi)
        pk = jnp.einsum("bhsd,hdf->bhsf", k, w_phi)
        phi_q = jnp.concatenate([_softmax(pq, axis=-1), _softmax(-pq, axis=-1)], axis=-1)
        phi_k = jnp.concatenate([_softmax(pk, axis=-1), _softmax(-pk, axis=-1)], axis=-1)
        kv = jnp.einsum("bhsf,bhsd->bhfd", phi_k, v)
        z  = jnp.einsum("bhsf->bhf", phi_k)
        num = jnp.einsum("bhqf,bhfd->bhqd", phi_q, kv)
        den = jnp.einsum("bhqf,bhf->bhq", phi_q, z)[..., None] + 1e-6
        o = num / den
        return (lambda x, *d: x.transpose(*d))(o, 0, 2, 1, 3).reshape(B, S, D) @ wo

    x = A_x
    x = x + _A_ref(_layernorm(x, axis=-1), A_wqkv, A_wo)
    x = x + _B_ref(_layernorm(x, axis=-1), B_wqkv, B_w_phi, B_wo)
    x = x + _A_ref(_layernorm(x, axis=-1), A_wqkv, A_wo)
    x = x + _B_ref(_layernorm(x, axis=-1), B_wqkv, B_w_phi, B_wo)
    return x
```

```python
import jax
import jax.numpy as jnp
from jax import lax
import jax.experimental.pallas as pl
import jax.experimental.pallas.tpu as pltpu

S, D, H, DH = 2048, 1024, 32, 32
W = 8
NC = S // 128
F32, BF16 = jnp.float32, jnp.bfloat16
NT = (((1,), (1,)), ((), ()))


def _mm(a, b):
    return jnp.dot(a, b, preferred_element_type=F32)


def _tree(f, xs):
    xs = list(xs)
    while len(xs) > 1:
        xs = [f(xs[i], xs[i + 1]) for i in range(0, len(xs), 2)]
    return xs[0]


def _kernel(x_ref, awqkv, awo, bwqkv, bphi, bwo, out_ref,
            wa, woa, wb, wob, xt, xn, ot, q0, k0, v0, q1, k1, v1, tmp, kvacc, zacc, kvm):
    qkv_buf = ((q0, k0, v0), (q1, k1, v1))

    def norm_store(c, x):
        m = jnp.sum(x, axis=0, keepdims=True) * (1.0 / D)
        d = x - m
        v = jnp.sum(d * d, axis=0, keepdims=True) * (1.0 / D)
        xn[c] = (d * lax.rsqrt(v + 1e-5)).astype(BF16)

    def prep(g, _):
        off = pl.multiple_of(g * 256, 256)
        for t in range(3):
            wt = awqkv[:, pl.ds(pl.multiple_of(t * D + off, 256), 256)].astype(F32).T
            for c in range(8):
                tmp[c, 0:256, :] = wt[:, c * 128:(c + 1) * 128]
            for c in range(8):
                for d in range(0, DH, 2):
                    r = jnp.concatenate([tmp[c, pl.ds(d, 8, stride=DH), :],
                                         tmp[c, pl.ds(d + 1, 8, stride=DH), :]], axis=0)
                    wa[g, t * 256 + d * 8:t * 256 + d * 8 + 16, c * 128:(c + 1) * 128] = r.astype(BF16)
        wf = awo[pl.ds(off, 256), :].astype(F32)
        for c in range(8):
            tmp[c, 0:256, :] = wf[:, c * 128:(c + 1) * 128]
        for c in range(8):
            r = jnp.concatenate([tmp[c, pl.ds(d, 8, stride=DH), :] for d in range(DH)], axis=0)
            woa[c * 128:(c + 1) * 128, pl.ds(off, 256)] = r.T.astype(BF16)
        wob[:, pl.ds(off, 256)] = bwo[pl.ds(off, 256), :].astype(F32).T.astype(BF16)
        wb[2, pl.ds(off, 256), :] = bwqkv[:, pl.ds(pl.multiple_of(2 * D + off, 256), 256)].astype(F32).T.astype(BF16)
        return 0
    lax.fori_loop(0, 4, prep, 0)

    def fold(g, _):
        f_i = lax.broadcasted_iota(jnp.int32, (DH, 128), 0)
        f_j = lax.broadcasted_iota(jnp.int32, (DH, 128), 1)
        rep = _mm(bphi[g], jnp.where(f_i == f_j // 4, 1.0, 0.0).astype(BF16)).T
        r_i = lax.broadcasted_iota(jnp.int32, (128, 128), 0)
        r_j = lax.broadcasted_iota(jnp.int32, (128, 128), 1)
        bd = jnp.where(r_i % 4 == r_j // DH, rep, 0.0).astype(BF16)
        off = pl.multiple_of(g * 128, 128)
        for t in range(2):
            wsl = bwqkv[:, pl.ds(pl.multiple_of(t * D + off, 128), 128)]
            wb[t, pl.ds(off, 128), :] = lax.dot_general(bd, wsl, NT, preferred_element_type=F32).astype(BF16)
        return 0
    lax.fori_loop(0, 8, fold, 0)

    for c in range(8):
        tmp[c] = x_ref[:, c * 128:(c + 1) * 128].astype(F32)

    def load_x(j, _):
        x = jnp.concatenate([tmp[c, pl.ds(j, 128, stride=NC), :].T for c in range(8)], axis=0)
        xt[j] = x
        norm_store(j, x)
        return 0
    lax.fori_loop(0, NC, load_x, 0)

    def cols2(ref, c0, c1):
        return jnp.concatenate([ref[c0], ref[c1]], axis=1)

    def finish(c0, c1, w_ref, o):
        x = cols2(xt, c0, c1) + _mm(w_ref[...], o)
        for i, c in enumerate((c0, c1)):
            xc = x[:, i * 128:(i + 1) * 128]
            xt[c] = xc
            norm_store(c, xc)

    def a_proj(g, p, jj):
        qr, kr, vr = qkv_buf[p]
        j = 2 * jj
        r = _mm(wa[g], cols2(xn, 2 * j + p, 2 * j + 2 + p))
        for i in range(2):
            ri = r[:, i * 128:(i + 1) * 128]
            qr[j + i] = ri[0:256] * (DH ** -0.5)
            kr[8 + j + i] = ri[256:512]
            vr[8 + j + i] = ri[512:768]
            kr[j + i] = pltpu.roll(ri[256:512], 1, 1)
            vr[j + i] = pltpu.roll(ri[512:768], 1, 1)

    lane0 = lax.broadcasted_iota(jnp.int32, (8, 128), 1) == 0

    def a_attn(g, p, jj):
        qr, kr, vr = qkv_buf[p]
        j = 2 * jj
        lg = [[None] * W for _ in range(2)]
        for d in range(DH):
            sl = slice(d * 8, d * 8 + 8)
            kk = [kr[j + 1 + i, sl, :] for i in range(W + 1)]
            for i in range(2):
                q = qr[j + i, sl, :]
                for w in range(W):
                    t = q * kk[7 + i - w]
                    lg[i][w] = t if d == 0 else lg[i][w] + t
        pr = []
        for i in range(2):
            l = [lg[i][0]] + [jnp.where(lane0 & (j + i < w), -1e9, lg[i][w]) for w in range(1, W)]
            m = _tree(jnp.maximum, l)
            e = [jnp.exp(t - m) for t in l]
            inv = 1.0 / _tree(jnp.add, e)
            pr.append([t * inv for t in e])
        off = pl.multiple_of(g * 256, 256)
        for d in range(0, DH, 2):
            o = [[], []]
            for dd in (d, d + 1):
                sl = slice(dd * 8, dd * 8 + 8)
                vv = [vr[j + 1 + i, sl, :] for i in range(W + 1)]
                for i in range(2):
                    o[i].append(_tree(jnp.add, [pr[i][w] * vv[7 + i - w] for w in range(W)]))
            for i in range(2):
                ot[p * 8 + j + i, pl.ds(pl.multiple_of(off + d * 8, 16), 16), :] = (
                    jnp.concatenate(o[i], axis=0).astype(BF16))

    def a_out(p, jj):
        j = 2 * jj
        finish(2 * j + p, 2 * j + 2 + p, woa, cols2(ot, p * 8 + j, p * 8 + j + 1))

    def loop4(*fns):
        def body(jj, _):
            for f in fns:
                f(jj)
            return 0
        lax.fori_loop(0, 4, body, 0)

    def layer_a():
        loop4(lambda jj: a_proj(0, 0, jj))

        def grp(g, _):
            loop4(lambda jj: a_proj(g, 1, jj), lambda jj: a_attn(g, 0, jj))

            @pl.when(g < 3)
            def _():
                loop4(lambda jj: a_proj(g + 1, 0, jj), lambda jj: a_attn(g, 1, jj))
            return 0
        lax.fori_loop(0, 4, grp, 0)
        loop4(lambda jj: a_out(0, jj), lambda jj: a_attn(3, 1, jj))
        loop4(lambda jj: a_out(1, jj))

    def allred(f, x):
        r = _tree(f, [x[i * 8:(i + 1) * 8] for i in range(16)])
        return f(r, pltpu.roll(r, 4, 0))

    def dual_exp(p):
        ep = jnp.exp(p - jnp.tile(allred(jnp.maximum, p), (16, 1)))
        en = jnp.exp(jnp.tile(allred(jnp.minimum, p), (16, 1)) - p)
        return ep, 1.0 / allred(jnp.add, ep), en, 1.0 / allred(jnp.add, en)

    def b_kv(jj, _):
        xin = cols2(xn, 2 * jj, 2 * jj + 1)
        phis = []
        for g in range(8):
            ep, ip, en, im = dual_exp(_mm(wb[1, g * 128:(g + 1) * 128, :], xin))
            ph = jnp.concatenate([ep * jnp.tile(ip, (16, 1)), en * jnp.tile(im, (16, 1))], axis=0)
            zacc[g] += ph[:, :128] + ph[:, 128:]
            phis.append(ph.astype(BF16))
        for g in range(8):
            v = _mm(wb[2, g * 128:(g + 1) * 128, :], xin).astype(BF16)
            kvacc[g] += lax.dot_general(v, phis[g], NT, preferred_element_type=F32)
        return 0

    def b_out(jj):
        xin = cols2(xn, 2 * jj, 2 * jj + 1)
        os = []
        for g in range(8):
            ep, ip, en, im = dual_exp(_mm(wb[0, g * 128:(g + 1) * 128, :], xin))
            z = zacc[g]
            den = (allred(jnp.add, ep * jnp.tile(z[:128], (1, 2))) * ip
                   + allred(jnp.add, en * jnp.tile(z[128:], (1, 2))) * im + 1e-6)
            r = 1.0 / den
            ph = jnp.concatenate([ep * jnp.tile(ip * r, (16, 1)), en * jnp.tile(im * r, (16, 1))], axis=0)
            os.append(_mm(kvm[g], ph.astype(BF16)).astype(BF16))
        finish(2 * jj, 2 * jj + 1, wob, jnp.concatenate(os, axis=0))

    def layer_b():
        zacc[...] = jnp.zeros_like(zacc)
        kvacc[...] = jnp.zeros_like(kvacc)
        lax.fori_loop(0, NC // 2, b_kv, 0)
        r_i = lax.broadcasted_iota(jnp.int32, (128, 256), 0)
        r_j = lax.broadcasted_iota(jnp.int32, (128, 256), 1)

        def fin(g, _):
            kvm[g] = jnp.where(r_i // DH == r_j % 4, kvacc[g], 0.0).astype(BF16)
            zacc[g] = jnp.broadcast_to(jnp.sum(zacc[g], axis=1, keepdims=True), (256, 128))
            return 0
        lax.fori_loop(0, 8, fin, 0)

        def body(jj, _):
            b_out(jj)
            return 0
        lax.fori_loop(0, NC // 2, body, 0)

    def pair(_, c):
        with jax.named_scope("layerA"):
            layer_a()
        with jax.named_scope("layerB"):
            layer_b()
        return 0
    lax.fori_loop(0, 2, pair, 0)

    def store_x(j, _):
        for c in range(8):
            tmp[c, pl.ds(j, 128, stride=NC), :] = xt[j, c * 128:(c + 1) * 128, :].T
        return 0
    lax.fori_loop(0, NC, store_x, 0)
    for c in range(8):
        out_ref[:, c * 128:(c + 1) * 128] = tmp[c].astype(BF16)


@jax.jit
def pallas_interleave_layers__sliding_local_dilated__linear_kernel_hedgehog__prompt_kernel(
        A_x, A_wqkv, A_wo, B_x, B_wqkv, B_w_phi, B_wo):
    del B_x
    vm = pl.BlockSpec(memory_space=pltpu.VMEM)
    V = pltpu.VMEM
    out = pl.pallas_call(
        _kernel,
        in_specs=[vm] * 6,
        out_specs=vm,
        out_shape=jax.ShapeDtypeStruct((S, D), BF16),
        scratch_shapes=[
            V((4, 768, D), BF16), V((D, D), BF16), V((3, D, D), BF16), V((D, D), BF16),
            V((NC, D, 128), F32), V((NC, D, 128), BF16), V((NC, D, 128), BF16),
            V((8, 256, 128), F32), V((16, 256, 128), F32), V((16, 256, 128), F32),
            V((8, 256, 128), F32), V((16, 256, 128), F32), V((16, 256, 128), F32),
            V((8, S, 128), F32), V((8, 128, 256), F32), V((8, 256, 128), F32), V((8, 128, 256), BF16),
        ],
        compiler_params=pltpu.CompilerParams(vmem_limit_bytes=110 * 1024 * 1024),
    )(A_x.reshape(S, D), A_wqkv, A_wo, B_wqkv, B_w_phi.reshape(8, 128, DH), B_wo)
    return out.reshape(1, S, D)
```

```python
import jax
import jax.numpy as jnp
from jax import lax
import jax.experimental.pallas as pl
import jax.experimental.pallas.tpu as pltpu

S, D, H, DH = 2048, 1024, 32, 32
W = 8
NC = S // 128
F32, BF16 = jnp.float32, jnp.bfloat16
NT = (((1,), (1,)), ((), ()))


def _mm(a, b):
    return jnp.dot(a, b, preferred_element_type=F32)


def _tree(f, xs):
    xs = list(xs)
    while len(xs) > 1:
        xs = [f(xs[i], xs[i + 1]) for i in range(0, len(xs), 2)]
    return xs[0]


def _weave(*gens):
    order = sorted(((k + 0.5) / n, gi) for gi, (_, n) in enumerate(gens) for k in range(n))
    for _, gi in order:
        next(gens[gi][0], None)
    for g, _ in gens:
        for _ in g:
            pass


NORM = 24


def _kernel(x_hbm, awqkv_hbm, awo_hbm, bwqkv_hbm, bphi, bwo_hbm, out_hbm,
            xio, awqkv, awo, bwqkv, bwo, sems, osems, bds,
            wa, woa, wb, wob, xt, xn, ot, q0, k0, v0, q1, k1, v1, tmp, kvacc, zacc, kvm):
    qkv_buf = ((q0, k0, v0), (q1, k1, v1))

    def norm(i):
        acc = None
        for r in range(8):
            t = _tree(jnp.add, [xt[i, r * 128 + k * 8:r * 128 + k * 8 + 8, :] for k in range(16)])
            acc = t if r == 0 else acc + t
            yield
        m = jnp.sum(acc, axis=0, keepdims=True) * (1.0 / D)
        for r in range(8):
            d = xt[i, r * 128:(r + 1) * 128, :] - m
            d = d * d
            t = _tree(jnp.add, [d[k * 8:k * 8 + 8] for k in range(16)])
            acc = t if r == 0 else acc + t
            yield
        inv = lax.rsqrt(jnp.sum(acc, axis=0, keepdims=True) * (1.0 / D) + 1e-5)
        for r in range(8):
            sl = slice(r * 128, (r + 1) * 128)
            xn[i, sl, :] = ((xt[i, sl, :] - m) * inv).astype(BF16)
            yield

    def norm_now(i):
        _weave((norm(i), NORM))

    def ds(i, n):
        return pl.ds(pl.multiple_of(i * n, n), n)

    def wrows(ref, g, r):
        return jnp.concatenate([ref[g, k, r * 128:(r + 1) * 128, :] for k in range(8)], axis=1)

    x_cp = [pltpu.make_async_copy(x_hbm.at[:, ds(c, 128)], xio.at[c], sems.at[c]) for c in range(8)]
    a_cp = [[pltpu.make_async_copy(awqkv_hbm.at[:, ds(t * 4 + g, 256)], awqkv.at[g, t], sems.at[8 + g * 3 + t])
             for t in range(3)] for g in range(4)]
    ao_cp = pltpu.make_async_copy(awo_hbm, awo, sems.at[20])
    b_cp = [pltpu.make_async_copy(bwqkv_hbm, bwqkv, sems.at[21]),
            pltpu.make_async_copy(bwo_hbm, bwo, sems.at[22])]
    for cp in x_cp + a_cp[0] + a_cp[1] + [ao_cp]:
        cp.start()

    def tr(blk):
        return blk.astype(F32).T

    def prep_a(g, c, u):
        for t in range(3):
            tmp[u * 4 + t] = tr(awqkv[g, t, ds(c, 128), :])
            yield
            r = jnp.concatenate([tmp[u * 4 + t, pl.ds(d, 8, stride=DH), :] for d in range(DH)], axis=0)
            wa[g, c, t * 256:(t + 1) * 256, :] = r.astype(BF16)
            yield

    def prep_ao(g, c, u):
        tmp[u * 4 + 3] = awo[ds(g, 256), ds(c, 128)].astype(F32)
        yield
        r = jnp.concatenate([tmp[u * 4 + 3, pl.ds(d, 8, stride=DH), :] for d in range(DH)], axis=0)
        woa[c, :, ds(g, 256)] = r.T.astype(BF16)
        yield

    def prep_b(g, c):
        wob[c, :, ds(g, 256)] = tr(bwo[ds(g, 256), ds(c, 128)]).astype(BF16)
        yield
        wb[2, c, ds(g, 256), :] = tr(bwqkv[ds(c, 128), ds(8 + g, 256)]).astype(BF16)
        yield
        for t in range(2):
            for h in range(2):
                wsl = bwqkv[ds(c, 128), ds(t * 8 + 2 * g + h, 128)]
                wb[t, c, ds(2 * g + h, 128), :] = lax.dot_general(
                    bds[2 * g + h], wsl, NT, preferred_element_type=F32).astype(BF16)
            yield

    f_i = lax.broadcasted_iota(jnp.int32, (DH, 128), 0)
    f_j = lax.broadcasted_iota(jnp.int32, (DH, 128), 1)
    rep = _mm(bphi[...], jnp.where(f_i == f_j // 4, 1.0, 0.0).astype(BF16))
    e_i = lax.broadcasted_iota(jnp.int32, (128, 128), 0)
    e_j = lax.broadcasted_iota(jnp.int32, (128, 128), 1)
    for g in range(8):
        bds[g] = jnp.where(e_i % 4 == e_j // DH, rep[g * 128:(g + 1) * 128].T, 0.0).astype(BF16)

    xio32 = xio.bitcast(jnp.uint32)

    def load_x(jj):
        for c in range(8):
            for h in range(2):
                w = xio32[c, pl.ds(2 * jj + h, 128, stride=8), :].T
                for p in range(2):
                    bits = (w << 16) if p == 0 else (w & jnp.uint32(0xFFFF0000))
                    xt[p * 4 + jj, c * 128:(c + 1) * 128, h * 128:(h + 1) * 128] = (
                        lax.bitcast_convert_type(bits, F32))
            yield

    def chain(*gens):
        for g in gens:
            yield from g

    def store_x(jj, _):
        for c in range(8):
            for h in range(2):
                e, o = [lax.bitcast_convert_type(
                    xt[p * 4 + jj, c * 128:(c + 1) * 128, h * 128:(h + 1) * 128].astype(BF16).astype(F32),
                    jnp.uint32) for p in range(2)]
                xio32[c, pl.ds(2 * jj + h, 128, stride=8), :] = ((e >> 16) | o).T
        return 0

    def out_proj(i, w_ref):
        o = ot[i]
        for r in range(8):
            sl = slice(r * 128, (r + 1) * 128)
            xt[i, sl, :] += _mm(w_ref[r], o)
            yield

    def a_proj(g, p, jj):
        qr, kr, vr = qkv_buf[p]
        j = 2 * jj
        xin = xn[p * 4 + jj]
        for r in range(6):
            t = _mm(wrows(wa, g, r), xin)
            sl = slice((r % 2) * 128, (r % 2 + 1) * 128)
            for i in range(2):
                ti = t[:, i * 128:(i + 1) * 128]
                if r < 2:
                    qr[j + i, sl, :] = ti * (DH ** -0.5)
                else:
                    dst = kr if r < 4 else vr
                    dst[8 + j + i, sl, :] = ti
                    dst[j + i, sl, :] = pltpu.roll(ti, 1, 1)
            yield

    lane0 = lax.broadcasted_iota(jnp.int32, (8, 128), 1) == 0

    def a_attn(g, p, jj):
        qr, kr, vr = qkv_buf[p]
        j = 2 * jj
        lg = [[None] * W for _ in range(2)]
        for d in range(DH):
            sl = slice(d * 8, d * 8 + 8)
            kk = [kr[j + 1 + i, sl, :] for i in range(W + 1)]
            for i in range(2):
                q = qr[j + i, sl, :]
                for w in range(W):
                    t = q * kk[7 + i - w]
                    lg[i][w] = t if d == 0 else lg[i][w] + t
            yield
        pr = []
        for i in range(2):
            l = [lg[i][0]] + [jnp.where(lane0 & (j + i < w), -1e9, lg[i][w]) for w in range(1, W)]
            m = _tree(jnp.maximum, l)
            e = [jnp.exp(t - m) for t in l]
            inv = 1.0 / _tree(jnp.add, e)
            pr.append([t * inv for t in e])
            yield
        off = pl.multiple_of(g * 256, 256)
        for d in range(0, DH, 2):
            o = [[], []]
            for dd in (d, d + 1):
                sl = slice(dd * 8, dd * 8 + 8)
                vv = [vr[j + 1 + i, sl, :] for i in range(W + 1)]
                for i in range(2):
                    o[i].append(_tree(jnp.add, [pr[i][w] * vv[7 + i - w] for w in range(W)]))
                if dd == d:
                    yield
            ot[p * 4 + jj, pl.ds(pl.multiple_of(off + d * 8, 16), 16), :] = jnp.concatenate(
                [jnp.concatenate(o[i], axis=0) for i in range(2)], axis=1).astype(BF16)
            yield

    def loop(lo, hi, make):
        def body(i, _):
            _weave(*make(i))
            return 0
        lax.fori_loop(lo, hi, body, 0)

    def layer_a(first):
        def part(g, p):
            def make(jj):
                gens = [(a_proj(g + p, 1 - p, jj), 6), (a_attn(g, p, jj), 66)]
                if first:
                    for u in range(2):
                        c = 2 * jj + u
                        if p == 1:
                            gens.append((prep_b(g, c), 4))
                        else:
                            gens.append((prep_ao(g, c, u), 2))
                            if not (isinstance(g, int) and g == 3):
                                gens.append((prep_a(g + 1, c, u), 6))
                return gens
            loop(0, 4, make)

        def grp(g, _):
            if first:
                @pl.when(g == 0)
                def _():
                    for cp in a_cp[1] + [ao_cp]:
                        cp.wait()
                    for cp in a_cp[2] + b_cp + a_cp[3]:
                        cp.start()
                for k in (2, 3):
                    @pl.when(g == k - 1)
                    def _():
                        for cp in a_cp[k]:
                            cp.wait()
            part(g, 0)
            if first:
                @pl.when(g == 0)
                def _():
                    for cp in b_cp:
                        cp.wait()
            part(g, 1)
            return 0
        lax.fori_loop(0, 3, grp, 0)
        part(3, 0)
        _weave((out_proj(0, woa), 8), (a_attn(3, 1, 0), 66))
        loop(1, 4, lambda i: [(out_proj(i, woa), 8), (a_attn(3, 1, i), 66), (norm(i - 1), NORM)])
        loop(4, 8, lambda i: [(out_proj(i, woa), 8), (norm(i - 1), NORM)] + (
            [(prep_b(3, 2 * i - 8), 4), (prep_b(3, 2 * i - 7), 4)] if first else []))

    def allred(f, x):
        r = _tree(f, [x[i * 8:(i + 1) * 8] for i in range(16)])
        return f(r, pltpu.roll(r, 4, 0))

    def dual_exp(p):
        ep = jnp.exp(p - jnp.tile(allred(jnp.maximum, p), (16, 1)))
        en = jnp.exp(jnp.tile(allred(jnp.minimum, p), (16, 1)) - p)
        return ep, 1.0 / allred(jnp.add, ep), en, 1.0 / allred(jnp.add, en)

    def b_kv(i):
        xin = xn[i]
        phis = []
        for g in range(9):
            if g < 8:
                pk = _mm(wrows(wb, 1, g), xin)
                v = _mm(wrows(wb, 2, g), xin).astype(BF16)
            if g > 0:
                kvacc[g - 1] += lax.dot_general(*phis[g - 1], NT, preferred_element_type=F32)
            yield
            if g < 8:
                ep, ip, en, im = dual_exp(pk)
                ph = jnp.concatenate([ep * jnp.tile(ip, (16, 1)), en * jnp.tile(im, (16, 1))], axis=0)
                zacc[g] += ph[:, :128] + ph[:, 128:]
                phis.append((v, ph.astype(BF16)))

    def b_fin(g):
        r_i = lax.broadcasted_iota(jnp.int32, (128, 256), 0)
        r_j = lax.broadcasted_iota(jnp.int32, (128, 256), 1)
        kvm[g] = jnp.where(r_i // DH == r_j % 4, kvacc[g], 0.0).astype(BF16)
        zacc[g] = jnp.broadcast_to(jnp.sum(zacc[g], axis=1, keepdims=True), (256, 128))

    def b_q(i, first=False):
        xin = xn[i]
        phis = []
        for g in range(9):
            if g < 8:
                pq = _mm(wrows(wb, 0, g), xin)
            if g > 0:
                ot[i, (g - 1) * 128:g * 128, :] = _mm(kvm[g - 1], phis[g - 1]).astype(BF16)
            yield
            if g < 8:
                if first:
                    b_fin(g)
                ep, ip, en, im = dual_exp(pq)
                z = zacc[g]
                den = (allred(jnp.add, ep * jnp.tile(z[:128], (1, 2))) * ip
                       + allred(jnp.add, en * jnp.tile(z[128:], (1, 2))) * im + 1e-6)
                r = 1.0 / den
                phis.append(jnp.concatenate(
                    [ep * jnp.tile(ip * r, (16, 1)), en * jnp.tile(im * r, (16, 1))], axis=0).astype(BF16))

    def layer_b():
        zacc[...] = jnp.zeros_like(zacc)
        kvacc[...] = jnp.zeros_like(kvacc)
        norm_now(7)
        loop(0, 8, lambda i: [(b_kv(i), 9)])
        _weave((b_q(0, True), 9))
        _weave((out_proj(0, wob), 8), (b_q(1), 9))
        loop(2, 8, lambda i: [(norm(i - 2), NORM), (out_proj(i - 1, wob), 8), (b_q(i), 9)])
        _weave((out_proj(7, wob), 8), (norm(6), NORM))

    for cp in x_cp:
        cp.wait()
    _weave((chain(load_x(0), norm(0), norm(4)), 56))
    for cp in a_cp[0]:
        cp.wait()
    _weave((chain(*[prep_a(0, c, c % 2) for c in range(8)]), 48))
    for jj in range(1, 4):
        _weave((a_proj(0, 0, jj - 1), 6), (chain(load_x(jj), norm(jj), norm(4 + jj)), 56))
    _weave((a_proj(0, 0, 3), 6))
    layer_a(True)
    layer_b()
    _weave((a_proj(0, 0, 0), 6), (norm(7), NORM))
    loop(1, 4, lambda jj: [(a_proj(0, 0, jj), 6)])
    layer_a(False)
    layer_b()
    for jj in range(4):
        store_x(jj, 0)
    o_cp = [pltpu.make_async_copy(xio.at[c], out_hbm.at[:, ds(c, 128)], osems.at[c]) for c in range(8)]
    for cp in o_cp:
        cp.start()
    for cp in o_cp:
        cp.wait()


@jax.jit
def pallas_interleave_layers__sliding_local_dilated__linear_kernel_hedgehog__prompt_kernel(
        A_x, A_wqkv, A_wo, B_x, B_wqkv, B_w_phi, B_wo):
    del B_x
    vm = pl.BlockSpec(memory_space=pltpu.VMEM)
    hbm = pl.BlockSpec(memory_space=pl.ANY)
    V = pltpu.VMEM
    out = pl.pallas_call(
        _kernel,
        in_specs=[hbm] * 4 + [vm, hbm],
        out_specs=hbm,
        out_shape=jax.ShapeDtypeStruct((S, D), BF16),
        scratch_shapes=[
            V((8, S, 128), BF16), V((4, 3, D, 256), BF16), V((D, D), BF16), V((D, 3 * D), BF16), V((D, D), BF16),
            pltpu.SemaphoreType.DMA((23,)), pltpu.SemaphoreType.DMA((8,)), V((8, 128, 128), BF16),
            V((4, 8, 768, 128), BF16), V((8, 128, D), BF16), V((3, 8, D, 128), BF16), V((8, 128, D), BF16),
            V((8, D, 256), F32), V((8, D, 256), BF16), V((8, D, 256), BF16),
            V((8, 256, 128), F32), V((16, 256, 128), F32), V((16, 256, 128), F32),
            V((8, 256, 128), F32), V((16, 256, 128), F32), V((16, 256, 128), F32),
            V((8, 256, 128), F32), V((8, 128, 256), F32), V((8, 256, 128), F32), V((8, 128, 256), BF16),
        ],
        compiler_params=pltpu.CompilerParams(vmem_limit_bytes=110 * 1024 * 1024),
    )(A_x.reshape(S, D), A_wqkv, A_wo, B_wqkv, B_w_phi.reshape(D, DH), B_wo)
    return out.reshape(1, S, D)
```

```python
import jax
import jax.numpy as jnp
from jax import lax
import jax.experimental.pallas as pl
import jax.experimental.pallas.tpu as pltpu

S, D, H, DH = 2048, 1024, 32, 32
W = 8
NC = S // 128
F32, BF16 = jnp.float32, jnp.bfloat16
NT = (((1,), (1,)), ((), ()))


def _mm(a, b):
    return jnp.dot(a, b, preferred_element_type=F32)


def _tree(f, xs):
    xs = list(xs)
    while len(xs) > 1:
        xs = [f(xs[i], xs[i + 1]) for i in range(0, len(xs), 2)]
    return xs[0]


def _weave(*gens):
    order = sorted(((k + (0.5 if gi else 0)) / n, gi) for gi, (_, n) in enumerate(gens) for k in range(n))
    for _, gi in order:
        next(gens[gi][0], None)
    for g, _ in gens:
        for _ in g:
            pass


NORM = 24


def _kernel(x_hbm, awqkv_hbm, awo_hbm, bwqkv_hbm, bphi, bwo_hbm, out_hbm,
            xio, awqkv, awo, bwqkv, bwo, sems, osems, bds,
            wa, woa, wb, wob, xt, xn, ot, q0, k0, v0, q1, k1, v1, tmp, kvacc, zacc, kvm):
    qkv_buf = ((q0, k0, v0), (q1, k1, v1))

    def norm(i):
        acc = None
        for r in range(8):
            t = _tree(jnp.add, [xt[i, r * 128 + k * 8:r * 128 + k * 8 + 8, :] for k in range(16)])
            acc = t if r == 0 else acc + t
            yield
        m = jnp.sum(acc, axis=0, keepdims=True) * (1.0 / D)
        for r in range(8):
            d = xt[i, r * 128:(r + 1) * 128, :] - m
            d = d * d
            t = _tree(jnp.add, [d[k * 8:k * 8 + 8] for k in range(16)])
            acc = t if r == 0 else acc + t
            yield
        inv = lax.rsqrt(jnp.sum(acc, axis=0, keepdims=True) * (1.0 / D) + 1e-5)
        for r in range(8):
            sl = slice(r * 128, (r + 1) * 128)
            xn[i, sl, :] = ((xt[i, sl, :] - m) * inv).astype(BF16)
            yield

    def norm_now(i):
        _weave((norm(i), NORM))

    def ds(i, n):
        return pl.ds(pl.multiple_of(i * n, n), n)

    def wrows(ref, g, r):
        return jnp.concatenate([ref[g, k, r * 128:(r + 1) * 128, :] for k in range(8)], axis=1)

    x_cp = [pltpu.make_async_copy(x_hbm.at[:, ds(c, 128)], xio.at[c], sems.at[c]) for c in range(8)]
    a_cp = [[pltpu.make_async_copy(awqkv_hbm.at[:, ds(t * 4 + g, 256)], awqkv.at[g, t], sems.at[8 + g * 3 + t])
             for t in range(3)] for g in range(4)]
    ao_cp = pltpu.make_async_copy(awo_hbm, awo, sems.at[20])
    b_cp = [pltpu.make_async_copy(bwqkv_hbm, bwqkv, sems.at[21]),
            pltpu.make_async_copy(bwo_hbm, bwo, sems.at[22])]
    for cp in x_cp + a_cp[0] + a_cp[1] + [ao_cp]:
        cp.start()

    def tr(blk):
        return blk.astype(F32).T

    def prep_a(g, c, u):
        for t in range(3):
            tmp[u * 4 + t] = tr(awqkv[g, t, ds(c, 128), :])
            yield
            r = jnp.concatenate([tmp[u * 4 + t, pl.ds(d, 8, stride=DH), :] for d in range(DH)], axis=0)
            wa[g, c, t * 256:(t + 1) * 256, :] = r.astype(BF16)
            yield

    def prep_ao(g, c, u):
        tmp[u * 4 + 3] = awo[ds(g, 256), ds(c, 128)].astype(F32)
        yield
        r = jnp.concatenate([tmp[u * 4 + 3, pl.ds(d, 8, stride=DH), :] for d in range(DH)], axis=0)
        woa[c, :, ds(g, 256)] = r.T.astype(BF16)
        yield

    def prep_b(g, c):
        wob[c, :, ds(g, 256)] = tr(bwo[ds(g, 256), ds(c, 128)]).astype(BF16)
        yield
        wb[2, c, ds(g, 256), :] = tr(bwqkv[ds(c, 128), ds(8 + g, 256)]).astype(BF16)
        yield
        for t in range(2):
            for h in range(2):
                wsl = bwqkv[ds(c, 128), ds(t * 8 + 2 * g + h, 128)]
                wb[t, c, ds(2 * g + h, 128), :] = lax.dot_general(
                    bds[2 * g + h], wsl, NT, preferred_element_type=F32).astype(BF16)
            yield

    f_i = lax.broadcasted_iota(jnp.int32, (DH, 128), 0)
    f_j = lax.broadcasted_iota(jnp.int32, (DH, 128), 1)
    rep = _mm(bphi[...], jnp.where(f_i == f_j % 64 // 2, 1.0, 0.0).astype(BF16))
    e_i = lax.broadcasted_iota(jnp.int32, (128, 128), 0)
    e_j = lax.broadcasted_iota(jnp.int32, (128, 128), 1)
    for g in range(8):
        bds[g] = jnp.where(e_i // 64 * 2 + e_i % 2 == e_j // DH, rep[g * 128:(g + 1) * 128].T, 0.0).astype(BF16)

    xio32 = xio.bitcast(jnp.uint32)

    def load_x(jj):
        for c in range(8):
            for h in range(2):
                w = xio32[c, pl.ds(2 * jj + h, 128, stride=8), :].T
                for p in range(2):
                    bits = (w << 16) if p == 0 else (w & jnp.uint32(0xFFFF0000))
                    xt[p * 4 + jj, c * 128:(c + 1) * 128, h * 128:(h + 1) * 128] = (
                        lax.bitcast_convert_type(bits, F32))
            yield

    def chain(*gens):
        for g in gens:
            yield from g

    def store_x(jj, _):
        for c in range(8):
            for h in range(2):
                e, o = [lax.bitcast_convert_type(
                    xt[p * 4 + jj, c * 128:(c + 1) * 128, h * 128:(h + 1) * 128].astype(BF16).astype(F32),
                    jnp.uint32) for p in range(2)]
                xio32[c, pl.ds(2 * jj + h, 128, stride=8), :] = ((e >> 16) | o).T
        return 0

    def out_proj(i, w_ref):
        o = ot[i]
        for r in range(8):
            sl = slice(r * 128, (r + 1) * 128)
            xt[i, sl, :] += _mm(w_ref[r], o)
            yield

    def a_proj(g, p, jj):
        qr, kr, vr = qkv_buf[p]
        j = 2 * jj
        xin = xn[p * 4 + jj]
        for r in range(6):
            t = _mm(wrows(wa, g, r), xin)
            sl = slice((r % 2) * 128, (r % 2 + 1) * 128)
            for i in range(2):
                ti = t[:, i * 128:(i + 1) * 128]
                if r < 2:
                    qr[j + i, sl, :] = ti * (DH ** -0.5)
                else:
                    dst = kr if r < 4 else vr
                    dst[8 + j + i, sl, :] = ti
                    dst[j + i, sl, :] = pltpu.roll(ti, 1, 1)
            yield

    lane0 = lax.broadcasted_iota(jnp.int32, (8, 128), 1) == 0

    def a_attn(g, p, jj):
        qr, kr, vr = qkv_buf[p]
        j = 2 * jj
        lg = [[None] * W for _ in range(2)]
        for d in range(DH):
            sl = slice(d * 8, d * 8 + 8)
            kk = [kr[j + 1 + i, sl, :] for i in range(W + 1)]
            for i in range(2):
                q = qr[j + i, sl, :]
                for w in range(W):
                    t = q * kk[7 + i - w]
                    lg[i][w] = t if d == 0 else lg[i][w] + t
            yield
        pr = []
        for i in range(2):
            l = [lg[i][0]] + [jnp.where(lane0 & (j + i < w), -1e9, lg[i][w]) for w in range(1, W)]
            m = _tree(jnp.maximum, l)
            e = [jnp.exp(t - m) for t in l]
            inv = 1.0 / _tree(jnp.add, e)
            pr.append([t * inv for t in e])
            yield
        off = pl.multiple_of(g * 256, 256)
        for d in range(0, DH, 2):
            o = [[], []]
            for dd in (d, d + 1):
                sl = slice(dd * 8, dd * 8 + 8)
                vv = [vr[j + 1 + i, sl, :] for i in range(W + 1)]
                for i in range(2):
                    o[i].append(_tree(jnp.add, [pr[i][w] * vv[7 + i - w] for w in range(W)]))
                if dd == d:
                    yield
            ot[p * 4 + jj, pl.ds(pl.multiple_of(off + d * 8, 16), 16), :] = jnp.concatenate(
                [jnp.concatenate(o[i], axis=0) for i in range(2)], axis=1).astype(BF16)
            yield

    def loop(lo, hi, make, u=4):
        if (hi - lo) % u:
            u = hi - lo

        def body(k, _):
            parts = [make(lo + k * u + t) for t in range(u)]
            _weave(*[(chain(*[take(*pt[a]) for pt in parts]), u * parts[0][a][1])
                     for a in range(len(parts[0]))])
            return 0
        lax.fori_loop(0, (hi - lo) // u, body, 0)

    def take(gen, n):
        for _ in range(n):
            next(gen, None)
            yield
        for _ in gen:
            pass

    def layer_a(first):
        def part(g, p):
            def make(jj):
                gens = [(a_proj(g + p, 1 - p, jj), 6), (a_attn(g, p, jj), 66)]
                if first:
                    for u in range(2):
                        c = 2 * jj + u
                        if p == 1:
                            gens.append((prep_b(g, c), 4))
                        else:
                            gens.append((prep_ao(g, c, u), 2))
                            if not (isinstance(g, int) and g == 3):
                                gens.append((prep_a(g + 1, c, u), 6))
                return gens
            loop(0, 4, make)

        def grp(g, _):
            if first:
                @pl.when(g == 0)
                def _():
                    for cp in a_cp[1] + [ao_cp]:
                        cp.wait()
                    for cp in a_cp[2] + b_cp + a_cp[3]:
                        cp.start()
                for k in (2, 3):
                    @pl.when(g == k - 1)
                    def _():
                        for cp in a_cp[k]:
                            cp.wait()
            part(g, 0)
            if first:
                @pl.when(g == 0)
                def _():
                    for cp in b_cp:
                        cp.wait()
            part(g, 1)
            return 0
        lax.fori_loop(0, 3, grp, 0)
        part(3, 0)
        _weave((out_proj(0, woa), 8), (a_attn(3, 1, 0), 66))
        loop(1, 4, lambda i: [(out_proj(i, woa), 8), (a_attn(3, 1, i), 66), (norm(i - 1), NORM)])
        loop(4, 8, lambda i: [(out_proj(i, woa), 8), (norm(i - 1), NORM)] + (
            [(prep_b(3, 2 * i - 8), 4), (prep_b(3, 2 * i - 7), 4)] if first else []))

    def allred(f, x):
        out = []
        for a in range(2):
            r = _tree(f, [x[a * 64 + i * 8:a * 64 + i * 8 + 8] for i in range(8)])
            r = f(r, pltpu.roll(r, 4, 0))
            out.append(f(r, pltpu.roll(r, 2, 0)))
        return out

    def bc(r):
        return jnp.concatenate([r[0]] * 8 + [r[1]] * 8, axis=0)

    def feat(p, g, is_q):
        ep = jnp.exp(p - bc(allred(jnp.maximum, p)))
        en = jnp.exp(bc(allred(jnp.minimum, p)) - p)
        ip = [1.0 / t for t in allred(jnp.add, ep)]
        im = [1.0 / t for t in allred(jnp.add, en)]
        if is_q:
            dp = allred(jnp.add, ep * jnp.tile(zacc[g, :128], (1, 2)))
            dn = allred(jnp.add, en * jnp.tile(zacc[g, 128:], (1, 2)))
            r = [1.0 / (dp[a] * ip[a] + dn[a] * im[a] + 1e-6) for a in range(2)]
            ip = [ip[a] * r[a] for a in range(2)]
            im = [im[a] * r[a] for a in range(2)]
        ep, en = ep * bc(ip), en * bc(im)
        if not is_q:
            zacc[g, :128] += ep[:, :128] + ep[:, 128:]
            zacc[g, 128:] += en[:, :128] + en[:, 128:]
        return [jnp.concatenate([ep[a * 64:(a + 1) * 64], en[a * 64:(a + 1) * 64]], axis=0).astype(BF16)
                for a in range(2)]

    def b_kv(i):
        xin = xn[i]
        phis = []
        for g in range(9):
            if g < 8:
                pk = _mm(wrows(wb, 1, g), xin)
                v = _mm(wrows(wb, 2, g), xin).astype(BF16)
            if g > 0:
                v1, ph = phis[g - 1]
                kvacc[g - 1] += jnp.concatenate(
                    [lax.dot_general(v1[a * 64:(a + 1) * 64], ph[a], NT, preferred_element_type=F32)
                     for a in range(2)], axis=0)
            yield
            if g < 8:
                phis.append((v, feat(pk, g, False)))

    def b_fin(g):
        r_i = lax.broadcasted_iota(jnp.int32, (128, 128), 0)
        r_j = lax.broadcasted_iota(jnp.int32, (128, 128), 1)
        kvm[g] = jnp.where(r_i // DH % 2 == r_j % 2, kvacc[g], 0.0).astype(BF16)
        zacc[g] = jnp.broadcast_to(jnp.sum(zacc[g], axis=1, keepdims=True), (256, 128))

    def b_q(i, first=False):
        xin = xn[i]
        phis = []
        for g in range(9):
            if g < 8:
                pq = _mm(wrows(wb, 0, g), xin)
            if g > 0:
                ot[i, (g - 1) * 128:g * 128, :] = jnp.concatenate(
                    [_mm(kvm[g - 1, a * 64:(a + 1) * 64], phis[g - 1][a]) for a in range(2)],
                    axis=0).astype(BF16)
            yield
            if g < 8:
                if first:
                    b_fin(g)
                phis.append(feat(pq, g, True))

    def layer_b():
        zacc[...] = jnp.zeros_like(zacc)
        kvacc[...] = jnp.zeros_like(kvacc)
        norm_now(7)
        loop(0, 8, lambda i: [(b_kv(i), 9)])
        _weave((b_q(0, True), 9))
        _weave((out_proj(0, wob), 8), (b_q(1), 9))
        loop(2, 8, lambda i: [(norm(i - 2), NORM), (out_proj(i - 1, wob), 8), (b_q(i), 9)])
        _weave((out_proj(7, wob), 8), (norm(6), NORM))

    for cp in x_cp:
        cp.wait()
    _weave((chain(load_x(0), norm(0), norm(4)), 56))
    for cp in a_cp[0]:
        cp.wait()
    _weave((chain(*[prep_a(0, c, c % 2) for c in range(8)]), 48))
    for jj in range(1, 4):
        _weave((a_proj(0, 0, jj - 1), 6), (chain(load_x(jj), norm(jj), norm(4 + jj)), 56))
    _weave((a_proj(0, 0, 3), 6))
    layer_a(True)
    layer_b()
    _weave((a_proj(0, 0, 0), 6), (norm(7), NORM))
    loop(1, 4, lambda jj: [(a_proj(0, 0, jj), 6)])
    layer_a(False)
    layer_b()
    for jj in range(4):
        store_x(jj, 0)
    o_cp = [pltpu.make_async_copy(xio.at[c], out_hbm.at[:, ds(c, 128)], osems.at[c]) for c in range(8)]
    for cp in o_cp:
        cp.start()
    for cp in o_cp:
        cp.wait()


@jax.jit
def pallas_interleave_layers__sliding_local_dilated__linear_kernel_hedgehog__prompt_kernel(
        A_x, A_wqkv, A_wo, B_x, B_wqkv, B_w_phi, B_wo):
    del B_x
    vm = pl.BlockSpec(memory_space=pltpu.VMEM)
    hbm = pl.BlockSpec(memory_space=pl.ANY)
    V = pltpu.VMEM
    out = pl.pallas_call(
        _kernel,
        in_specs=[hbm] * 4 + [vm, hbm],
        out_specs=hbm,
        out_shape=jax.ShapeDtypeStruct((S, D), BF16),
        scratch_shapes=[
            V((8, S, 128), BF16), V((4, 3, D, 256), BF16), V((D, D), BF16), V((D, 3 * D), BF16), V((D, D), BF16),
            pltpu.SemaphoreType.DMA((23,)), pltpu.SemaphoreType.DMA((8,)), V((8, 128, 128), BF16),
            V((4, 8, 768, 128), BF16), V((8, 128, D), BF16), V((3, 8, D, 128), BF16), V((8, 128, D), BF16),
            V((8, D, 256), F32), V((8, D, 256), BF16), V((8, D, 256), BF16),
            V((8, 256, 128), F32), V((16, 256, 128), F32), V((16, 256, 128), F32),
            V((8, 256, 128), F32), V((16, 256, 128), F32), V((16, 256, 128), F32),
            V((8, 256, 128), F32), V((8, 128, 128), F32), V((8, 256, 128), F32), V((8, 128, 128), BF16),
        ],
        compiler_params=pltpu.CompilerParams(vmem_limit_bytes=110 * 1024 * 1024),
    )(A_x.reshape(S, D), A_wqkv, A_wo, B_wqkv, B_w_phi.reshape(D, DH), B_wo)
    return out.reshape(1, S, D)
```

```python
import jax
import jax.numpy as jnp
from jax import lax
import jax.experimental.pallas as pl
import jax.experimental.pallas.tpu as pltpu

S, D, H, DH = 2048, 1024, 32, 32
W = 8
NC = S // 128
F32, BF16 = jnp.float32, jnp.bfloat16
NT = (((1,), (1,)), ((), ()))


def _mm(a, b):
    return jnp.dot(a, b, preferred_element_type=F32)


def _tree(f, xs):
    xs = list(xs)
    while len(xs) > 1:
        xs = [f(xs[i], xs[i + 1]) for i in range(0, len(xs), 2)]
    return xs[0]


def _weave(*gens):
    order = sorted(((k + (0.5 if gi else 0)) / n, gi) for gi, (_, n) in enumerate(gens) for k in range(n))
    for _, gi in order:
        next(gens[gi][0], None)
    for g, _ in gens:
        for _ in g:
            pass


NORM = 24


def _kernel(x_hbm, awqkv_hbm, awo_hbm, bwqkv_hbm, bphi, bwo_hbm, out_hbm,
            xio, awqkv, awo, bwqkv, bwo, sems, osems, bds,
            wa, woa, wb, wob, xt, xn, ot, q0, k0, v0, q1, k1, v1, tmp, kvacc, zacc, kvm):
    qkv_buf = ((q0, k0, v0), (q1, k1, v1))

    def norm(i):
        acc = None
        for r in range(8):
            t = _tree(jnp.add, [xt[i, r * 128 + k * 8:r * 128 + k * 8 + 8, :] for k in range(16)])
            acc = t if r == 0 else acc + t
            yield
        m = jnp.sum(acc, axis=0, keepdims=True) * (1.0 / D)
        for r in range(8):
            d = xt[i, r * 128:(r + 1) * 128, :] - m
            d = d * d
            t = _tree(jnp.add, [d[k * 8:k * 8 + 8] for k in range(16)])
            acc = t if r == 0 else acc + t
            yield
        inv = lax.rsqrt(jnp.sum(acc, axis=0, keepdims=True) * (1.0 / D) + 1e-5)
        for r in range(8):
            sl = slice(r * 128, (r + 1) * 128)
            xn[i, sl, :] = ((xt[i, sl, :] - m) * inv).astype(BF16)
            yield

    def norm_now(i):
        _weave((norm(i), NORM))

    def ds(i, n):
        return pl.ds(pl.multiple_of(i * n, n), n)

    def wrows(ref, g, r):
        return jnp.concatenate([ref[g, k, r * 128:(r + 1) * 128, :] for k in range(8)], axis=1)

    x_cp = [pltpu.make_async_copy(x_hbm.at[:, ds(c, 128)], xio.at[c], sems.at[c]) for c in range(8)]
    a_cp = [[pltpu.make_async_copy(awqkv_hbm.at[:, ds(t * 4 + g, 256)], awqkv.at[g, t], sems.at[8 + g * 3 + t])
             for t in range(3)] for g in range(4)]
    ao_cp = pltpu.make_async_copy(awo_hbm, awo, sems.at[20])
    b_cp = [pltpu.make_async_copy(bwqkv_hbm, bwqkv, sems.at[21]),
            pltpu.make_async_copy(bwo_hbm, bwo, sems.at[22])]
    for cp in a_cp[0] + x_cp:
        cp.start()

    def tr(blk):
        return blk.astype(F32).T

    def put(slot, val):
        for h in range(8):
            tmp[slot, h * (DH + 1):h * (DH + 1) + DH, :] = val[h * DH:(h + 1) * DH]

    def prep_a(g, c, u):
        for t in range(3):
            put(u * 4 + t, tr(awqkv[g, t, ds(c, 128), :]))
            yield
            r = jnp.concatenate([tmp[u * 4 + t, pl.ds(d, 8, stride=DH + 1), :] for d in range(DH)], axis=0)
            wa[g, c, t * 256:(t + 1) * 256, :] = r.astype(BF16)
            yield

    def prep_ao(g, c, u):
        put(u * 4 + 3, awo[ds(g, 256), ds(c, 128)].astype(F32))
        yield
        r = jnp.concatenate([tmp[u * 4 + 3, pl.ds(d, 8, stride=DH + 1), :] for d in range(DH)], axis=0)
        woa[c, :, ds(g, 256)] = r.T.astype(BF16)
        yield

    def prep_b(g, c):
        wob[c, :, ds(g, 256)] = tr(bwo[ds(g, 256), ds(c, 128)]).astype(BF16)
        yield
        wb[2, c, ds(g, 256), :] = tr(bwqkv[ds(c, 128), ds(8 + g, 256)]).astype(BF16)
        yield
        for t in range(2):
            for h in range(2):
                wsl = bwqkv[ds(c, 128), ds(t * 8 + 2 * g + h, 128)]
                wb[t, c, ds(2 * g + h, 128), :] = lax.dot_general(
                    bds[2 * g + h], wsl, NT, preferred_element_type=F32).astype(BF16)
            yield

    f_i = lax.broadcasted_iota(jnp.int32, (DH, 128), 0)
    f_j = lax.broadcasted_iota(jnp.int32, (DH, 128), 1)
    rep = _mm(bphi[...], jnp.where(f_i == f_j % 64 // 2, 1.0, 0.0).astype(BF16))
    e_i = lax.broadcasted_iota(jnp.int32, (128, 128), 0)
    e_j = lax.broadcasted_iota(jnp.int32, (128, 128), 1)
    for g in range(8):
        bds[g] = jnp.where(e_i // 64 * 2 + e_i % 2 == e_j // DH, rep[g * 128:(g + 1) * 128].T, 0.0).astype(BF16)

    xio32 = xio.bitcast(jnp.uint32)

    def load_x(jj):
        for c in range(8):
            for h in range(2):
                w = xio32[c, pl.ds(2 * jj + h, 128, stride=8), :].T
                for p in range(2):
                    bits = (w << 16) if p == 0 else (w & jnp.uint32(0xFFFF0000))
                    xt[p * 4 + jj, c * 128:(c + 1) * 128, h * 128:(h + 1) * 128] = (
                        lax.bitcast_convert_type(bits, F32))
            yield

    def chain(*gens):
        for g in gens:
            yield from g

    def store_x(c):
        for jj in range(4):
            for h in range(2):
                e, o = [lax.bitcast_convert_type(
                    xt[p * 4 + jj, c * 128:(c + 1) * 128, h * 128:(h + 1) * 128].astype(BF16).astype(F32),
                    jnp.uint32) for p in range(2)]
                xio32[c, pl.ds(2 * jj + h, 128, stride=8), :] = ((e >> 16) | o).T

    def out_proj(i, w_ref):
        o = ot[i]
        for r in range(8):
            sl = slice(r * 128, (r + 1) * 128)
            xt[i, sl, :] += _mm(w_ref[r], o)
            yield

    def a_proj(g, p, jj):
        qr, kr, vr = qkv_buf[p]
        j = 2 * jj
        xin = xn[p * 4 + jj]
        for r in range(6):
            t = _mm(wrows(wa, g, r), xin)
            sl = slice((r % 2) * 128, (r % 2 + 1) * 128)
            for i in range(2):
                ti = t[:, i * 128:(i + 1) * 128]
                if r < 2:
                    qr[j + i, sl, :] = ti * (DH ** -0.5)
                else:
                    dst = kr if r < 4 else vr
                    dst[8 + j + i, sl, :] = ti
                    dst[j + i, sl, :] = pltpu.roll(ti, 1, 1)
            yield

    lane0 = lax.broadcasted_iota(jnp.int32, (8, 128), 1) == 0

    def a_attn(g, p, jj):
        qr, kr, vr = qkv_buf[p]
        j = 2 * jj
        lg = [[None] * W for _ in range(2)]
        for d in range(DH):
            sl = slice(d * 8, d * 8 + 8)
            kk = [kr[j + 1 + i, sl, :] for i in range(W + 1)]
            for i in range(2):
                q = qr[j + i, sl, :]
                for w in range(W):
                    t = q * kk[7 + i - w]
                    lg[i][w] = t if d == 0 else lg[i][w] + t
            yield
        pr = []
        for i in range(2):
            l = [lg[i][0]] + [jnp.where(lane0 & (j + i < w), -1e9, lg[i][w]) for w in range(1, W)]
            m = _tree(jnp.maximum, l)
            e = [jnp.exp(t - m) for t in l]
            inv = 1.0 / _tree(jnp.add, e)
            pr.append([t * inv for t in e])
            yield
        off = pl.multiple_of(g * 256, 256)
        for d in range(0, DH, 2):
            o = [[], []]
            for dd in (d, d + 1):
                sl = slice(dd * 8, dd * 8 + 8)
                vv = [vr[j + 1 + i, sl, :] for i in range(W + 1)]
                for i in range(2):
                    o[i].append(_tree(jnp.add, [pr[i][w] * vv[7 + i - w] for w in range(W)]))
                if dd == d:
                    yield
            ot[p * 4 + jj, pl.ds(pl.multiple_of(off + d * 8, 16), 16), :] = jnp.concatenate(
                [jnp.concatenate(o[i], axis=0) for i in range(2)], axis=1).astype(BF16)
            yield

    def loop(lo, hi, make, u=2):
        if (hi - lo) % u:
            u = hi - lo

        def body(k, _):
            parts = [make(lo + k * u + t) for t in range(u)]
            _weave(*[(chain(*[take(*pt[a]) for pt in parts]), u * parts[0][a][1])
                     for a in range(len(parts[0]))])
            return 0
        lax.fori_loop(0, (hi - lo) // u, body, 0)

    def take(gen, n):
        for _ in range(n):
            next(gen, None)
            yield
        for _ in gen:
            pass

    def layer_a(first):
        def part(g, p):
            def make(jj):
                gens = [(a_proj(g + p, 1 - p, jj), 6), (a_attn(g, p, jj), 66)]
                if first:
                    for u in range(2):
                        c = 2 * jj + u
                        if p == 1:
                            gens.append((prep_b(g, c), 4))
                        else:
                            gens.append((prep_ao(g, c, u), 2))
                            if not (isinstance(g, int) and g == 3):
                                gens.append((prep_a(g + 1, c, u), 6))
                return gens
            loop(0, 4, make)

        def grp(g, _):
            if first:
                @pl.when(g == 0)
                def _():
                    for cp in a_cp[1] + [ao_cp]:
                        cp.wait()
                    for cp in a_cp[2] + b_cp + a_cp[3]:
                        cp.start()
                for k in (2, 3):
                    @pl.when(g == k - 1)
                    def _():
                        for cp in a_cp[k]:
                            cp.wait()
            part(g, 0)
            if first:
                @pl.when(g == 0)
                def _():
                    for cp in b_cp:
                        cp.wait()
            part(g, 1)
            return 0
        lax.fori_loop(0, 3, grp, 0)
        part(3, 0)
        _weave((out_proj(0, woa), 8), (a_attn(3, 1, 0), 66))
        loop(1, 4, lambda i: [(out_proj(i, woa), 8), (a_attn(3, 1, i), 66), (norm(i - 1), NORM)])
        loop(4, 8, lambda i: [(out_proj(i, woa), 8), (norm(i - 1), NORM)] + (
            [(prep_b(3, 2 * i - 8), 4), (prep_b(3, 2 * i - 7), 4)] if first else []))

    def allred(f, x):
        out = []
        for a in range(2):
            r = _tree(f, [x[a * 64 + i * 8:a * 64 + i * 8 + 8] for i in range(8)])
            r = f(r, pltpu.roll(r, 4, 0))
            out.append(f(r, pltpu.roll(r, 2, 0)))
        return out

    def bc(r):
        return jnp.concatenate([r[0]] * 8 + [r[1]] * 8, axis=0)

    def feat(p, g, is_q):
        ep = jnp.exp(p - bc(allred(jnp.maximum, p)))
        en = jnp.exp(bc(allred(jnp.minimum, p)) - p)
        ip = [1.0 / t for t in allred(jnp.add, ep)]
        im = [1.0 / t for t in allred(jnp.add, en)]
        if is_q:
            dp = allred(jnp.add, ep * jnp.tile(zacc[g, :128], (1, 2)))
            dn = allred(jnp.add, en * jnp.tile(zacc[g, 128:], (1, 2)))
            r = [1.0 / (dp[a] * ip[a] + dn[a] * im[a] + 1e-6) for a in range(2)]
            ip = [ip[a] * r[a] for a in range(2)]
            im = [im[a] * r[a] for a in range(2)]
        ep, en = ep * bc(ip), en * bc(im)
        if not is_q:
            zacc[g, :128] += ep[:, :128] + ep[:, 128:]
            zacc[g, 128:] += en[:, :128] + en[:, 128:]
        return [jnp.concatenate([ep[a * 64:(a + 1) * 64], en[a * 64:(a + 1) * 64]], axis=0).astype(BF16)
                for a in range(2)]

    def b_kv(i):
        xin = xn[i]
        phis = []
        for g in range(9):
            if g < 8:
                pk = _mm(wrows(wb, 1, g), xin) if g == 0 else nxt
                if g < 7:
                    nxt = _mm(wrows(wb, 1, g + 1), xin)
                v = _mm(wrows(wb, 2, g), xin).astype(BF16)
            if g > 0:
                v1, ph = phis[g - 1]
                kvacc[g - 1] += jnp.concatenate(
                    [lax.dot_general(v1[a * 64:(a + 1) * 64], ph[a], NT, preferred_element_type=F32)
                     for a in range(2)], axis=0)
            yield
            if g < 8:
                phis.append((v, feat(pk, g, False)))

    def b_fin(g):
        r_i = lax.broadcasted_iota(jnp.int32, (128, 128), 0)
        r_j = lax.broadcasted_iota(jnp.int32, (128, 128), 1)
        kvm[g] = jnp.where(r_i // DH % 2 == r_j % 2, kvacc[g], 0.0).astype(BF16)
        zacc[g] = jnp.broadcast_to(jnp.sum(zacc[g], axis=1, keepdims=True), (256, 128))

    def b_q(i, first=False):
        xin = xn[i]
        phis = []
        for g in range(9):
            if g < 8:
                pq = _mm(wrows(wb, 0, g), xin) if g == 0 else nxt
                if g < 7:
                    nxt = _mm(wrows(wb, 0, g + 1), xin)
            if g > 0:
                ot[i, (g - 1) * 128:g * 128, :] = jnp.concatenate(
                    [_mm(kvm[g - 1, a * 64:(a + 1) * 64], phis[g - 1][a]) for a in range(2)],
                    axis=0).astype(BF16)
            yield
            if g < 8:
                if first:
                    b_fin(g)
                phis.append(feat(pq, g, True))

    def layer_b():
        zacc[...] = jnp.zeros_like(zacc)
        kvacc[...] = jnp.zeros_like(kvacc)
        _weave((b_kv(0), 9), (norm(7), NORM * 2))
        loop(1, 8, lambda i: [(b_kv(i), 9)], 1)
        _weave((b_q(0, True), 9))
        _weave((out_proj(0, wob), 8), (b_q(1), 9))
        loop(2, 8, lambda i: [(norm(i - 2), NORM), (out_proj(i - 1, wob), 8), (b_q(i), 9)])
        _weave((out_proj(7, wob), 8), (norm(6), NORM))

    for cp in a_cp[0]:
        cp.wait()
    _weave((chain(*[prep_a(0, c, c % 2) for c in range(8)]), 48))
    for cp in x_cp:
        cp.wait()
    for cp in a_cp[1] + [ao_cp]:
        cp.start()
    _weave((chain(load_x(0), norm(0)), 32))
    for jj in range(1, 4):
        _weave((a_proj(0, 0, jj - 1), 6), (chain(load_x(jj), norm(jj), norm(3 + jj)), 56))
    _weave((a_proj(0, 0, 3), 6), (norm(7), NORM))
    layer_a(True)
    layer_b()
    _weave((a_proj(0, 0, 0), 6), (norm(7), NORM))
    loop(1, 4, lambda jj: [(a_proj(0, 0, jj), 6)])
    layer_a(False)
    layer_b()
    o_cp = [pltpu.make_async_copy(xio.at[c], out_hbm.at[:, ds(c, 128)], osems.at[c]) for c in range(8)]
    for c, cp in enumerate(o_cp):
        store_x(c)
        cp.start()
    for cp in o_cp:
        cp.wait()


@jax.jit
def pallas_interleave_layers__sliding_local_dilated__linear_kernel_hedgehog__prompt_kernel(
        A_x, A_wqkv, A_wo, B_x, B_wqkv, B_w_phi, B_wo):
    del B_x
    vm = pl.BlockSpec(memory_space=pltpu.VMEM)
    hbm = pl.BlockSpec(memory_space=pl.ANY)
    V = pltpu.VMEM
    out = pl.pallas_call(
        _kernel,
        in_specs=[hbm] * 4 + [vm, hbm],
        out_specs=hbm,
        out_shape=jax.ShapeDtypeStruct((S, D), BF16),
        scratch_shapes=[
            V((8, S, 128), BF16), V((4, 3, D, 256), BF16), V((D, D), BF16), V((D, 3 * D), BF16), V((D, D), BF16),
            pltpu.SemaphoreType.DMA((23,)), pltpu.SemaphoreType.DMA((8,)), V((8, 128, 128), BF16),
            V((4, 8, 768, 128), BF16), V((8, 128, D), BF16), V((3, 8, D, 128), BF16), V((8, 128, D), BF16),
            V((8, D, 256), F32), V((8, D, 256), BF16), V((8, D, 256), BF16),
            V((8, 256, 128), F32), V((16, 256, 128), F32), V((16, 256, 128), F32),
            V((8, 256, 128), F32), V((16, 256, 128), F32), V((16, 256, 128), F32),
            V((8, 264, 128), F32), V((8, 128, 128), F32), V((8, 256, 128), F32), V((8, 128, 128), BF16),
        ],
        compiler_params=pltpu.CompilerParams(vmem_limit_bytes=110 * 1024 * 1024),
    )(A_x.reshape(S, D), A_wqkv, A_wo, B_wqkv, B_w_phi.reshape(D, DH), B_wo)
    return out.reshape(1, S, D)
```

```python
import jax
import jax.numpy as jnp
from jax import lax
import jax.experimental.pallas as pl
import jax.experimental.pallas.tpu as pltpu

S, D, H, DH = 2048, 1024, 32, 32
W = 8
NC = S // 128
F32, BF16 = jnp.float32, jnp.bfloat16
NT = (((1,), (1,)), ((), ()))


def _mm(a, b):
    return jnp.dot(a, b, preferred_element_type=F32)


def _tree(f, xs):
    xs = list(xs)
    while len(xs) > 1:
        xs = [f(xs[i], xs[i + 1]) for i in range(0, len(xs), 2)]
    return xs[0]


def _weave(*gens):
    order = sorted(((k + (0.5 if gi else 0)) / n, gi) for gi, (_, n) in enumerate(gens) for k in range(n))
    for _, gi in order:
        next(gens[gi][0], None)
    for g, _ in gens:
        for _ in g:
            pass


NORM = 24


def _kernel(x_hbm, awqkv_hbm, awo_hbm, bwqkv_hbm, bphi, bwo_hbm, out_hbm,
            xio, awqkv, awo, bwqkv, bwo, sems, osems, bds,
            wa, woa, wb, wob, xt, xn, ot, q0, k0, v0, q1, k1, v1, tmp, kvacc, zacc, kvm):
    qkv_buf = ((q0, k0, v0), (q1, k1, v1))

    def norm(i):
        acc = None
        for r in range(8):
            t = _tree(jnp.add, [xt[i, r * 128 + k * 8:r * 128 + k * 8 + 8, :] for k in range(16)])
            acc = t if r == 0 else acc + t
            yield
        m = jnp.sum(acc, axis=0, keepdims=True) * (1.0 / D)
        for r in range(8):
            d = xt[i, r * 128:(r + 1) * 128, :] - m
            d = d * d
            t = _tree(jnp.add, [d[k * 8:k * 8 + 8] for k in range(16)])
            acc = t if r == 0 else acc + t
            yield
        inv = lax.rsqrt(jnp.sum(acc, axis=0, keepdims=True) * (1.0 / D) + 1e-5)
        for r in range(8):
            sl = slice(r * 128, (r + 1) * 128)
            xn[i, sl, :] = ((xt[i, sl, :] - m) * inv).astype(BF16)
            yield

    def norm_now(i):
        _weave((norm(i), NORM))

    def ds(i, n):
        return pl.ds(pl.multiple_of(i * n, n), n)

    def wrows(ref, g, r):
        return jnp.concatenate([ref[g, k, r * 128:(r + 1) * 128, :] for k in range(8)], axis=1)

    x_cp = [pltpu.make_async_copy(x_hbm.at[:, ds(c, 128)], xio.at[c], sems.at[c]) for c in range(8)]
    a_cp = [[pltpu.make_async_copy(awqkv_hbm.at[:, ds(t * 4 + g, 256)], awqkv.at[g, t], sems.at[8 + g * 3 + t])
             for t in range(3)] for g in range(4)]
    ao_cp = pltpu.make_async_copy(awo_hbm, awo, sems.at[20])
    b_cp = [pltpu.make_async_copy(bwqkv_hbm, bwqkv, sems.at[21]),
            pltpu.make_async_copy(bwo_hbm, bwo, sems.at[22])]
    for cp in a_cp[0] + x_cp:
        cp.start()

    def tr(blk):
        return blk.astype(F32).T

    def put(slot, val):
        for h in range(8):
            tmp[slot, h * (DH + 1):h * (DH + 1) + DH, :] = val[h * DH:(h + 1) * DH]

    def prep_a(g, c, u):
        for t in range(3):
            put(u * 4 + t, tr(awqkv[g, t, ds(c, 128), :]))
            yield
            r = jnp.concatenate([tmp[u * 4 + t, pl.ds(d, 8, stride=DH + 1), :] for d in range(DH)], axis=0)
            wa[g, c, t * 256:(t + 1) * 256, :] = r.astype(BF16)
            yield

    def prep_ao(g, c, u):
        put(u * 4 + 3, awo[ds(g, 256), ds(c, 128)].astype(F32))
        yield
        r = jnp.concatenate([tmp[u * 4 + 3, pl.ds(d, 8, stride=DH + 1), :] for d in range(DH)], axis=0)
        woa[c, :, ds(g, 256)] = r.T.astype(BF16)
        yield

    def prep_b(g, c):
        wob[c, :, ds(g, 256)] = tr(bwo[ds(g, 256), ds(c, 128)]).astype(BF16)
        yield
        wb[2, c, ds(g, 256), :] = tr(bwqkv[ds(c, 128), ds(8 + g, 256)]).astype(BF16)
        yield
        for t in range(2):
            for h in range(2):
                wsl = bwqkv[ds(c, 128), ds(t * 8 + 2 * g + h, 128)]
                wb[t, c, ds(2 * g + h, 128), :] = lax.dot_general(
                    bds[2 * g + h], wsl, NT, preferred_element_type=F32).astype(BF16)
            yield

    f_i = lax.broadcasted_iota(jnp.int32, (DH, 128), 0)
    f_j = lax.broadcasted_iota(jnp.int32, (DH, 128), 1)
    rep = _mm(bphi[...], jnp.where(f_i == f_j % 64 // 2, 1.0, 0.0).astype(BF16))
    e_i = lax.broadcasted_iota(jnp.int32, (128, 128), 0)
    e_j = lax.broadcasted_iota(jnp.int32, (128, 128), 1)
    for g in range(8):
        bds[g] = jnp.where(e_i // 64 * 2 + e_i % 2 == e_j // DH, rep[g * 128:(g + 1) * 128].T, 0.0).astype(BF16)

    xio32 = xio.bitcast(jnp.uint32)

    def load_x(jj):
        for c in range(8):
            for h in range(2):
                w = xio32[c, pl.ds(2 * jj + h, 128, stride=8), :].T
                for p in range(2):
                    bits = (w << 16) if p == 0 else (w & jnp.uint32(0xFFFF0000))
                    xt[p * 4 + jj, c * 128:(c + 1) * 128, h * 128:(h + 1) * 128] = (
                        lax.bitcast_convert_type(bits, F32))
            yield

    def chain(*gens):
        for g in gens:
            yield from g

    def store_x(c):
        for jj in range(4):
            for h in range(2):
                e, o = [lax.bitcast_convert_type(
                    xt[p * 4 + jj, c * 128:(c + 1) * 128, h * 128:(h + 1) * 128].astype(BF16).astype(F32),
                    jnp.uint32) for p in range(2)]
                xio32[c, pl.ds(2 * jj + h, 128, stride=8), :] = ((e >> 16) | o).T

    def out_proj(i, w_ref):
        o = ot[i]
        for r in range(8):
            sl = slice(r * 128, (r + 1) * 128)
            xt[i, sl, :] += _mm(w_ref[r], o)
            yield

    def a_proj(g, p, jj):
        qr, kr, vr = qkv_buf[p]
        j = 2 * jj
        xin = xn[p * 4 + jj]
        for r in range(6):
            t = _mm(wrows(wa, g, r), xin)
            sl = slice((r % 2) * 128, (r % 2 + 1) * 128)
            for i in range(2):
                ti = t[:, i * 128:(i + 1) * 128]
                if r < 2:
                    qr[j + i, sl, :] = ti * (DH ** -0.5)
                else:
                    dst = kr if r < 4 else vr
                    dst[8 + j + i, sl, :] = ti
                    dst[j + i, sl, :] = pltpu.roll(ti, 1, 1)
            yield

    lane0 = lax.broadcasted_iota(jnp.int32, (8, 128), 1) == 0

    def a_attn(g, p, jj):
        qr, kr, vr = qkv_buf[p]
        j = 2 * jj
        lg = [[None] * W for _ in range(2)]
        for d in range(DH):
            sl = slice(d * 8, d * 8 + 8)
            kk = [kr[j + 1 + i, sl, :] for i in range(W + 1)]
            for i in range(2):
                q = qr[j + i, sl, :]
                for w in range(W):
                    t = q * kk[7 + i - w]
                    lg[i][w] = t if d == 0 else lg[i][w] + t
            yield
        pr = []
        for i in range(2):
            l = [lg[i][0]] + [jnp.where(lane0 & (j + i < w), -1e9, lg[i][w]) for w in range(1, W)]
            m = _tree(jnp.maximum, l)
            e = [jnp.exp(t - m) for t in l]
            inv = 1.0 / _tree(jnp.add, e)
            pr.append([t * inv for t in e])
            yield
        off = pl.multiple_of(g * 256, 256)
        for d in range(0, DH, 2):
            o = [[], []]
            for dd in (d, d + 1):
                sl = slice(dd * 8, dd * 8 + 8)
                vv = [vr[j + 1 + i, sl, :] for i in range(W + 1)]
                for i in range(2):
                    o[i].append(_tree(jnp.add, [pr[i][w] * vv[7 + i - w] for w in range(W)]))
                if dd == d:
                    yield
            ot[p * 4 + jj, pl.ds(pl.multiple_of(off + d * 8, 16), 16), :] = jnp.concatenate(
                [jnp.concatenate(o[i], axis=0) for i in range(2)], axis=1).astype(BF16)
            yield

    def loop(lo, hi, make, u=2):
        if (hi - lo) % u:
            u = hi - lo

        def body(k, _):
            parts = [make(lo + k * u + t) for t in range(u)]
            _weave(*[(chain(*[take(*pt[a]) for pt in parts]), u * parts[0][a][1])
                     for a in range(len(parts[0]))])
            return 0
        lax.fori_loop(0, (hi - lo) // u, body, 0)

    def take(gen, n):
        for _ in range(n):
            next(gen, None)
            yield
        for _ in gen:
            pass

    def layer_a(first):
        def part(g, p):
            def make(jj):
                gens = [(a_proj(g + p, 1 - p, jj), 6), (a_attn(g, p, jj), 66)]
                if first:
                    for u in range(2):
                        c = 2 * jj + u
                        if p == 1:
                            gens.append((prep_b(g, c), 4))
                        else:
                            gens.append((prep_ao(g, c, u), 2))
                            if not (isinstance(g, int) and g == 3):
                                gens.append((prep_a(g + 1, c, u), 6))
                return gens
            loop(0, 4, make)

        def grp(g, _):
            if first:
                @pl.when(g == 0)
                def _():
                    for cp in a_cp[1] + [ao_cp]:
                        cp.wait()
                    for cp in a_cp[2] + b_cp + a_cp[3]:
                        cp.start()
                for k in (2, 3):
                    @pl.when(g == k - 1)
                    def _():
                        for cp in a_cp[k]:
                            cp.wait()
            part(g, 0)
            if first:
                @pl.when(g == 0)
                def _():
                    for cp in b_cp:
                        cp.wait()
            if first:
                part(g, 1)
            else:
                pl.when(g < 3)(lambda: part(g, 1))
            return 0
        lax.fori_loop(0, 3 if first else 4, grp, 0)
        if first:
            part(3, 0)
        _weave((out_proj(0, woa), 8), (a_attn(3, 1, 0), 66))
        loop(1, 4, lambda i: [(out_proj(i, woa), 8), (a_attn(3, 1, i), 66), (norm(i - 1), NORM)])
        loop(4, 8, lambda i: [(out_proj(i, woa), 8), (norm(i - 1), NORM)] + (
            [(prep_b(3, 2 * i - 8), 4), (prep_b(3, 2 * i - 7), 4)] if first else []))

    def allred(f, x):
        out = []
        for a in range(2):
            r = _tree(f, [x[a * 64 + i * 8:a * 64 + i * 8 + 8] for i in range(8)])
            r = f(r, pltpu.roll(r, 4, 0))
            out.append(f(r, pltpu.roll(r, 2, 0)))
        return out

    def bc(r):
        return jnp.concatenate([r[0]] * 8 + [r[1]] * 8, axis=0)

    def feat(p, g, is_q):
        ep = jnp.exp(p - bc(allred(jnp.maximum, p)))
        en = jnp.exp(bc(allred(jnp.minimum, p)) - p)
        ip = [1.0 / t for t in allred(jnp.add, ep)]
        im = [1.0 / t for t in allred(jnp.add, en)]
        if is_q:
            dp = allred(jnp.add, ep * jnp.tile(zacc[g, :128], (1, 2)))
            dn = allred(jnp.add, en * jnp.tile(zacc[g, 128:], (1, 2)))
            r = [1.0 / (dp[a] * ip[a] + dn[a] * im[a] + 1e-6) for a in range(2)]
            ip = [ip[a] * r[a] for a in range(2)]
            im = [im[a] * r[a] for a in range(2)]
        ep, en = ep * bc(ip), en * bc(im)
        if not is_q:
            zacc[g, :128] += ep[:, :128] + ep[:, 128:]
            zacc[g, 128:] += en[:, :128] + en[:, 128:]
        return [jnp.concatenate([ep[a * 64:(a + 1) * 64], en[a * 64:(a + 1) * 64]], axis=0).astype(BF16)
                for a in range(2)]

    def b_kv(i):
        xin = xn[i]
        phis = []
        for g in range(9):
            if g < 8:
                pk = _mm(wrows(wb, 1, g), xin) if g == 0 else nxt
                if g < 7:
                    nxt = _mm(wrows(wb, 1, g + 1), xin)
                v = _mm(wrows(wb, 2, g), xin).astype(BF16)
            if g > 0:
                v1, ph = phis[g - 1]
                kvacc[g - 1] += jnp.concatenate(
                    [lax.dot_general(v1[a * 64:(a + 1) * 64], ph[a], NT, preferred_element_type=F32)
                     for a in range(2)], axis=0)
            yield
            if g < 8:
                phis.append((v, feat(pk, g, False)))

    def b_fin(g):
        r_i = lax.broadcasted_iota(jnp.int32, (128, 128), 0)
        r_j = lax.broadcasted_iota(jnp.int32, (128, 128), 1)
        kvm[g] = jnp.where(r_i // DH % 2 == r_j % 2, kvacc[g], 0.0).astype(BF16)
        zacc[g] = jnp.broadcast_to(jnp.sum(zacc[g], axis=1, keepdims=True), (256, 128))

    def b_q(i, first=False):
        xin = xn[i]
        phis = []
        for g in range(9):
            if g < 8:
                pq = _mm(wrows(wb, 0, g), xin) if g == 0 else nxt
                if g < 7:
                    nxt = _mm(wrows(wb, 0, g + 1), xin)
            if g > 0:
                ot[i, (g - 1) * 128:g * 128, :] = jnp.concatenate(
                    [_mm(kvm[g - 1, a * 64:(a + 1) * 64], phis[g - 1][a]) for a in range(2)],
                    axis=0).astype(BF16)
            yield
            if g < 8:
                if first:
                    b_fin(g)
                phis.append(feat(pq, g, True))

    def layer_b():
        zacc[...] = jnp.zeros_like(zacc)
        kvacc[...] = jnp.zeros_like(kvacc)
        _weave((b_kv(0), 9), (norm(7), NORM * 2))
        loop(1, 8, lambda i: [(b_kv(i), 9)], 1)
        _weave((b_q(0, True), 9))
        _weave((out_proj(0, wob), 8), (b_q(1), 9))
        loop(2, 8, lambda i: [(norm(i - 2), NORM), (out_proj(i - 1, wob), 8), (b_q(i), 9)], 1)
        _weave((out_proj(7, wob), 8), (norm(6), NORM))

    for cp in a_cp[0]:
        cp.wait()
    _weave((chain(*[prep_a(0, c, c % 2) for c in range(8)]), 48))
    for cp in x_cp:
        cp.wait()
    for cp in a_cp[1] + [ao_cp]:
        cp.start()
    _weave((chain(load_x(0), norm(0)), 32))
    for jj in range(1, 4):
        _weave((a_proj(0, 0, jj - 1), 6), (chain(load_x(jj), norm(jj), norm(3 + jj)), 56))
    _weave((a_proj(0, 0, 3), 6), (norm(7), NORM))
    layer_a(True)
    layer_b()
    _weave((a_proj(0, 0, 0), 6), (norm(7), NORM))
    loop(1, 4, lambda jj: [(a_proj(0, 0, jj), 6)])
    layer_a(False)
    layer_b()
    o_cp = [pltpu.make_async_copy(xio.at[c], out_hbm.at[:, ds(c, 128)], osems.at[c]) for c in range(8)]
    for c, cp in enumerate(o_cp):
        store_x(c)
        cp.start()
    for cp in o_cp:
        cp.wait()


@jax.jit
def pallas_interleave_layers__sliding_local_dilated__linear_kernel_hedgehog__prompt_kernel(
        A_x, A_wqkv, A_wo, B_x, B_wqkv, B_w_phi, B_wo):
    del B_x
    vm = pl.BlockSpec(memory_space=pltpu.VMEM)
    hbm = pl.BlockSpec(memory_space=pl.ANY)
    V = pltpu.VMEM
    out = pl.pallas_call(
        _kernel,
        in_specs=[hbm] * 4 + [vm, hbm],
        out_specs=hbm,
        out_shape=jax.ShapeDtypeStruct((S, D), BF16),
        scratch_shapes=[
            V((8, S, 128), BF16), V((4, 3, D, 256), BF16), V((D, D), BF16), V((D, 3 * D), BF16), V((D, D), BF16),
            pltpu.SemaphoreType.DMA((23,)), pltpu.SemaphoreType.DMA((8,)), V((8, 128, 128), BF16),
            V((4, 8, 768, 128), BF16), V((8, 128, D), BF16), V((3, 8, D, 128), BF16), V((8, 128, D), BF16),
            V((8, D, 256), F32), V((8, D, 256), BF16), V((8, D, 256), BF16),
            V((8, 256, 128), F32), V((16, 256, 128), F32), V((16, 256, 128), F32),
            V((8, 256, 128), F32), V((16, 256, 128), F32), V((16, 256, 128), F32),
            V((8, 264, 128), F32), V((8, 128, 128), F32), V((8, 256, 128), F32), V((8, 128, 128), BF16),
        ],
        compiler_params=pltpu.CompilerParams(vmem_limit_bytes=110 * 1024 * 1024),
    )(A_x.reshape(S, D), A_wqkv, A_wo, B_wqkv, B_w_phi.reshape(D, DH), B_wo)
    return out.reshape(1, S, D)
```

```python
import functools

import numpy as np
import jax
import jax.numpy as jnp
from jax import lax
import jax.experimental.pallas as pl
import jax.experimental.pallas.tpu as pltpu

S, D, H, DH = 2048, 1024, 32, 32
W = 8
NC = S // 128
F32, BF16, U32 = jnp.float32, jnp.bfloat16, jnp.uint32
NT = (((1,), (1,)), ((), ()))


def _mm(a, b):
    return jnp.dot(a, b, preferred_element_type=F32)


def _pk(x):
    return pltpu.bitcast(x.astype(BF16), U32)


def _up(x):
    return pltpu.bitcast(x, BF16)


def _half(w, p):
    return lax.bitcast_convert_type((w << 16) if p == 0 else (w & jnp.uint32(0xFFFF0000)), F32)


def _tree(f, xs):
    xs = list(xs)
    while len(xs) > 1:
        xs = [f(xs[i], xs[i + 1]) for i in range(0, len(xs), 2)]
    return xs[0]


def _weave(*gens):
    order = sorted(((k + (0.5 if gi else 0)) / n, gi) for gi, (_, n) in enumerate(gens) for k in range(n))
    for _, gi in order:
        next(gens[gi][0], None)
    for g, _ in gens:
        for _ in g:
            pass


NORM = 24


def _kernel(zero_ref, x_hbm, awqkv_hbm, awo_hbm, bwqkv_hbm, bphi, bwo_hbm, out_hbm,
            xio, awqkv, awo, bwqkv, bwo, sems, osems, bds,
            wa, woa, wb, wob, xt, xn, ot, q0, k0, v0, q1, k1, v1, tmp, kvacc, zacc, kvm):
    never = lax.broadcasted_iota(jnp.int32, (8, 128), 0) < zero_ref[0]
    pace = []

    def gate(xs):
        if not pace:
            return xs
        t = pace.pop()
        return [jnp.where(never, t, x) for x in xs]

    def chunks(n, lhs, x_ref, i, finish):
        for r in range(n):
            for k in range(0, 8, 2):
                yield
                t = _mm(_up(jnp.concatenate([lhs(r, k), lhs(r, k + 1)], axis=1)),
                        _up(jnp.concatenate([x_ref[i, h, k * 64:(k + 2) * 64, :] for h in range(2)], axis=1)))
                acc = t if k == 0 else acc + t
                pace[:] = [t[:8, :128]]
            finish(r, acc)

    qkv_buf = ((q0, k0, v0), (q1, k1, v1))

    def norm(i):
        ms, invs = [], []
        for h in range(2):
            acc = None
            for r in range(4):
                t = _tree(jnp.add, [xt[i, h, r * 256 + k * 8:r * 256 + k * 8 + 8, :] for k in range(32)])
                acc = t if r == 0 else acc + t
                yield
            ms.append(jnp.sum(acc, axis=0, keepdims=True) * (1.0 / D))
        for h in range(2):
            acc = None
            for r in range(4):
                d = xt[i, h, r * 256:(r + 1) * 256, :] - ms[h]
                d = d * d
                t = _tree(jnp.add, [d[k * 8:k * 8 + 8] for k in range(32)])
                acc = t if r == 0 else acc + t
                yield
            invs.append(lax.rsqrt(jnp.sum(acc, axis=0, keepdims=True) * (1.0 / D) + 1e-5))
        for h in range(2):
            for r in range(4):
                for p in range(2):
                    x = xt[i, h, pl.ds(r * 256 + p, 128, stride=2), :]
                    xn[i, h, r * 128 + p * 64:r * 128 + p * 64 + 64, :] = _pk((x - ms[h]) * invs[h])
                yield

    def ds(i, n):
        return pl.ds(pl.multiple_of(i * n, n), n)

    def wrows(ref, g, r):
        return _up(jnp.concatenate([ref[g, k, r * 64:(r + 1) * 64, :] for k in range(8)], axis=1))

    def rhs(ref, i):
        return _up(jnp.concatenate([ref[i, 0], ref[i, 1]], axis=1))

    def lanes(src, dst, first, n, sem0):
        return [pltpu.make_async_copy(src.at[:, ds(first + c, 128)], dst.at[c], sems.at[sem0 + c])
                for c in range(n)]

    x_cp = lanes(x_hbm, xio, 0, 8, 0)
    a_cp = [[cp for t in range(3) for cp in lanes(awqkv_hbm, awqkv.at[g * 3 + t], t * 8 + g * 2, 2, 8 + g * 6 + t * 2)]
            for g in range(4)]
    ao_cp = lanes(awo_hbm, awo, 0, 8, 32)
    b_cp = lanes(bwqkv_hbm, bwqkv, 0, 24, 40) + lanes(bwo_hbm, bwo, 0, 8, 64)
    for cp in a_cp[0] + x_cp:
        cp.start()

    awqkv32, awo32, bwqkv32, bwo32 = [r.bitcast(U32) for r in (awqkv, awo, bwqkv, bwo)]

    def prep_a(g, c, t, u):
        for n in range(2):
            w = awqkv32[g * 3 + t, n, ds(c, 128), :].T
            for h in range(4):
                tmp[u, pl.ds((n * 4 + h) * (DH + 1), DH), :] = w[h * DH:(h + 1) * DH]
            yield
        for half in range(2):
            w = jnp.concatenate([tmp[u, pl.ds(half * 16 + d, 8, stride=DH + 1), :] for d in range(16)], axis=0)
            for p in range(2):
                wa[g, 2 * c + p, t * 128 + half * 64:t * 128 + half * 64 + 64, :] = _pk(_half(w, p))
            yield

    def prep_ao(g, c, u):
        w = awo32[c, ds(g, 128), :]
        for h in range(8):
            tmp[u, pl.ds(h * 17, 16), :] = w[h * 16:(h + 1) * 16]
        yield
        w = jnp.concatenate([tmp[u, pl.ds(d, 8, stride=17), :] for d in range(16)], axis=0).T
        for p in range(2):
            woa[c, 2 * g + p] = _pk(_half(w, p))
        yield

    def prep_b(g, c, n):
        w = bwo32[2 * c + n, ds(g, 128), :].T
        for p in range(2):
            wob[2 * c + n, 2 * g + p] = _pk(_half(w, p))
        yield
        w = bwqkv32[16 + 2 * g + n, ds(c, 128), :].T
        for p in range(2):
            wb[2, 2 * c + p, ds(2 * g + n, 64), :] = _pk(_half(w, p))
        yield
        for t in range(2):
            w = bwqkv32[t * 8 + 2 * g + n, ds(c, 128), :]
            for p in range(2):
                wb[t, 2 * c + p, ds(2 * g + n, 64), :] = _pk(lax.dot_general(
                    _up(bds[2 * g + n]), _half(w, p).astype(BF16), NT, preferred_element_type=F32))
            yield

    f_i = lax.broadcasted_iota(jnp.int32, (DH, 128), 0)
    f_j = lax.broadcasted_iota(jnp.int32, (DH, 128), 1)
    rep = _mm(bphi[...], jnp.where(f_i == f_j % 64 // 2, 1.0, 0.0).astype(BF16))
    e_i = lax.broadcasted_iota(jnp.int32, (128, 128), 0)
    e_j = lax.broadcasted_iota(jnp.int32, (128, 128), 1)
    for g in range(8):
        bds[g] = _pk(jnp.where(e_i // 64 * 2 + e_i % 2 == e_j // DH, rep[g * 128:(g + 1) * 128].T, 0.0))

    xio32 = xio.bitcast(U32)

    def load_x(jj):
        for c in range(8):
            for h in range(2):
                w = xio32[c, pl.ds(2 * jj + h, 128, stride=8), :].T
                for p in range(2):
                    xt[p * 4 + jj, h, c * 128:(c + 1) * 128, :] = _half(w, p)
            yield

    def chain(*gens):
        for g in gens:
            yield from g

    def store_x(c):
        for jj in range(4):
            for h in range(2):
                e, o = [lax.bitcast_convert_type(
                    xt[p * 4 + jj, h, c * 128:(c + 1) * 128, :].astype(BF16).astype(F32), U32) for p in range(2)]
                xio32[c, pl.ds(2 * jj + h, 128, stride=8), :] = ((e >> 16) | o).T

    def a_out(i):
        def finish(r, t):
            for h in range(2):
                xt[i, h, r * 128:(r + 1) * 128, :] += t[:, h * 128:(h + 1) * 128]
        return chunks(8, lambda r, k: woa[r, k], ot, i, finish)

    def out_proj(i, w_ref):
        o = rhs(ot, i)
        for r in range(8):
            t = _mm(_up(jnp.concatenate([w_ref[r, k] for k in range(8)], axis=1)), o)
            for h in range(2):
                xt[i, h, r * 128:(r + 1) * 128, :] += t[:, h * 128:(h + 1) * 128]
            yield

    def a_proj(g, p, jj):
        qr, kr, vr = qkv_buf[p]
        j = 2 * jj

        def finish(r, t):
            sl = slice((r % 2) * 128, (r % 2 + 1) * 128)
            for i in range(2):
                ti = t[:, i * 128:(i + 1) * 128]
                if r < 2:
                    qr[j + i, sl, :] = ti
                else:
                    dst = kr if r < 4 else vr
                    dst[8 + j + i, sl, :] = ti
                    dst[j + i, sl, :] = pltpu.roll(ti, 1, 1)
        return chunks(6, lambda r, k: wa[g, k, r * 64:(r + 1) * 64, :], xn, p * 4 + jj, finish)

    lane0 = lax.broadcasted_iota(jnp.int32, (8, 128), 1) == 0

    def a_attn(g, p, jj):
        qr, kr, vr = qkv_buf[p]
        j = 2 * jj
        lg = [[None] * W for _ in range(2)]
        for d in range(DH):
            sl = slice(d * 8, d * 8 + 8)
            kk = [kr[j + 1 + i, sl, :] for i in range(W + 1)]
            for i, q in enumerate(gate([qr[j + i, sl, :] for i in range(2)])):
                for w in range(W):
                    t = q * kk[7 + i - w]
                    lg[i][w] = t if d == 0 else lg[i][w] + t
            yield
        pr = []
        for i in range(2):
            l = [t * (DH ** -0.5) for t in lg[i]]
            l = [l[0]] + [jnp.where(lane0 & (j + i < w), -1e9, l[w]) for w in range(1, W)]
            m = _tree(jnp.maximum, l)
            e = [jnp.exp(t - m) for t in l]
            inv = 1.0 / _tree(jnp.add, e)
            pr.append([t * inv for t in e])
            yield
        for par in range(2):
            for d in range(0, DH // 2, 2):
                o = [[], []]
                for dd in (d, d + 1):
                    pp = gate(pr[0] + pr[1])
                    pr = [pp[:W], pp[W:]]
                    sl = slice((2 * dd + par) * 8, (2 * dd + par) * 8 + 8)
                    vv = [vr[j + 1 + i, sl, :] for i in range(W + 1)]
                    for i in range(2):
                        o[i].append(_tree(jnp.add, [pr[i][w] * vv[7 + i - w] for w in range(W)]))
                    if dd == d:
                        yield
                for i in range(2):
                    ot[p * 4 + jj, i, ds(g * 16 + par * 8 + d // 2, 8), :] = _pk(jnp.concatenate(o[i], axis=0))
                yield

    def loop(lo, hi, make, u=2):
        if (hi - lo) % u:
            u = hi - lo

        def body(k, _):
            parts = [make(lo + k * u + t) for t in range(u)]
            pace.clear()
            _weave(*[(chain(*[take(*pt[a]) for pt in parts]), u * parts[0][a][1])
                     for a in range(len(parts[0]))])
            pace.clear()
            return 0
        lax.fori_loop(0, (hi - lo) // u, body, 0)

    def take(gen, n):
        for _ in range(n):
            next(gen, None)
            yield
        for _ in gen:
            pass

    def layer_a(first):
        pace.clear()

        def part(g, p):
            def make(jj):
                gens = [(a_proj(g + p, 1 - p, jj), 24), (a_attn(g, p, jj), 66)]
                if first:
                    if p == 1:
                        gens += [(prep_b(g, jj, n), 4) for n in range(2)]
                    else:
                        gens.append((chain(*[prep_ao(g, 2 * jj + n, 3 + n) for n in range(2)]), 4))
                        if not (isinstance(g, int) and g == 3):
                            gens.append((chain(*[prep_a(g + 1, jj, t, t) for t in range(3)]), 12))
                return gens
            loop(0, 4, make)

        def grp(g, _):
            if first:
                @pl.when(g == 0)
                def _():
                    for cp in a_cp[1] + ao_cp:
                        cp.wait()
                    for cp in a_cp[2] + b_cp + a_cp[3]:
                        cp.start()
                for k in (2, 3):
                    @pl.when(g == k - 1)
                    def _():
                        for cp in a_cp[k]:
                            cp.wait()
            part(g, 0)
            if first:
                @pl.when(g == 0)
                def _():
                    for cp in b_cp:
                        cp.wait()
            if first:
                part(g, 1)
            else:
                pl.when(g < 3)(lambda: part(g, 1))
            return 0
        lax.fori_loop(0, 3 if first else 4, grp, 0)
        if first:
            part(3, 0)
        _weave((a_out(0), 32), (a_attn(3, 1, 0), 66))
        loop(1, 4, lambda i: [(a_out(i), 32), (a_attn(3, 1, i), 66), (norm(i - 1), NORM)])
        loop(4, 8, lambda i: [(a_out(i), 32), (norm(i - 1), NORM)] + (
            [(prep_b(3, i - 4, n), 4) for n in range(2)] if first else []))

    def allred(f, x):
        out = []
        for a in range(2):
            r = _tree(f, [x[a * 64 + i * 8:a * 64 + i * 8 + 8] for i in range(8)])
            r = f(r, pltpu.roll(r, 4, 0))
            out.append(f(r, pltpu.roll(r, 2, 0)))
        return out

    def bc(r):
        return jnp.concatenate([r[0]] * 8 + [r[1]] * 8, axis=0)

    def feat(p, g, is_q):
        ep = jnp.exp(p - bc(allred(jnp.maximum, p)))
        en = jnp.exp(bc(allred(jnp.minimum, p)) - p)
        ip = [1.0 / t for t in allred(jnp.add, ep)]
        im = [1.0 / t for t in allred(jnp.add, en)]
        if is_q:
            dp = allred(jnp.add, ep * jnp.tile(zacc[g, :128], (1, 2)))
            dn = allred(jnp.add, en * jnp.tile(zacc[g, 128:], (1, 2)))
            r = [1.0 / (dp[a] * ip[a] + dn[a] * im[a] + 1e-6) for a in range(2)]
            ip = [ip[a] * r[a] for a in range(2)]
            im = [im[a] * r[a] for a in range(2)]
        ep, en = ep * bc(ip), en * bc(im)
        if not is_q:
            zacc[g, :128] += ep[:, :128] + ep[:, 128:]
            zacc[g, 128:] += en[:, :128] + en[:, 128:]
        return [jnp.concatenate([ep[a * 64:(a + 1) * 64], en[a * 64:(a + 1) * 64]], axis=0).astype(BF16)
                for a in range(2)]

    def b_kv(i):
        xin = rhs(xn, i)
        phis = []
        for g in range(9):
            if g < 8:
                pk = _mm(wrows(wb, 1, g), xin) if g == 0 else nxt
                if g < 7:
                    nxt = _mm(wrows(wb, 1, g + 1), xin)
                v = _mm(wrows(wb, 2, g), xin).astype(BF16)
            if g > 0:
                v1, ph = phis[g - 1]
                kvacc[g - 1] += jnp.concatenate(
                    [lax.dot_general(v1[a * 64:(a + 1) * 64], ph[a], NT, preferred_element_type=F32)
                     for a in range(2)], axis=0)
            yield
            if g < 8:
                phis.append((v, feat(pk, g, False)))

    def b_fin(g):
        r_i = lax.broadcasted_iota(jnp.int32, (128, 128), 0)
        r_j = lax.broadcasted_iota(jnp.int32, (128, 128), 1)
        kv = jnp.concatenate([kvacc[g, pl.ds(a * 64 + p, DH, stride=2), :]
                              for a in range(2) for p in range(2)], axis=0)
        kvm[g] = _pk(jnp.where(r_i // 16 % 2 == r_j % 2, kv, 0.0))
        zacc[g] = jnp.broadcast_to(jnp.sum(zacc[g], axis=1, keepdims=True), (256, 128))

    def b_q(i, first=False):
        xin = rhs(xn, i)
        phis = []
        for g in range(9):
            if g < 8:
                pq = _mm(wrows(wb, 0, g), xin) if g == 0 else nxt
                if g < 7:
                    nxt = _mm(wrows(wb, 0, g + 1), xin)
            if g > 0:
                for a in range(2):
                    o = _pk(_mm(_up(kvm[g - 1, a * 32:(a + 1) * 32]), phis[g - 1][a]))
                    for p in range(2):
                        row = (g - 1) // 2 * 128 + p * 64 + ((g - 1) % 2 * 2 + a) * 16
                        for h in range(2):
                            ot[i, h, row:row + 16, :] = o[p * 16:(p + 1) * 16, h * 128:(h + 1) * 128]
            yield
            if g < 8:
                if first:
                    b_fin(g)
                phis.append(feat(pq, g, True))

    def layer_b():
        zacc[...] = jnp.zeros_like(zacc)
        kvacc[...] = jnp.zeros_like(kvacc)
        _weave((b_kv(0), 9), (norm(7), NORM * 2))
        loop(1, 8, lambda i: [(b_kv(i), 9)], 1)
        _weave((b_q(0, True), 9))
        _weave((out_proj(0, wob), 8), (b_q(1), 9))
        loop(2, 8, lambda i: [(norm(i - 2), NORM), (out_proj(i - 1, wob), 8), (b_q(i), 9)], 1)
        _weave((out_proj(7, wob), 8), (norm(6), NORM))

    for cp in a_cp[0]:
        cp.wait()
    _weave((chain(*[prep_a(0, c, t, t) for c in range(4) for t in range(3)]), 48))
    for cp in x_cp:
        cp.wait()
    for cp in a_cp[1] + ao_cp:
        cp.start()
    _weave((chain(load_x(0), norm(0)), 32))
    for jj in range(1, 4):
        _weave((a_proj(0, 0, jj - 1), 24), (chain(load_x(jj), norm(jj), norm(3 + jj)), 56))
    _weave((a_proj(0, 0, 3), 24), (norm(7), NORM))
    layer_a(True)
    layer_b()
    _weave((a_proj(0, 0, 0), 24), (norm(7), NORM))
    loop(1, 4, lambda jj: [(a_proj(0, 0, jj), 24)])
    layer_a(False)
    layer_b()
    o_cp = [pltpu.make_async_copy(xio.at[c], out_hbm.at[:, ds(c, 128)], osems.at[c]) for c in range(8)]
    for c, cp in enumerate(o_cp):
        store_x(c)
        cp.start()
    for cp in o_cp:
        cp.wait()


@jax.jit
def pallas_interleave_layers__sliding_local_dilated__linear_kernel_hedgehog__prompt_kernel(
        A_x, A_wqkv, A_wo, B_x, B_wqkv, B_w_phi, B_wo):
    del B_x
    vm = pl.BlockSpec(memory_space=pltpu.VMEM)
    hbm = pl.BlockSpec(memory_space=pl.ANY)
    V = pltpu.VMEM
    out = pl.pallas_call(
        _kernel,
        in_specs=[pl.BlockSpec(memory_space=pltpu.SMEM)] + [hbm] * 4 + [vm, hbm],
        out_specs=hbm,
        out_shape=jax.ShapeDtypeStruct((S, D), BF16),
        scratch_shapes=[
            V((8, S, 128), BF16), V((12, 2, D, 128), BF16), V((8, D, 128), BF16),
            V((24, D, 128), BF16), V((8, D, 128), BF16),
            pltpu.SemaphoreType.DMA((72,)), pltpu.SemaphoreType.DMA((8,)), V((8, 64, 128), U32),
            V((4, 8, 384, 128), U32), V((8, 8, 64, 128), U32),
            V((3, 8, D // 2, 128), U32), V((8, 8, 64, 128), U32),
            V((8, 2, D, 128), F32), V((8, 2, D // 2, 128), U32), V((8, 2, D // 2, 128), U32),
            V((8, 256, 128), F32), V((16, 256, 128), F32), V((16, 256, 128), F32),
            V((8, 256, 128), F32), V((16, 256, 128), F32), V((16, 256, 128), F32),
            V((5, 264, 128), U32), V((8, 128, 128), F32), V((8, 256, 128), F32), V((8, 64, 128), U32),
        ],
        compiler_params=pltpu.CompilerParams(vmem_limit_bytes=110 * 1024 * 1024),
    )(np.zeros((1,), np.int32), A_x.reshape(S, D), A_wqkv, A_wo, B_wqkv, B_w_phi.reshape(D, DH), B_wo)
    return out.reshape(1, S, D)
```

```python
import functools

import numpy as np
import jax
import jax.numpy as jnp
from jax import lax
import jax.experimental.pallas as pl
import jax.experimental.pallas.tpu as pltpu

S, D, H, DH = 2048, 1024, 32, 32
W = 8
NC = S // 128
F32, BF16, U32 = jnp.float32, jnp.bfloat16, jnp.uint32
NT = (((1,), (1,)), ((), ()))


def _mm(a, b):
    return jnp.dot(a, b, preferred_element_type=F32)


def _pk(x):
    return pltpu.bitcast(x.astype(BF16), U32)


def _up(x):
    return pltpu.bitcast(x, BF16)


def _half(w, p):
    return lax.bitcast_convert_type((w << 16) if p == 0 else (w & jnp.uint32(0xFFFF0000)), F32)


def _tree(f, xs):
    xs = list(xs)
    while len(xs) > 1:
        xs = [f(xs[i], xs[i + 1]) for i in range(0, len(xs), 2)]
    return xs[0]


def _weave(*gens):
    order = sorted(((k + (0.5 if gi else 0)) / n, gi) for gi, (_, n) in enumerate(gens) for k in range(n))
    for _, gi in order:
        next(gens[gi][0], None)
    for g, _ in gens:
        for _ in g:
            pass


NORM = 16


def _kernel(zero_ref, x_hbm, awqkv_hbm, awo_hbm, bwqkv_hbm, bphi, bwo_hbm, out_hbm,
            xio, awqkv, awo, bwqkv, bwo, sems, osems, bds,
            wa, woa, wb, wob, xt, xsum, xn, ot, q0, k0, v0, q1, k1, v1, tmp, kvacc, zacc, kvm):
    never = lax.broadcasted_iota(jnp.int32, (8, 128), 0) < zero_ref[0]
    pace = []

    def gate(xs, who):
        if not pace or who in pace[1]:
            return xs
        pace[1].append(who)
        return [jnp.where(never, lax.bitcast_convert_type(pace[0], x.dtype), x) for x in xs]

    def chunks(n, lhs, x_ref, i, finish):
        for r in range(n):
            for k in range(0, 8, 2):
                yield
                t = _mm(_up(jnp.concatenate([lhs(r, k), lhs(r, k + 1)], axis=1)),
                        _up(jnp.concatenate([x_ref[i, h, k * 64:(k + 2) * 64, :] for h in range(2)], axis=1)))
                acc = t if k == 0 else acc + t
                pace[:] = [t[:8, :128], []]
            finish(r, acc)

    qkv_buf = ((q0, k0, v0), (q1, k1, v1))

    def norm(i):
        ms = [jnp.broadcast_to(jnp.sum(xsum[i, h], axis=0, keepdims=True) * (1.0 / D), (8, 128))
              for h in range(2)]
        invs = []
        for h in range(2):
            acc = None
            for r in range(4):
                ms[h], = gate([ms[h]], 'norm')
                d = xt[i, h, r * 256:(r + 1) * 256, :] - jnp.tile(ms[h], (32, 1))
                d = d * d
                t = _tree(jnp.add, [d[k * 8:k * 8 + 8] for k in range(32)])
                acc = t if r == 0 else acc + t
                yield
            invs.append(lax.rsqrt(jnp.sum(acc, axis=0, keepdims=True) * (1.0 / D) + 1e-5))
        for h in range(2):
            for r in range(4):
                ms[h], = gate([ms[h]], 'norm')
                for p in range(2):
                    x = xt[i, h, pl.ds(r * 256 + p, 128, stride=2), :]
                    xn[i, h, r * 128 + p * 64:r * 128 + p * 64 + 64, :] = _pk((x - jnp.tile(ms[h], (16, 1))) * invs[h])
                yield

    def put_x(i, h, r, x, sums):
        xt[i, h, r * 128:(r + 1) * 128, :] = x
        t = _tree(jnp.add, [x[k * 8:k * 8 + 8] for k in range(16)])
        sums[h] = t if r == 0 else sums[h] + t
        if r == 7:
            xsum[i, h] = sums[h]

    def ds(i, n):
        return pl.ds(pl.multiple_of(i * n, n), n)

    def wrows(ref, g, r):
        return _up(jnp.concatenate([ref[g, k, r * 64:(r + 1) * 64, :] for k in range(8)], axis=1))

    def rhs(ref, i):
        return _up(jnp.concatenate([ref[i, 0], ref[i, 1]], axis=1))

    def lanes(src, dst, first, n, sem0):
        return [pltpu.make_async_copy(src.at[:, ds(first + c, 128)], dst.at[c], sems.at[sem0 + c])
                for c in range(n)]

    x_cp = lanes(x_hbm, xio, 0, 8, 0)
    a_cp = [[cp for t in range(3) for cp in lanes(awqkv_hbm, awqkv.at[g * 3 + t], t * 8 + g * 2, 2, 8 + g * 6 + t * 2)]
            for g in range(4)]
    ao_cp = lanes(awo_hbm, awo, 0, 8, 32)
    b_cp = lanes(bwqkv_hbm, bwqkv, 0, 24, 40) + lanes(bwo_hbm, bwo, 0, 8, 64)
    for cp in a_cp[0] + x_cp:
        cp.start()

    awqkv32, awo32, bwqkv32, bwo32 = [r.bitcast(U32) for r in (awqkv, awo, bwqkv, bwo)]

    def prep_a(g, c, t, u):
        for n in range(2):
            w = awqkv32[g * 3 + t, n, ds(c, 128), :].T
            for h in range(4):
                tmp[u, pl.ds((n * 4 + h) * (DH + 1), DH), :] = w[h * DH:(h + 1) * DH]
            yield
        for half in range(2):
            w = jnp.concatenate([tmp[u, pl.ds(half * 16 + d, 8, stride=DH + 1), :] for d in range(16)], axis=0)
            for p in range(2):
                wa[g, 2 * c + p, t * 128 + half * 64:t * 128 + half * 64 + 64, :] = _pk(_half(w, p))
            yield

    def prep_ao(g, c, u):
        w = awo32[c, ds(g, 128), :]
        for h in range(8):
            tmp[u, pl.ds(h * 17, 16), :] = w[h * 16:(h + 1) * 16]
        yield
        w = jnp.concatenate([tmp[u, pl.ds(d, 8, stride=17), :] for d in range(16)], axis=0).T
        for p in range(2):
            woa[c, 2 * g + p] = _pk(_half(w, p))
        yield

    def prep_b(g, c, n):
        w = bwo32[2 * c + n, ds(g, 128), :].T
        for p in range(2):
            wob[2 * c + n, 2 * g + p] = _pk(_half(w, p))
        yield
        w = bwqkv32[16 + 2 * g + n, ds(c, 128), :].T
        for p in range(2):
            wb[2, 2 * c + p, ds(2 * g + n, 64), :] = _pk(_half(w, p))
        yield
        for t in range(2):
            w = bwqkv32[t * 8 + 2 * g + n, ds(c, 128), :]
            for p in range(2):
                wb[t, 2 * c + p, ds(2 * g + n, 64), :] = _pk(lax.dot_general(
                    _up(bds[2 * g + n]), _half(w, p).astype(BF16), NT, preferred_element_type=F32))
            yield

    f_i = lax.broadcasted_iota(jnp.int32, (DH, 128), 0)
    f_j = lax.broadcasted_iota(jnp.int32, (DH, 128), 1)
    rep = _mm(bphi[...], jnp.where(f_i == f_j % 64 // 2, 1.0, 0.0).astype(BF16))
    e_i = lax.broadcasted_iota(jnp.int32, (128, 128), 0)
    e_j = lax.broadcasted_iota(jnp.int32, (128, 128), 1)
    for g in range(8):
        bds[g] = _pk(jnp.where(e_i // 64 * 2 + e_i % 2 == e_j // DH, rep[g * 128:(g + 1) * 128].T, 0.0))

    xio32 = xio.bitcast(U32)

    def load_x(jj):
        sums = [{}, {}]
        for c in range(8):
            for h in range(2):
                w = xio32[c, pl.ds(2 * jj + h, 128, stride=8), :].T
                for p in range(2):
                    put_x(p * 4 + jj, h, c, _half(w, p), sums[p])
            yield

    def chain(*gens):
        for g in gens:
            yield from g

    def store_x(c):
        for jj in range(4):
            for h in range(2):
                e, o = [lax.bitcast_convert_type(
                    xt[p * 4 + jj, h, c * 128:(c + 1) * 128, :].astype(BF16).astype(F32), U32) for p in range(2)]
                xio32[c, pl.ds(2 * jj + h, 128, stride=8), :] = ((e >> 16) | o).T

    def out_proj(i, w_ref):
        sums = {}

        def finish(r, t):
            for h in range(2):
                put_x(i, h, r, xt[i, h, r * 128:(r + 1) * 128, :] + t[:, h * 128:(h + 1) * 128], sums)
        return chunks(8, lambda r, k: w_ref[r, k], ot, i, finish)

    def a_proj(g, p, jj):
        qr, kr, vr = qkv_buf[p]
        j = 2 * jj

        def finish(r, t):
            sl = slice((r % 2) * 128, (r % 2 + 1) * 128)
            for i in range(2):
                ti = t[:, i * 128:(i + 1) * 128]
                if r < 2:
                    qr[j + i, sl, :] = ti
                else:
                    dst = kr if r < 4 else vr
                    dst[8 + j + i, sl, :] = ti
                    dst[j + i, sl, :] = pltpu.roll(ti, 1, 1)
        return chunks(6, lambda r, k: wa[g, k, r * 64:(r + 1) * 64, :], xn, p * 4 + jj, finish)

    lane0 = lax.broadcasted_iota(jnp.int32, (8, 128), 1) == 0

    def a_attn(g, p, jj):
        qr, kr, vr = qkv_buf[p]
        j = 2 * jj
        lg = [[None] * W for _ in range(2)]
        for d in range(DH):
            sl = slice(d * 8, d * 8 + 8)
            kk = [kr[j + 1 + i, sl, :] for i in range(W + 1)]
            for i, q in enumerate(gate([qr[j + i, sl, :] for i in range(2)], 'attn')):
                for w in range(W):
                    t = q * kk[7 + i - w]
                    lg[i][w] = t if d == 0 else lg[i][w] + t
            yield
        pr = []
        for i in range(2):
            l = [t * (DH ** -0.5) for t in lg[i]]
            l = [l[0]] + [jnp.where(lane0 & (j + i < w), -1e9, l[w]) for w in range(1, W)]
            m = _tree(jnp.maximum, l)
            e = [jnp.exp(t - m) for t in l]
            inv = 1.0 / _tree(jnp.add, e)
            pr.append([t * inv for t in e])
            yield
        for par in range(2):
            for d in range(0, DH // 2, 2):
                o = [[], []]
                for dd in (d, d + 1):
                    pp = gate(pr[0] + pr[1], 'attn')
                    pr = [pp[:W], pp[W:]]
                    sl = slice((2 * dd + par) * 8, (2 * dd + par) * 8 + 8)
                    vv = [vr[j + 1 + i, sl, :] for i in range(W + 1)]
                    for i in range(2):
                        o[i].append(_tree(jnp.add, [pr[i][w] * vv[7 + i - w] for w in range(W)]))
                    if dd == d:
                        yield
                for i in range(2):
                    ot[p * 4 + jj, i, ds(g * 16 + par * 8 + d // 2, 8), :] = _pk(jnp.concatenate(o[i], axis=0))
                yield

    def weave(*gens):
        pace.clear()
        _weave(*gens)
        pace.clear()

    def loop(lo, hi, make, u=2):
        if (hi - lo) % u:
            u = hi - lo

        def body(k, _):
            parts = [make(lo + k * u + t) for t in range(u)]
            weave(*[(chain(*[take(*pt[a]) for pt in parts]), u * parts[0][a][1])
                    for a in range(len(parts[0]))])
            return 0
        lax.fori_loop(0, (hi - lo) // u, body, 0)

    def take(gen, n):
        for _ in range(n):
            next(gen, None)
            yield
        for _ in gen:
            pass

    def layer_a(first):
        def part(g, p):
            def make(jj):
                gens = [(a_proj(g + p, 1 - p, jj), 24), (a_attn(g, p, jj), 66)]
                if first:
                    if p == 1:
                        gens += [(prep_b(g, jj, n), 4) for n in range(2)]
                    else:
                        gens.append((chain(*[prep_ao(g, 2 * jj + n, 3 + n) for n in range(2)]), 4))
                        if not (isinstance(g, int) and g == 3):
                            gens.append((chain(*[prep_a(g + 1, jj, t, t) for t in range(3)]), 12))
                return gens
            loop(0, 4, make)

        def grp(g, _):
            if first:
                @pl.when(g == 0)
                def _():
                    for cp in a_cp[1] + ao_cp:
                        cp.wait()
                    for cp in a_cp[2] + b_cp + a_cp[3]:
                        cp.start()
                for k in (2, 3):
                    @pl.when(g == k - 1)
                    def _():
                        for cp in a_cp[k]:
                            cp.wait()
            part(g, 0)
            if first:
                @pl.when(g == 0)
                def _():
                    for cp in b_cp:
                        cp.wait()
            if first:
                part(g, 1)
            else:
                pl.when(g < 3)(lambda: part(g, 1))
            return 0
        lax.fori_loop(0, 3 if first else 4, grp, 0)
        if first:
            part(3, 0)
        weave((out_proj(0, woa), 32), (a_attn(3, 1, 0), 66))
        loop(1, 4, lambda i: [(out_proj(i, woa), 32), (a_attn(3, 1, i), 66), (norm(i - 1), NORM)])
        loop(4, 8, lambda i: [(out_proj(i, woa), 32), (norm(i - 1), NORM)] + (
            [(prep_b(3, i - 4, n), 4) for n in range(2)] if first else []))

    def allred(f, x):
        out = []
        for a in range(2):
            r = _tree(f, [x[a * 64 + i * 8:a * 64 + i * 8 + 8] for i in range(8)])
            r = f(r, pltpu.roll(r, 4, 0))
            out.append(f(r, pltpu.roll(r, 2, 0)))
        return out

    def bc(r):
        return jnp.concatenate([r[0]] * 8 + [r[1]] * 8, axis=0)

    def feat(p, g, is_q):
        ep = jnp.exp(p - bc(allred(jnp.maximum, p)))
        en = jnp.exp(bc(allred(jnp.minimum, p)) - p)
        ip = [1.0 / t for t in allred(jnp.add, ep)]
        im = [1.0 / t for t in allred(jnp.add, en)]
        if is_q:
            dp = allred(jnp.add, ep * jnp.tile(zacc[g, :128], (1, 2)))
            dn = allred(jnp.add, en * jnp.tile(zacc[g, 128:], (1, 2)))
            r = [1.0 / (dp[a] * ip[a] + dn[a] * im[a] + 1e-6) for a in range(2)]
            ip = [ip[a] * r[a] for a in range(2)]
            im = [im[a] * r[a] for a in range(2)]
        ep, en = ep * bc(ip), en * bc(im)
        if not is_q:
            zacc[g, :128] += ep[:, :128] + ep[:, 128:]
            zacc[g, 128:] += en[:, :128] + en[:, 128:]
        return [jnp.concatenate([ep[a * 64:(a + 1) * 64], en[a * 64:(a + 1) * 64]], axis=0).astype(BF16)
                for a in range(2)]

    def b_kv(i):
        xin = rhs(xn, i)
        phis = []
        for g in range(9):
            if g < 8:
                pk = _mm(wrows(wb, 1, g), xin) if g == 0 else nxt
                if g < 7:
                    nxt = _mm(wrows(wb, 1, g + 1), xin)
                v = _mm(wrows(wb, 2, g), xin).astype(BF16)
            if g > 0:
                v1, ph = phis[g - 1]
                kvacc[g - 1] += jnp.concatenate(
                    [lax.dot_general(v1[a * 64:(a + 1) * 64], ph[a], NT, preferred_element_type=F32)
                     for a in range(2)], axis=0)
            yield
            if g < 8:
                phis.append((v, feat(pk, g, False)))

    def b_fin(g):
        r_i = lax.broadcasted_iota(jnp.int32, (128, 128), 0)
        r_j = lax.broadcasted_iota(jnp.int32, (128, 128), 1)
        kv = jnp.concatenate([kvacc[g, pl.ds(a * 64 + p, DH, stride=2), :]
                              for a in range(2) for p in range(2)], axis=0)
        kvm[g] = _pk(jnp.where(r_i // 16 % 2 == r_j % 2, kv, 0.0))
        zacc[g] = jnp.broadcast_to(jnp.sum(zacc[g], axis=1, keepdims=True), (256, 128))

    def b_q(i, first=False):
        xin = rhs(xn, i)
        phis = []
        for g in range(9):
            if g < 8:
                pq = _mm(wrows(wb, 0, g), xin) if g == 0 else nxt
                if g < 7:
                    nxt = _mm(wrows(wb, 0, g + 1), xin)
            if g > 0:
                for a in range(2):
                    o = _pk(_mm(_up(kvm[g - 1, a * 32:(a + 1) * 32]), phis[g - 1][a]))
                    for p in range(2):
                        row = (g - 1) // 2 * 128 + p * 64 + ((g - 1) % 2 * 2 + a) * 16
                        for h in range(2):
                            ot[i, h, row:row + 16, :] = o[p * 16:(p + 1) * 16, h * 128:(h + 1) * 128]
            yield
            if g < 8:
                if first:
                    b_fin(g)
                phis.append(feat(pq, g, True))

    def layer_b():
        zacc[...] = jnp.zeros_like(zacc)
        kvacc[...] = jnp.zeros_like(kvacc)
        weave((b_kv(0), 9), (norm(7), NORM * 2))
        loop(1, 8, lambda i: [(b_kv(i), 9)], 1)
        weave((b_q(0, True), 9))
        weave((out_proj(0, wob), 32), (b_q(1), 9))
        loop(2, 8, lambda i: [(norm(i - 2), NORM), (out_proj(i - 1, wob), 32), (b_q(i), 9)], 1)
        weave((out_proj(7, wob), 32), (norm(6), NORM))

    for cp in a_cp[0]:
        cp.wait()
    weave((chain(*[prep_a(0, c, t, t) for c in range(4) for t in range(3)]), 48))
    for cp in x_cp:
        cp.wait()
    for cp in a_cp[1] + ao_cp:
        cp.start()
    weave((chain(load_x(0), norm(0)), 24))
    for jj in range(1, 4):
        weave((a_proj(0, 0, jj - 1), 24), (chain(load_x(jj), norm(jj), norm(3 + jj)), 40))
    weave((a_proj(0, 0, 3), 24), (norm(7), NORM))
    layer_a(True)
    layer_b()
    weave((a_proj(0, 0, 0), 24), (norm(7), NORM))
    loop(1, 4, lambda jj: [(a_proj(0, 0, jj), 24)])
    layer_a(False)
    layer_b()
    o_cp = [pltpu.make_async_copy(xio.at[c], out_hbm.at[:, ds(c, 128)], osems.at[c]) for c in range(8)]
    for c, cp in enumerate(o_cp):
        store_x(c)
        cp.start()
    for cp in o_cp:
        cp.wait()


@jax.jit
def pallas_interleave_layers__sliding_local_dilated__linear_kernel_hedgehog__prompt_kernel(
        A_x, A_wqkv, A_wo, B_x, B_wqkv, B_w_phi, B_wo):
    del B_x
    vm = pl.BlockSpec(memory_space=pltpu.VMEM)
    hbm = pl.BlockSpec(memory_space=pl.ANY)
    V = pltpu.VMEM
    out = pl.pallas_call(
        _kernel,
        in_specs=[pl.BlockSpec(memory_space=pltpu.SMEM)] + [hbm] * 4 + [vm, hbm],
        out_specs=hbm,
        out_shape=jax.ShapeDtypeStruct((S, D), BF16),
        scratch_shapes=[
            V((8, S, 128), BF16), V((12, 2, D, 128), BF16), V((8, D, 128), BF16),
            V((24, D, 128), BF16), V((8, D, 128), BF16),
            pltpu.SemaphoreType.DMA((72,)), pltpu.SemaphoreType.DMA((8,)), V((8, 64, 128), U32),
            V((4, 8, 384, 128), U32), V((8, 8, 64, 128), U32),
            V((3, 8, D // 2, 128), U32), V((8, 8, 64, 128), U32),
            V((8, 2, D, 128), F32), V((8, 2, 8, 128), F32), V((8, 2, D // 2, 128), U32), V((8, 2, D // 2, 128), U32),
            V((8, 256, 128), F32), V((16, 256, 128), F32), V((16, 256, 128), F32),
            V((8, 256, 128), F32), V((16, 256, 128), F32), V((16, 256, 128), F32),
            V((5, 264, 128), U32), V((8, 128, 128), F32), V((8, 256, 128), F32), V((8, 64, 128), U32),
        ],
        compiler_params=pltpu.CompilerParams(vmem_limit_bytes=110 * 1024 * 1024),
    )(np.zeros((1,), np.int32), A_x.reshape(S, D), A_wqkv, A_wo, B_wqkv, B_w_phi.reshape(D, DH), B_wo)
    return out.reshape(1, S, D)
```

```python
import functools

import numpy as np
import jax
import jax.numpy as jnp
from jax import lax
import jax.experimental.pallas as pl
import jax.experimental.pallas.tpu as pltpu

S, D, H, DH = 2048, 1024, 32, 32
W = 8
NC = S // 128
F32, BF16, U32 = jnp.float32, jnp.bfloat16, jnp.uint32
NT = (((1,), (1,)), ((), ()))


def _mm(a, b):
    return jnp.dot(a, b, preferred_element_type=F32)


def _pk(x):
    return pltpu.bitcast(x.astype(BF16), U32)


def _up(x):
    return pltpu.bitcast(x, BF16)


def _half(w, p):
    return lax.bitcast_convert_type((w << 16) if p == 0 else (w & jnp.uint32(0xFFFF0000)), F32)


def _tree(f, xs):
    xs = list(xs)
    while len(xs) > 1:
        xs = [f(xs[i], xs[i + 1]) for i in range(0, len(xs), 2)]
    return xs[0]


def _weave(*gens):
    order = sorted(((k + (0.5 if gi else 0)) / n, gi) for gi, (_, n) in enumerate(gens) for k in range(n))
    for _, gi in order:
        next(gens[gi][0], None)
    for g, _ in gens:
        for _ in g:
            pass


NORM = 16


def _kernel(zero_ref, x_hbm, awqkv_hbm, awo_hbm, bwqkv_hbm, bphi, bwo_hbm, out_hbm,
            xio, awqkv, awo, bwqkv, bwo, sems, osems, bds,
            wa, woa, wb, wob, xt, xsum, xn, ot, q0, k0, v0, q1, k1, v1, tmp, kvacc, zacc, kvm):
    never = lax.broadcasted_iota(jnp.int32, (8, 128), 0) < zero_ref[0]
    pace = []

    def gate(xs, who):
        if not pace or who in pace[1]:
            return xs
        pace[1].append(who)
        return [jnp.where(never, lax.bitcast_convert_type(pace[0], x.dtype), x) for x in xs]

    def gate1(w):
        return jnp.concatenate(gate([w[:8]], 'prep') + [w[8:]], axis=0)

    def chunks(n, lhs, x_ref, i, finish):
        for r in range(n):
            for k in range(0, 8, 2):
                yield
                t = _mm(_up(jnp.concatenate([lhs(r, k), lhs(r, k + 1)], axis=1)),
                        _up(jnp.concatenate([x_ref[i, h, k * 64:(k + 2) * 64, :] for h in range(2)], axis=1)))
                acc = t if k == 0 else acc + t
                pace[:] = [t[:8, :128], []]
            finish(r, acc)

    qkv_buf = ((q0, k0, v0), (q1, k1, v1))

    def norm(i):
        ms = [jnp.broadcast_to(jnp.sum(xsum[i, h], axis=0, keepdims=True) * (1.0 / D), (8, 128))
              for h in range(2)]
        invs = []
        for h in range(2):
            acc = None
            for r in range(4):
                ms[h], = gate([ms[h]], 'norm')
                d = xt[i, h, r * 256:(r + 1) * 256, :] - jnp.tile(ms[h], (32, 1))
                d = d * d
                t = _tree(jnp.add, [d[k * 8:k * 8 + 8] for k in range(32)])
                acc = t if r == 0 else acc + t
                yield
            invs.append(lax.rsqrt(jnp.sum(acc, axis=0, keepdims=True) * (1.0 / D) + 1e-5))
        for h in range(2):
            for r in range(4):
                ms[h], = gate([ms[h]], 'norm')
                for p in range(2):
                    x = xt[i, h, pl.ds(r * 256 + p, 128, stride=2), :]
                    xn[i, h, r * 128 + p * 64:r * 128 + p * 64 + 64, :] = _pk((x - jnp.tile(ms[h], (16, 1))) * invs[h])
                yield

    def put_x(i, h, r, x):
        xt[i, h, r * 128:(r + 1) * 128, :] = x
        t = _tree(jnp.add, [x[k * 8:k * 8 + 8] for k in range(16)])
        xsum[i, h] = t if r == 0 else xsum[i, h] + t

    def ds(i, n):
        return pl.ds(pl.multiple_of(i * n, n), n)

    def wrows(ref, g, r):
        return _up(jnp.concatenate([ref[g, k, r * 64:(r + 1) * 64, :] for k in range(8)], axis=1))

    def rhs(ref, i):
        return _up(jnp.concatenate([ref[i, 0], ref[i, 1]], axis=1))

    def lanes(src, dst, first, n, sem0):
        return [pltpu.make_async_copy(src.at[:, ds(first + c, 128)], dst.at[c], sems.at[sem0 + c])
                for c in range(n)]

    x_cp = lanes(x_hbm, xio, 0, 8, 0)
    a_cp = [[cp for t in range(3) for cp in lanes(awqkv_hbm, awqkv.at[g * 3 + t], t * 8 + g * 2, 2, 8 + g * 6 + t * 2)]
            for g in range(4)]
    ao_cp = lanes(awo_hbm, awo, 0, 8, 32)
    b_cp = lanes(bwqkv_hbm, bwqkv, 0, 24, 40) + lanes(bwo_hbm, bwo, 0, 8, 64)
    for cp in a_cp[0] + x_cp[:3]:
        cp.start()

    awqkv32, awo32, bwqkv32, bwo32 = [r.bitcast(U32) for r in (awqkv, awo, bwqkv, bwo)]

    def prep_a(g, c, t, u):
        for n in range(2):
            w = gate1(awqkv32[g * 3 + t, n, ds(c, 128), :]).T
            for h in range(4):
                tmp[u, pl.ds((n * 4 + h) * (DH + 1), DH), :] = w[h * DH:(h + 1) * DH]
            yield
        for half in range(2):
            w = jnp.concatenate([tmp[u, pl.ds(half * 16 + d, 8, stride=DH + 1), :] for d in range(16)], axis=0)
            for p in range(2):
                wa[g, 2 * c + p, t * 128 + half * 64:t * 128 + half * 64 + 64, :] = _pk(_half(w, p))
            yield

    def prep_ao(g, c, u):
        w = awo32[c, ds(g, 128), :]
        for h in range(8):
            tmp[u, pl.ds(h * 17, 16), :] = w[h * 16:(h + 1) * 16]
        yield
        w = jnp.concatenate([tmp[u, pl.ds(d, 8, stride=17), :] for d in range(16)], axis=0)
        w = gate1(w).T
        for p in range(2):
            woa[c, 2 * g + p] = _pk(_half(w, p))
        yield

    def prep_b(g, c, n):
        w = gate1(bwo32[2 * c + n, ds(g, 128), :]).T
        for p in range(2):
            wob[2 * c + n, 2 * g + p] = _pk(_half(w, p))
        yield
        w = gate1(bwqkv32[16 + 2 * g + n, ds(c, 128), :]).T
        for p in range(2):
            wb[2, 2 * c + p, ds(2 * g + n, 64), :] = _pk(_half(w, p))
        yield
        for t in range(2):
            w = bwqkv32[t * 8 + 2 * g + n, ds(c, 128), :]
            for p in range(2):
                wb[t, 2 * c + p, ds(2 * g + n, 64), :] = _pk(lax.dot_general(
                    _up(bds[2 * g + n]), _half(w, p).astype(BF16), NT, preferred_element_type=F32))
            yield

    f_i = lax.broadcasted_iota(jnp.int32, (DH, 128), 0)
    f_j = lax.broadcasted_iota(jnp.int32, (DH, 128), 1)
    rep = _mm(bphi[...], jnp.where(f_i == f_j % 64 // 2, 1.0, 0.0).astype(BF16))
    e_i = lax.broadcasted_iota(jnp.int32, (128, 128), 0)
    e_j = lax.broadcasted_iota(jnp.int32, (128, 128), 1)
    for g in range(8):
        bds[g] = _pk(jnp.where(e_i // 64 * 2 + e_i % 2 == e_j // DH, rep[g * 128:(g + 1) * 128].T, 0.0))

    xio32 = xio.bitcast(U32)

    def load_x(c):
        for jj in range(4):
            for h in range(2):
                w = xio32[c, pl.ds(2 * jj + h, 128, stride=8), :].T
                for p in range(2):
                    put_x(p * 4 + jj, h, c, _half(w, p))

    def chain(*gens):
        for g in gens:
            yield from g

    def o_cp(c):
        return pltpu.make_async_copy(xio.at[c], out_hbm.at[:, ds(c, 128)], osems.at[c])

    def final(c, _):
        w = _up(jnp.concatenate([wob[c, k] for k in range(8)], axis=1))
        for jj in range(4):
            t = [_mm(w, rhs(ot, p * 4 + jj)) for p in range(2)]
            for h in range(2):
                e, o = [lax.bitcast_convert_type(
                    (xt[p * 4 + jj, h, ds(c, 128), :] + t[p][:, h * 128:(h + 1) * 128]).astype(BF16).astype(F32),
                    U32) for p in range(2)]
                xio32[c, pl.ds(2 * jj + h, 128, stride=8), :] = ((e >> 16) | o).T
        o_cp(c).start()
        return 0

    def out_proj(i, w_ref):
        def finish(r, t):
            for h in range(2):
                put_x(i, h, r, xt[i, h, r * 128:(r + 1) * 128, :] + t[:, h * 128:(h + 1) * 128])
        return chunks(8, lambda r, k: w_ref[r, k], ot, i, finish)

    def a_proj(g, p, jj):
        qr, kr, vr = qkv_buf[p]
        j = 2 * jj

        def finish(r, t):
            sl = slice((r % 2) * 128, (r % 2 + 1) * 128)
            for i in range(2):
                ti = t[:, i * 128:(i + 1) * 128]
                if r < 2:
                    qr[j + i, sl, :] = ti
                else:
                    dst = kr if r < 4 else vr
                    dst[8 + j + i, sl, :] = ti
                    dst[j + i, sl, :] = pltpu.roll(ti, 1, 1)
        return chunks(6, lambda r, k: wa[g, k, r * 64:(r + 1) * 64, :], xn, p * 4 + jj, finish)

    lane0 = lax.broadcasted_iota(jnp.int32, (8, 128), 1) == 0

    def a_attn(g, p, jj):
        qr, kr, vr = qkv_buf[p]
        j = 2 * jj
        lg = [[None] * W for _ in range(2)]
        for d in range(DH):
            sl = slice(d * 8, d * 8 + 8)
            kk = [kr[j + 1 + i, sl, :] for i in range(W + 1)]
            for i, q in enumerate(gate([qr[j + i, sl, :] for i in range(2)], 'attn')):
                for w in range(W):
                    t = q * kk[7 + i - w]
                    lg[i][w] = t if d == 0 else lg[i][w] + t
            yield
        pr = []
        for i in range(2):
            l = [t * (DH ** -0.5) for t in lg[i]]
            l = [l[0]] + [jnp.where(lane0 & (j + i < w), -1e9, l[w]) for w in range(1, W)]
            m = _tree(jnp.maximum, l)
            e = [jnp.exp(t - m) for t in l]
            inv = 1.0 / _tree(jnp.add, e)
            pr.append([t * inv for t in e])
            yield
        for par in range(2):
            for d in range(0, DH // 2, 2):
                o = [[], []]
                for dd in (d, d + 1):
                    pp = gate(pr[0] + pr[1], 'attn')
                    pr = [pp[:W], pp[W:]]
                    sl = slice((2 * dd + par) * 8, (2 * dd + par) * 8 + 8)
                    vv = [vr[j + 1 + i, sl, :] for i in range(W + 1)]
                    for i in range(2):
                        o[i].append(_tree(jnp.add, [pr[i][w] * vv[7 + i - w] for w in range(W)]))
                    if dd == d:
                        yield
                for i in range(2):
                    ot[p * 4 + jj, i, ds(g * 16 + par * 8 + d // 2, 8), :] = _pk(jnp.concatenate(o[i], axis=0))
                yield

    def weave(*gens):
        pace.clear()
        _weave(*gens)
        pace.clear()

    def loop(lo, hi, make, u=2):
        if (hi - lo) % u:
            u = hi - lo

        def body(k, _):
            parts = [make(lo + k * u + t) for t in range(u)]
            weave(*[(chain(*[take(*pt[a]) for pt in parts]), u * parts[0][a][1])
                    for a in range(len(parts[0]))])
            return 0
        lax.fori_loop(0, (hi - lo) // u, body, 0)

    def take(gen, n):
        for _ in range(n):
            next(gen, None)
            yield
        for _ in gen:
            pass

    def layer_a(first):
        def part(g, p):
            def make(jj):
                gens = [(a_proj(g + p, 1 - p, jj), 24), (a_attn(g, p, jj), 66)]
                if first:
                    if p == 1:
                        gens += [(prep_b(g, jj, n), 4) for n in range(2)]
                    else:
                        gens.append((chain(*[prep_ao(g, 2 * jj + n, 3 + n) for n in range(2)]), 4))
                        if not (isinstance(g, int) and g == 3):
                            gens.append((chain(*[prep_a(g + 1, jj, t, t) for t in range(3)]), 12))
                return gens
            loop(0, 4, make)

        def grp(g, _):
            if first:
                @pl.when(g == 0)
                def _():
                    for cp in a_cp[1] + ao_cp:
                        cp.wait()
                    for cp in a_cp[2] + b_cp + a_cp[3]:
                        cp.start()
                for k in (2, 3):
                    @pl.when(g == k - 1)
                    def _():
                        for cp in a_cp[k]:
                            cp.wait()
            part(g, 0)
            if first:
                @pl.when(g == 0)
                def _():
                    for cp in b_cp:
                        cp.wait()
            if first:
                part(g, 1)
            else:
                pl.when(g < 3)(lambda: part(g, 1))
            return 0
        lax.fori_loop(0, 3 if first else 4, grp, 0)
        if first:
            part(3, 0)
        weave((out_proj(0, woa), 32), (a_attn(3, 1, 0), 66))
        loop(1, 4, lambda i: [(out_proj(i, woa), 32), (a_attn(3, 1, i), 66), (norm(i - 1), NORM)])
        loop(4, 8, lambda i: [(out_proj(i, woa), 32), (norm(i - 1), NORM)] + (
            [(prep_b(3, i - 4, n), 4) for n in range(2)] if first else []))

    def allred(f, x):
        out = []
        for a in range(2):
            r = _tree(f, [x[a * 64 + i * 8:a * 64 + i * 8 + 8] for i in range(8)])
            r = f(r, pltpu.roll(r, 4, 0))
            out.append(f(r, pltpu.roll(r, 2, 0)))
        return out

    def bc(r):
        return jnp.concatenate([r[0]] * 8 + [r[1]] * 8, axis=0)

    def feat(p, g, is_q):
        ep = jnp.exp(p - bc(allred(jnp.maximum, p)))
        en = jnp.exp(bc(allred(jnp.minimum, p)) - p)
        ip = [1.0 / t for t in allred(jnp.add, ep)]
        im = [1.0 / t for t in allred(jnp.add, en)]
        if is_q:
            dp = allred(jnp.add, ep * jnp.tile(zacc[g, :128], (1, 2)))
            dn = allred(jnp.add, en * jnp.tile(zacc[g, 128:], (1, 2)))
            r = [1.0 / (dp[a] * ip[a] + dn[a] * im[a] + 1e-6) for a in range(2)]
            ip = [ip[a] * r[a] for a in range(2)]
            im = [im[a] * r[a] for a in range(2)]
        ep, en = ep * bc(ip), en * bc(im)
        if not is_q:
            zacc[g, :128] += ep[:, :128] + ep[:, 128:]
            zacc[g, 128:] += en[:, :128] + en[:, 128:]
        return [jnp.concatenate([ep[a * 64:(a + 1) * 64], en[a * 64:(a + 1) * 64]], axis=0).astype(BF16)
                for a in range(2)]

    def b_kv(i):
        xin = rhs(xn, i)
        phis = []
        for g in range(9):
            if g < 8:
                pk = _mm(wrows(wb, 1, g), xin) if g == 0 else nxt
                if g < 7:
                    nxt = _mm(wrows(wb, 1, g + 1), xin)
                v = _mm(wrows(wb, 2, g), xin).astype(BF16)
            if g > 0:
                v1, ph = phis[g - 1]
                kvacc[g - 1] += jnp.concatenate(
                    [lax.dot_general(v1[a * 64:(a + 1) * 64], ph[a], NT, preferred_element_type=F32)
                     for a in range(2)], axis=0)
            yield
            if g < 8:
                phis.append((v, feat(pk, g, False)))

    def b_fin(g):
        r_i = lax.broadcasted_iota(jnp.int32, (128, 128), 0)
        r_j = lax.broadcasted_iota(jnp.int32, (128, 128), 1)
        kv = jnp.concatenate([kvacc[g, pl.ds(a * 64 + p, DH, stride=2), :]
                              for a in range(2) for p in range(2)], axis=0)
        kvm[g] = _pk(jnp.where(r_i // 16 % 2 == r_j % 2, kv, 0.0))
        zacc[g] = jnp.broadcast_to(jnp.sum(zacc[g], axis=1, keepdims=True), (256, 128))

    def b_q(i, first=False):
        xin = rhs(xn, i)
        phis = []
        for g in range(9):
            if g < 8:
                pq = _mm(wrows(wb, 0, g), xin) if g == 0 else nxt
                if g < 7:
                    nxt = _mm(wrows(wb, 0, g + 1), xin)
            if g > 0:
                for a in range(2):
                    o = _pk(_mm(_up(kvm[g - 1, a * 32:(a + 1) * 32]), phis[g - 1][a]))
                    for p in range(2):
                        row = (g - 1) // 2 * 128 + p * 64 + ((g - 1) % 2 * 2 + a) * 16
                        for h in range(2):
                            ot[i, h, row:row + 16, :] = o[p * 16:(p + 1) * 16, h * 128:(h + 1) * 128]
            yield
            if g < 8:
                if first:
                    b_fin(g)
                phis.append(feat(pq, g, True))

    def layer_b(last):
        zacc[...] = jnp.zeros_like(zacc)
        kvacc[...] = jnp.zeros_like(kvacc)
        weave((b_kv(0), 9), (norm(7), NORM * 2))
        loop(1, 8, lambda i: [(b_kv(i), 9)], 1)
        weave((b_q(0, True), 9))
        if last:
            loop(1, 8, lambda i: [(b_q(i), 9)], 1)
            lax.fori_loop(0, 8, final, 0)
            return
        weave((out_proj(0, wob), 32), (b_q(1), 9))
        loop(2, 8, lambda i: [(norm(i - 2), NORM), (out_proj(i - 1, wob), 32), (b_q(i), 9)], 1)
        weave((out_proj(7, wob), 32), (norm(6), NORM))

    for cp in a_cp[0]:
        cp.wait()
    weave((chain(*[prep_a(0, c, t, t) for c in range(4) for t in range(3)]), 48))
    for c in range(8):
        x_cp[c].wait()
        if c + 3 < 8:
            x_cp[c + 3].start()
        if c == 5:
            for cp in a_cp[1] + ao_cp:
                cp.start()
        load_x(c)
    weave((norm(0), NORM))
    for jj in range(4):
        weave((a_proj(0, 0, jj), 24), (chain(*[norm(i) for i in ((1, 4), (2, 5), (3, 6), (7,))[jj]]), 2 * NORM))
    layer_a(True)
    layer_b(False)
    weave((a_proj(0, 0, 0), 24), (norm(7), NORM))
    loop(1, 4, lambda jj: [(a_proj(0, 0, jj), 24)])
    layer_a(False)
    layer_b(True)
    for c in range(8):
        o_cp(c).wait()


@jax.jit
def pallas_interleave_layers__sliding_local_dilated__linear_kernel_hedgehog__prompt_kernel(
        A_x, A_wqkv, A_wo, B_x, B_wqkv, B_w_phi, B_wo):
    del B_x
    vm = pl.BlockSpec(memory_space=pltpu.VMEM)
    hbm = pl.BlockSpec(memory_space=pl.ANY)
    V = pltpu.VMEM
    out = pl.pallas_call(
        _kernel,
        in_specs=[pl.BlockSpec(memory_space=pltpu.SMEM)] + [hbm] * 4 + [vm, hbm],
        out_specs=hbm,
        out_shape=jax.ShapeDtypeStruct((S, D), BF16),
        scratch_shapes=[
            V((8, S, 128), BF16), V((12, 2, D, 128), BF16), V((8, D, 128), BF16),
            V((24, D, 128), BF16), V((8, D, 128), BF16),
            pltpu.SemaphoreType.DMA((72,)), pltpu.SemaphoreType.DMA((8,)), V((8, 64, 128), U32),
            V((4, 8, 384, 128), U32), V((8, 8, 64, 128), U32),
            V((3, 8, D // 2, 128), U32), V((8, 8, 64, 128), U32),
            V((8, 2, D, 128), F32), V((8, 2, 8, 128), F32), V((8, 2, D // 2, 128), U32), V((8, 2, D // 2, 128), U32),
            V((8, 256, 128), F32), V((16, 256, 128), F32), V((16, 256, 128), F32),
            V((8, 256, 128), F32), V((16, 256, 128), F32), V((16, 256, 128), F32),
            V((5, 264, 128), U32), V((8, 128, 128), F32), V((8, 256, 128), F32), V((8, 64, 128), U32),
        ],
        compiler_params=pltpu.CompilerParams(vmem_limit_bytes=110 * 1024 * 1024),
    )(np.zeros((1,), np.int32), A_x.reshape(S, D), A_wqkv, A_wo, B_wqkv, B_w_phi.reshape(D, DH), B_wo)
    return out.reshape(1, S, D)
```

```python
import functools

import numpy as np
import jax
import jax.numpy as jnp
from jax import lax
import jax.experimental.pallas as pl
import jax.experimental.pallas.tpu as pltpu

S, D, H, DH = 2048, 1024, 32, 32
W = 8
NC = S // 128
F32, BF16, U32 = jnp.float32, jnp.bfloat16, jnp.uint32
NT = (((1,), (1,)), ((), ()))


def _mm(a, b):
    return jnp.dot(a, b, preferred_element_type=F32)


def _pk(x):
    return pltpu.bitcast(x.astype(BF16), U32)


def _up(x):
    return pltpu.bitcast(x, BF16)


def _half(w, p):
    return lax.bitcast_convert_type((w << 16) if p == 0 else (w & jnp.uint32(0xFFFF0000)), F32)


def _tree(f, xs):
    xs = list(xs)
    while len(xs) > 1:
        xs = [f(xs[i], xs[i + 1]) for i in range(0, len(xs), 2)]
    return xs[0]


def _weave(*gens):
    order = sorted(((k + (0.5 if gi else 0)) / n, gi) for gi, (_, n) in enumerate(gens) for k in range(n))
    for _, gi in order:
        next(gens[gi][0], None)
    for g, _ in gens:
        for _ in g:
            pass


NORM = 16


def _kernel(zero_ref, x_hbm, awqkv_hbm, awo_hbm, bwqkv_hbm, bphi, bwo_hbm, out_hbm,
            xio, awqkv, awo, bwqkv, bwo, sems, osems, bds,
            wa, woa, wb, wob, xt, xsum, xn, ot, q0, k0, v0, q1, k1, v1, tmp, kvacc, zacc, kvm):
    never = lax.broadcasted_iota(jnp.int32, (8, 128), 0) < zero_ref[0]
    pace = []

    def gate(xs, who):
        if not pace or who in pace[1]:
            return xs
        pace[1].append(who)
        return [jnp.where(never, lax.bitcast_convert_type(pace[0], x.dtype), x) for x in xs]

    def gate1(w):
        return jnp.concatenate(gate([w[:8]], 'prep') + [w[8:]], axis=0)

    def chunks(n, lhs, x_ref, i, finish):
        for r in range(n):
            for k in range(0, 8, 2):
                yield
                t = _mm(_up(jnp.concatenate([lhs(r, k), lhs(r, k + 1)], axis=1)),
                        _up(jnp.concatenate([x_ref[i, h, k * 64:(k + 2) * 64, :] for h in range(2)], axis=1)))
                acc = t if k == 0 else acc + t
                pace[:] = [t[:8, :128], []]
            finish(r, acc)

    qkv_buf = ((q0, k0, v0), (q1, k1, v1))

    def norm(i):
        ms = [jnp.broadcast_to(jnp.sum(xsum[i, h], axis=0, keepdims=True) * (1.0 / D), (8, 128))
              for h in range(2)]
        invs = []
        for h in range(2):
            acc = None
            for r in range(4):
                ms[h], = gate([ms[h]], 'norm')
                d = xt[i, h, r * 256:(r + 1) * 256, :] - jnp.tile(ms[h], (32, 1))
                d = d * d
                t = _tree(jnp.add, [d[k * 8:k * 8 + 8] for k in range(32)])
                acc = t if r == 0 else acc + t
                yield
            invs.append(lax.rsqrt(jnp.sum(acc, axis=0, keepdims=True) * (1.0 / D) + 1e-5))
        for h in range(2):
            for r in range(4):
                ms[h], = gate([ms[h]], 'norm')
                for p in range(2):
                    x = xt[i, h, pl.ds(r * 256 + p, 128, stride=2), :]
                    xn[i, h, r * 128 + p * 64:r * 128 + p * 64 + 64, :] = _pk((x - jnp.tile(ms[h], (16, 1))) * invs[h])
                yield

    def put_x(i, h, r, x):
        xt[i, h, r * 128:(r + 1) * 128, :] = x
        t = _tree(jnp.add, [x[k * 8:k * 8 + 8] for k in range(16)])
        xsum[i, h] = t if r == 0 else xsum[i, h] + t

    def ds(i, n):
        return pl.ds(pl.multiple_of(i * n, n), n)

    def wrows(ref, g, r):
        return _up(jnp.concatenate([ref[g, k, r * 64:(r + 1) * 64, :] for k in range(8)], axis=1))

    def rhs(ref, i):
        return _up(jnp.concatenate([ref[i, 0], ref[i, 1]], axis=1))

    def lanes(src, dst, first, n, sem0):
        return [pltpu.make_async_copy(src.at[:, ds(first + c, 128)], dst.at[c], sems.at[sem0 + c])
                for c in range(n)]

    x_cp = lanes(x_hbm, xio, 0, 8, 0)
    a_cp = [[cp for t in range(3) for cp in lanes(awqkv_hbm, awqkv.at[g * 3 + t], t * 8 + g * 2, 2, 8 + g * 6 + t * 2)]
            for g in range(4)]
    ao_cp = lanes(awo_hbm, awo, 0, 8, 32)
    bq_cp = lanes(bwqkv_hbm, bwqkv, 0, 24, 40)
    b_cp = [[bq_cp[t * 8 + 2 * g + n] for t in range(3) for n in range(2)] for g in range(4)]
    b_cp[0] += lanes(bwo_hbm, bwo, 0, 8, 64)
    for cp in a_cp[0] + x_cp[:3]:
        cp.start()

    awqkv32, awo32, bwqkv32, bwo32 = [r.bitcast(U32) for r in (awqkv, awo, bwqkv, bwo)]

    def prep_a(g, c, t, u):
        for n in range(2):
            w = gate1(awqkv32[g * 3 + t, n, ds(c, 128), :]).T
            for h in range(4):
                tmp[u, pl.ds((n * 4 + h) * (DH + 1), DH), :] = w[h * DH:(h + 1) * DH]
            yield
        for half in range(2):
            w = jnp.concatenate([tmp[u, pl.ds(half * 16 + d, 8, stride=DH + 1), :] for d in range(16)], axis=0)
            for p in range(2):
                wa[g, 2 * c + p, t * 128 + half * 64:t * 128 + half * 64 + 64, :] = _pk(_half(w, p))
            yield

    def prep_ao(g, c, u):
        w = awo32[c, ds(g, 128), :]
        for h in range(8):
            tmp[u, pl.ds(h * 17, 16), :] = w[h * 16:(h + 1) * 16]
        yield
        w = jnp.concatenate([tmp[u, pl.ds(d, 8, stride=17), :] for d in range(16)], axis=0)
        w = gate1(w).T
        for p in range(2):
            woa[c, 2 * g + p] = _pk(_half(w, p))
        yield

    def prep_b(g, c, n):
        w = gate1(bwo32[2 * c + n, ds(g, 128), :]).T
        for p in range(2):
            wob[2 * c + n, 2 * g + p] = _pk(_half(w, p))
        yield
        w = gate1(bwqkv32[16 + 2 * g + n, ds(c, 128), :]).T
        for p in range(2):
            wb[2, 2 * c + p, ds(2 * g + n, 64), :] = _pk(_half(w, p))
        yield
        for t in range(2):
            w = bwqkv32[t * 8 + 2 * g + n, ds(c, 128), :]
            for p in range(2):
                wb[t, 2 * c + p, ds(2 * g + n, 64), :] = _pk(lax.dot_general(
                    _up(bds[2 * g + n]), _half(w, p).astype(BF16), NT, preferred_element_type=F32))
            yield

    f_i = lax.broadcasted_iota(jnp.int32, (DH, 128), 0)
    f_j = lax.broadcasted_iota(jnp.int32, (DH, 128), 1)
    rep = _mm(bphi[...], jnp.where(f_i == f_j % 64 // 2, 1.0, 0.0).astype(BF16))
    e_i = lax.broadcasted_iota(jnp.int32, (128, 128), 0)
    e_j = lax.broadcasted_iota(jnp.int32, (128, 128), 1)
    for g in range(8):
        bds[g] = _pk(jnp.where(e_i // 64 * 2 + e_i % 2 == e_j // DH, rep[g * 128:(g + 1) * 128].T, 0.0))

    xio32 = xio.bitcast(U32)

    def load_x(c):
        for jj in range(4):
            for h in range(2):
                w = xio32[c, pl.ds(2 * jj + h, 128, stride=8), :].T
                for p in range(2):
                    put_x(p * 4 + jj, h, c, _half(w, p))

    def chain(*gens):
        for g in gens:
            yield from g

    def o_cp(c):
        return pltpu.make_async_copy(xio.at[c], out_hbm.at[:, ds(c, 128)], osems.at[c])

    def final(c, _):
        w = _up(jnp.concatenate([wob[c, k] for k in range(8)], axis=1))
        for jj in range(4):
            t = [_mm(w, rhs(ot, p * 4 + jj)) for p in range(2)]
            for h in range(2):
                e, o = [lax.bitcast_convert_type(
                    (xt[p * 4 + jj, h, ds(c, 128), :] + t[p][:, h * 128:(h + 1) * 128]).astype(BF16).astype(F32),
                    U32) for p in range(2)]
                xio32[c, pl.ds(2 * jj + h, 128, stride=8), :] = ((e >> 16) | o).T
        o_cp(c).start()
        return 0

    def out_proj(i, w_ref):
        def finish(r, t):
            for h in range(2):
                put_x(i, h, r, xt[i, h, r * 128:(r + 1) * 128, :] + t[:, h * 128:(h + 1) * 128])
        return chunks(8, lambda r, k: w_ref[r, k], ot, i, finish)

    def a_proj(g, p, jj):
        qr, kr, vr = qkv_buf[p]
        j = 2 * jj

        def finish(r, t):
            sl = slice((r % 2) * 128, (r % 2 + 1) * 128)
            for i in range(2):
                ti = t[:, i * 128:(i + 1) * 128]
                if r < 2:
                    qr[j + i, sl, :] = ti
                else:
                    dst = kr if r < 4 else vr
                    dst[8 + j + i, sl, :] = ti
                    dst[j + i, sl, :] = pltpu.roll(ti, 1, 1)
        return chunks(6, lambda r, k: wa[g, k, r * 64:(r + 1) * 64, :], xn, p * 4 + jj, finish)

    lane0 = lax.broadcasted_iota(jnp.int32, (8, 128), 1) == 0

    def a_attn(g, p, jj):
        qr, kr, vr = qkv_buf[p]
        j = 2 * jj
        lg = [[None] * W for _ in range(2)]
        for d in range(DH):
            sl = slice(d * 8, d * 8 + 8)
            kk = [kr[j + 1 + i, sl, :] for i in range(W + 1)]
            for i, q in enumerate(gate([qr[j + i, sl, :] for i in range(2)], 'attn')):
                for w in range(W):
                    t = q * kk[7 + i - w]
                    lg[i][w] = t if d == 0 else lg[i][w] + t
            yield
        pr = []
        for i in range(2):
            l = [t * (DH ** -0.5) for t in lg[i]]
            l = [l[0]] + [jnp.where(lane0 & (j + i < w), -1e9, l[w]) for w in range(1, W)]
            m = _tree(jnp.maximum, l)
            e = [jnp.exp(t - m) for t in l]
            inv = 1.0 / _tree(jnp.add, e)
            pr.append([t * inv for t in e])
            yield
        for par in range(2):
            for d in range(0, DH // 2, 2):
                o = [[], []]
                for dd in (d, d + 1):
                    pp = gate(pr[0] + pr[1], 'attn')
                    pr = [pp[:W], pp[W:]]
                    sl = slice((2 * dd + par) * 8, (2 * dd + par) * 8 + 8)
                    vv = [vr[j + 1 + i, sl, :] for i in range(W + 1)]
                    for i in range(2):
                        o[i].append(_tree(jnp.add, [pr[i][w] * vv[7 + i - w] for w in range(W)]))
                    if dd == d:
                        yield
                for i in range(2):
                    ot[p * 4 + jj, i, ds(g * 16 + par * 8 + d // 2, 8), :] = _pk(jnp.concatenate(o[i], axis=0))
                yield

    def weave(*gens):
        pace.clear()
        _weave(*gens)
        pace.clear()

    def loop(lo, hi, make, u=2):
        if (hi - lo) % u:
            u = hi - lo

        def body(k, _):
            parts = [make(lo + k * u + t) for t in range(u)]
            weave(*[(chain(*[take(*pt[a]) for pt in parts]), u * parts[0][a][1])
                    for a in range(len(parts[0]))])
            return 0
        lax.fori_loop(0, (hi - lo) // u, body, 0)

    def take(gen, n):
        for _ in range(n):
            next(gen, None)
            yield
        for _ in gen:
            pass

    def layer_a(first):
        def part(g, p):
            def make(jj):
                gens = [(a_proj(g + p, 1 - p, jj), 24), (a_attn(g, p, jj), 66)]
                if first:
                    if p == 1:
                        gens += [(prep_b(g, jj, n), 4) for n in range(2)]
                    else:
                        gens.append((chain(*[prep_ao(g, 2 * jj + n, 3 + n) for n in range(2)]), 4))
                        if not (isinstance(g, int) and g == 3):
                            gens.append((chain(*[prep_a(g + 1, jj, t, t) for t in range(3)]), 12))
                return gens
            loop(0, 4, make)

        def grp(g, _):
            def at(g0, wait, start):
                @pl.when(g == g0)
                def _():
                    for cp in wait:
                        cp.wait()
                    for cp in start:
                        cp.start()
            if first:
                at(0, a_cp[1] + ao_cp, a_cp[2] + b_cp[0])
                at(1, a_cp[2], b_cp[2])
                at(2, a_cp[3], [])
            part(g, 0)
            if first:
                at(0, b_cp[0], a_cp[3] + b_cp[1])
                at(1, b_cp[1], b_cp[3])
                at(2, b_cp[2] + b_cp[3], [])
            if first:
                part(g, 1)
            else:
                pl.when(g < 3)(lambda: part(g, 1))
            return 0
        lax.fori_loop(0, 3 if first else 4, grp, 0)
        if first:
            part(3, 0)
        weave((out_proj(0, woa), 32), (a_attn(3, 1, 0), 66))
        loop(1, 4, lambda i: [(out_proj(i, woa), 32), (a_attn(3, 1, i), 66), (norm(i - 1), NORM)])
        loop(4, 8, lambda i: [(out_proj(i, woa), 32), (norm(i - 1), NORM)] + (
            [(prep_b(3, i - 4, n), 4) for n in range(2)] if first else []))

    def allred(f, x):
        out = []
        for a in range(2):
            r = _tree(f, [x[a * 64 + i * 8:a * 64 + i * 8 + 8] for i in range(8)])
            r = f(r, pltpu.roll(r, 4, 0))
            out.append(f(r, pltpu.roll(r, 2, 0)))
        return out

    def bc(r):
        return jnp.concatenate([r[0]] * 8 + [r[1]] * 8, axis=0)

    def feat(p, g, is_q):
        ep = jnp.exp(p - bc(allred(jnp.maximum, p)))
        en = jnp.exp(bc(allred(jnp.minimum, p)) - p)
        ip = [1.0 / t for t in allred(jnp.add, ep)]
        im = [1.0 / t for t in allred(jnp.add, en)]
        if is_q:
            dp = allred(jnp.add, ep * jnp.tile(zacc[g, :128], (1, 2)))
            dn = allred(jnp.add, en * jnp.tile(zacc[g, 128:], (1, 2)))
            r = [1.0 / (dp[a] * ip[a] + dn[a] * im[a] + 1e-6) for a in range(2)]
            ip = [ip[a] * r[a] for a in range(2)]
            im = [im[a] * r[a] for a in range(2)]
        ep, en = ep * bc(ip), en * bc(im)
        if not is_q:
            zacc[g, :128] += ep[:, :128] + ep[:, 128:]
            zacc[g, 128:] += en[:, :128] + en[:, 128:]
        return [jnp.concatenate([ep[a * 64:(a + 1) * 64], en[a * 64:(a + 1) * 64]], axis=0).astype(BF16)
                for a in range(2)]

    def b_kv(i):
        xin = rhs(xn, i)
        phis = []
        for g in range(9):
            if g < 8:
                pk = _mm(wrows(wb, 1, g), xin) if g == 0 else nxt
                if g < 7:
                    nxt = _mm(wrows(wb, 1, g + 1), xin)
                v = _mm(wrows(wb, 2, g), xin).astype(BF16)
            if g > 0:
                v1, ph = phis[g - 1]
                kvacc[g - 1] += jnp.concatenate(
                    [lax.dot_general(v1[a * 64:(a + 1) * 64], ph[a], NT, preferred_element_type=F32)
                     for a in range(2)], axis=0)
            yield
            if g < 8:
                phis.append((v, feat(pk, g, False)))

    def b_fin(g):
        r_i = lax.broadcasted_iota(jnp.int32, (128, 128), 0)
        r_j = lax.broadcasted_iota(jnp.int32, (128, 128), 1)
        kv = jnp.concatenate([kvacc[g, pl.ds(a * 64 + p, DH, stride=2), :]
                              for a in range(2) for p in range(2)], axis=0)
        kvm[g] = _pk(jnp.where(r_i // 16 % 2 == r_j % 2, kv, 0.0))
        zacc[g] = jnp.broadcast_to(jnp.sum(zacc[g], axis=1, keepdims=True), (256, 128))

    def b_q(i, first=False):
        xin = rhs(xn, i)
        phis = []
        for g in range(9):
            if g < 8:
                pq = _mm(wrows(wb, 0, g), xin) if g == 0 else nxt
                if g < 7:
                    nxt = _mm(wrows(wb, 0, g + 1), xin)
            if g > 0:
                for a in range(2):
                    o = _pk(_mm(_up(kvm[g - 1, a * 32:(a + 1) * 32]), phis[g - 1][a]))
                    for p in range(2):
                        row = (g - 1) // 2 * 128 + p * 64 + ((g - 1) % 2 * 2 + a) * 16
                        for h in range(2):
                            ot[i, h, row:row + 16, :] = o[p * 16:(p + 1) * 16, h * 128:(h + 1) * 128]
            yield
            if g < 8:
                if first:
                    b_fin(g)
                phis.append(feat(pq, g, True))

    def layer_b(last):
        zacc[...] = jnp.zeros_like(zacc)
        kvacc[...] = jnp.zeros_like(kvacc)
        weave((b_kv(0), 9), (norm(7), NORM * 2))
        loop(1, 8, lambda i: [(b_kv(i), 9)], 1)
        weave((b_q(0, True), 9))
        if last:
            loop(1, 8, lambda i: [(b_q(i), 9)], 1)
            lax.fori_loop(0, 8, final, 0)
            return
        weave((out_proj(0, wob), 32), (b_q(1), 9))
        loop(2, 8, lambda i: [(norm(i - 2), NORM), (out_proj(i - 1, wob), 32), (b_q(i), 9)], 1)
        weave((out_proj(7, wob), 32), (norm(6), NORM))

    for cp in a_cp[0]:
        cp.wait()
    weave((chain(*[prep_a(0, c, t, t) for c in range(4) for t in range(3)]), 48))
    for c in range(8):
        x_cp[c].wait()
        if c + 3 < 8:
            x_cp[c + 3].start()
        if c == 5:
            for cp in a_cp[1] + ao_cp:
                cp.start()
        load_x(c)
    weave((norm(0), NORM))
    for jj in range(4):
        weave((a_proj(0, 0, jj), 24), (chain(*[norm(i) for i in ((1, 4), (2, 5), (3, 6), (7,))[jj]]), 2 * NORM))
    layer_a(True)
    layer_b(False)
    weave((a_proj(0, 0, 0), 24), (norm(7), NORM))
    loop(1, 4, lambda jj: [(a_proj(0, 0, jj), 24)])
    layer_a(False)
    layer_b(True)
    for c in range(8):
        o_cp(c).wait()


@jax.jit
def pallas_interleave_layers__sliding_local_dilated__linear_kernel_hedgehog__prompt_kernel(
        A_x, A_wqkv, A_wo, B_x, B_wqkv, B_w_phi, B_wo):
    del B_x
    vm = pl.BlockSpec(memory_space=pltpu.VMEM)
    hbm = pl.BlockSpec(memory_space=pl.ANY)
    V = pltpu.VMEM
    out = pl.pallas_call(
        _kernel,
        in_specs=[pl.BlockSpec(memory_space=pltpu.SMEM)] + [hbm] * 4 + [vm, hbm],
        out_specs=hbm,
        out_shape=jax.ShapeDtypeStruct((S, D), BF16),
        scratch_shapes=[
            V((8, S, 128), BF16), V((12, 2, D, 128), BF16), V((8, D, 128), BF16),
            V((24, D, 128), BF16), V((8, D, 128), BF16),
            pltpu.SemaphoreType.DMA((72,)), pltpu.SemaphoreType.DMA((8,)), V((8, 64, 128), U32),
            V((4, 8, 384, 128), U32), V((8, 8, 64, 128), U32),
            V((3, 8, D // 2, 128), U32), V((8, 8, 64, 128), U32),
            V((8, 2, D, 128), F32), V((8, 2, 8, 128), F32), V((8, 2, D // 2, 128), U32), V((8, 2, D // 2, 128), U32),
            V((8, 256, 128), F32), V((16, 256, 128), F32), V((16, 256, 128), F32),
            V((8, 256, 128), F32), V((16, 256, 128), F32), V((16, 256, 128), F32),
            V((5, 264, 128), U32), V((8, 128, 128), F32), V((8, 256, 128), F32), V((8, 64, 128), U32),
        ],
        compiler_params=pltpu.CompilerParams(vmem_limit_bytes=110 * 1024 * 1024),
    )(np.zeros((1,), np.int32), A_x.reshape(S, D), A_wqkv, A_wo, B_wqkv, B_w_phi.reshape(D, DH), B_wo)
    return out.reshape(1, S, D)
```

```python
import functools

import numpy as np
import jax
import jax.numpy as jnp
from jax import lax
import jax.experimental.pallas as pl
import jax.experimental.pallas.tpu as pltpu

S, D, H, DH = 2048, 1024, 32, 32
W = 8
NC = S // 128
F32, BF16, U32 = jnp.float32, jnp.bfloat16, jnp.uint32
NT = (((1,), (1,)), ((), ()))


def _mm(a, b):
    return jnp.dot(a, b, preferred_element_type=F32)


def _pk(x):
    return pltpu.bitcast(x.astype(BF16), U32)


def _up(x):
    return pltpu.bitcast(x, BF16)


def _half(w, p):
    return lax.bitcast_convert_type((w << 16) if p == 0 else (w & jnp.uint32(0xFFFF0000)), F32)


def _tree(f, xs):
    xs = list(xs)
    while len(xs) > 1:
        xs = [f(xs[i], xs[i + 1]) for i in range(0, len(xs), 2)]
    return xs[0]


def _weave(*gens):
    order = sorted(((k + (0.5 if gi else 0)) / n, gi) for gi, (_, n) in enumerate(gens) for k in range(n))
    for _, gi in order:
        next(gens[gi][0], None)
    for g, _ in gens:
        for _ in g:
            pass


NORM = 16


def _kernel(zero_ref, x_hbm, awqkv_hbm, awo_hbm, bwqkv_hbm, bphi, bwo_hbm, out_hbm,
            xio, awqkv, awo, bwqkv, bwo, sems, osems, bds,
            wa, woa, wb, wob, xt, xsum, xn, ot, q0, k0, v0, q1, k1, v1, tmp, kvacc, zacc, kvm):
    never = lax.broadcasted_iota(jnp.int32, (8, 128), 0) < zero_ref[0]
    pace = []

    def gate(xs, who):
        if not pace or who in pace[1]:
            return xs
        pace[1].append(who)
        return [jnp.where(never, lax.bitcast_convert_type(pace[0], x.dtype), x) for x in xs]

    def gate1(w):
        return jnp.concatenate(gate([w[:8]], 'prep') + [w[8:]], axis=0)

    def chunks(n, lhs, x_ref, i, finish):
        for r in range(n):
            for k in range(0, 8, 2):
                yield
                t = _mm(_up(jnp.concatenate([lhs(r, k), lhs(r, k + 1)], axis=1)),
                        _up(jnp.concatenate([x_ref[i, h, k * 64:(k + 2) * 64, :] for h in range(2)], axis=1)))
                acc = t if k == 0 else acc + t
                pace[:] = [t[:8, :128], []]
            finish(r, acc)

    qkv_buf = ((q0, k0, v0), (q1, k1, v1))

    def norm(i):
        ms = [jnp.broadcast_to(jnp.sum(xsum[i, h], axis=0, keepdims=True) * (1.0 / D), (8, 128))
              for h in range(2)]
        invs = []
        for h in range(2):
            acc = None
            for r in range(4):
                ms[h], = gate([ms[h]], 'norm')
                d = xt[i, h, r * 256:(r + 1) * 256, :] - jnp.tile(ms[h], (32, 1))
                d = d * d
                t = _tree(jnp.add, [d[k * 8:k * 8 + 8] for k in range(32)])
                acc = t if r == 0 else acc + t
                yield
            invs.append(lax.rsqrt(jnp.sum(acc, axis=0, keepdims=True) * (1.0 / D) + 1e-5))
        for h in range(2):
            for r in range(4):
                ms[h], = gate([ms[h]], 'norm')
                for p in range(2):
                    x = xt[i, h, pl.ds(r * 256 + p, 128, stride=2), :]
                    xn[i, h, r * 128 + p * 64:r * 128 + p * 64 + 64, :] = _pk((x - jnp.tile(ms[h], (16, 1))) * invs[h])
                yield

    def put_x(i, h, r, x):
        xt[i, h, r * 128:(r + 1) * 128, :] = x
        t = _tree(jnp.add, [x[k * 8:k * 8 + 8] for k in range(16)])
        xsum[i, h] = t if r == 0 else xsum[i, h] + t

    def ds(i, n):
        return pl.ds(pl.multiple_of(i * n, n), n)

    def wrows(ref, g, r):
        return _up(jnp.concatenate([ref[g, k, r * 64:(r + 1) * 64, :] for k in range(8)], axis=1))

    def rhs(ref, i):
        return _up(jnp.concatenate([ref[i, 0], ref[i, 1]], axis=1))

    def lanes(src, dst, first, n, sem0):
        return [pltpu.make_async_copy(src.at[:, ds(first + c, 128)], dst.at[c], sems.at[sem0 + c])
                for c in range(n)]

    x_cp = lanes(x_hbm, xio, 0, 8, 0)
    a_cp = [[cp for t in range(3) for cp in lanes(awqkv_hbm, awqkv.at[g * 3 + t], t * 8 + g * 2, 2, 8 + g * 6 + t * 2)]
            for g in range(4)]
    ao_cp = lanes(awo_hbm, awo, 0, 8, 32)
    bq_cp = lanes(bwqkv_hbm, bwqkv, 0, 24, 40)
    b_cp = [[bq_cp[t * 8 + 2 * g + n] for t in range(3) for n in range(2)] for g in range(4)]
    b_cp[0] += lanes(bwo_hbm, bwo, 0, 8, 64)
    for cp in a_cp[0] + x_cp[:3]:
        cp.start()

    awqkv32, awo32, bwqkv32, bwo32 = [r.bitcast(U32) for r in (awqkv, awo, bwqkv, bwo)]

    def prep_a(g, c, t, u):
        for n in range(2):
            w = gate1(awqkv32[g * 3 + t, n, ds(c, 128), :]).T
            for h in range(4):
                tmp[u, pl.ds((n * 4 + h) * (DH + 1), DH), :] = w[h * DH:(h + 1) * DH]
            yield
        for half in range(2):
            w = jnp.concatenate([tmp[u, pl.ds(half * 16 + d, 8, stride=DH + 1), :] for d in range(16)], axis=0)
            for p in range(2):
                wa[g, 2 * c + p, t * 128 + half * 64:t * 128 + half * 64 + 64, :] = _pk(_half(w, p))
            yield

    def prep_ao(g, c, u):
        w = awo32[c, ds(g, 128), :]
        for h in range(8):
            tmp[u, pl.ds(h * 17, 16), :] = w[h * 16:(h + 1) * 16]
        yield
        w = jnp.concatenate([tmp[u, pl.ds(d, 8, stride=17), :] for d in range(16)], axis=0)
        w = gate1(w).T
        for p in range(2):
            woa[c, 2 * g + p] = _pk(_half(w, p))
        yield

    def prep_b(g, c, n):
        w = gate1(bwo32[2 * c + n, ds(g, 128), :]).T
        for p in range(2):
            wob[2 * c + n, 2 * g + p] = _pk(_half(w, p))
        yield
        w = gate1(bwqkv32[16 + 2 * g + n, ds(c, 128), :]).T
        for p in range(2):
            wb[2, 2 * c + p, ds(2 * g + n, 64), :] = _pk(_half(w, p))
        yield
        for t in range(2):
            w = bwqkv32[t * 8 + 2 * g + n, ds(c, 128), :]
            for p in range(2):
                wb[t, 2 * c + p, ds(2 * g + n, 64), :] = _pk(lax.dot_general(
                    _up(bds[2 * g + n]), _half(w, p).astype(BF16), NT, preferred_element_type=F32))
            yield

    f_i = lax.broadcasted_iota(jnp.int32, (DH, 128), 0)
    f_j = lax.broadcasted_iota(jnp.int32, (DH, 128), 1)
    rep = _mm(bphi[...], jnp.where(f_i == f_j % 64 // 2, 1.0, 0.0).astype(BF16))
    e_i = lax.broadcasted_iota(jnp.int32, (128, 128), 0)
    e_j = lax.broadcasted_iota(jnp.int32, (128, 128), 1)
    for g in range(8):
        bds[g] = _pk(jnp.where(e_i // 64 * 2 + e_i % 2 == e_j // DH, rep[g * 128:(g + 1) * 128].T, 0.0))

    xio32 = xio.bitcast(U32)

    def load_x(c):
        for jj in range(4):
            for h in range(2):
                w = xio32[c, pl.ds(2 * jj + h, 128, stride=8), :].T
                for p in range(2):
                    put_x(p * 4 + jj, h, c, _half(w, p))

    def chain(*gens):
        for g in gens:
            yield from g

    def o_cp(c):
        return pltpu.make_async_copy(xio.at[c], out_hbm.at[:, ds(c, 128)], osems.at[c])

    def final(c, _):
        w = _up(jnp.concatenate([wob[c, k] for k in range(8)], axis=1))
        for jj in range(4):
            t = [_mm(w, rhs(ot, p * 4 + jj)) for p in range(2)]
            for h in range(2):
                e, o = [lax.bitcast_convert_type(
                    (xt[p * 4 + jj, h, ds(c, 128), :] + t[p][:, h * 128:(h + 1) * 128]).astype(BF16).astype(F32),
                    U32) for p in range(2)]
                xio32[c, pl.ds(2 * jj + h, 128, stride=8), :] = ((e >> 16) | o).T
        o_cp(c).start()
        return 0

    def out_proj(i, w_ref):
        def finish(r, t):
            for h in range(2):
                put_x(i, h, r, xt[i, h, r * 128:(r + 1) * 128, :] + t[:, h * 128:(h + 1) * 128])
        return chunks(8, lambda r, k: w_ref[r, k], ot, i, finish)

    def a_proj(g, p, jj):
        qr, kr, vr = qkv_buf[p]
        j = 2 * jj

        def finish(r, t):
            sl = slice((r % 2) * 128, (r % 2 + 1) * 128)
            for i in range(2):
                ti = t[:, i * 128:(i + 1) * 128]
                if r < 2:
                    qr[j + i, sl, :] = ti
                else:
                    dst = kr if r < 4 else vr
                    dst[8 + j + i, sl, :] = ti
                    dst[j + i, sl, :] = pltpu.roll(ti, 1, 1)
        return chunks(6, lambda r, k: wa[g, k, r * 64:(r + 1) * 64, :], xn, p * 4 + jj, finish)

    lane0 = lax.broadcasted_iota(jnp.int32, (8, 128), 1) == 0

    def a_attn(g, p, jj):
        qr, kr, vr = qkv_buf[p]
        for i in range(2):
            j = 2 * jj + i
            lg = [None] * W
            for d in range(DH):
                sl = slice(d * 8, d * 8 + 8)
                q, = gate([qr[j, sl, :]], 'attn')
                for w in range(W):
                    t = q * kr[8 + j - w, sl, :]
                    lg[w] = t if d == 0 else lg[w] + t
                yield
            l = [t * (DH ** -0.5) for t in lg]
            l = [l[0]] + [jnp.where(lane0 & (j < w), -1e9, l[w]) for w in range(1, W)]
            m = _tree(jnp.maximum, l)
            e = [jnp.exp(t - m) for t in l]
            inv = 1.0 / _tree(jnp.add, e)
            pr = [t * inv for t in e]
            yield
            for par in range(2):
                o = []
                for dd in range(DH // 2):
                    pr = gate(pr, 'attn')
                    sl = slice((2 * dd + par) * 8, (2 * dd + par) * 8 + 8)
                    o.append(_tree(jnp.add, [pr[w] * vr[8 + j - w, sl, :] for w in range(W)]))
                    if dd % 2:
                        ot[p * 4 + jj, i, ds(g * 16 + par * 8 + dd // 2, 8), :] = _pk(
                            jnp.concatenate(o[-2:], axis=0))
                    yield

    def weave(*gens):
        pace.clear()
        _weave(*gens)
        pace.clear()

    def loop(lo, hi, make, u=2):
        if (hi - lo) % u:
            u = hi - lo

        def body(k, _):
            parts = [make(lo + k * u + t) for t in range(u)]
            weave(*[(chain(*[take(*pt[a]) for pt in parts]), u * parts[0][a][1])
                    for a in range(len(parts[0]))])
            return 0
        lax.fori_loop(0, (hi - lo) // u, body, 0)

    def take(gen, n):
        for _ in range(n):
            next(gen, None)
            yield
        for _ in gen:
            pass

    def layer_a(first):
        def part(g, p):
            def make(jj):
                gens = [(a_proj(g + p, 1 - p, jj), 24), (a_attn(g, p, jj), 130)]
                if first:
                    if p == 1:
                        gens += [(prep_b(g, jj, n), 4) for n in range(2)]
                    else:
                        gens.append((chain(*[prep_ao(g, 2 * jj + n, 3 + n) for n in range(2)]), 4))
                        if not (isinstance(g, int) and g == 3):
                            gens.append((chain(*[prep_a(g + 1, jj, t, t) for t in range(3)]), 12))
                return gens
            loop(0, 4, make, 4)

        def grp(g, _):
            def at(g0, wait, start):
                @pl.when(g == g0)
                def _():
                    for cp in wait:
                        cp.wait()
                    for cp in start:
                        cp.start()
            if first:
                at(0, a_cp[1] + ao_cp, a_cp[2] + b_cp[0])
                at(1, a_cp[2], b_cp[2])
                at(2, a_cp[3], [])
            part(g, 0)
            if first:
                at(0, b_cp[0], a_cp[3] + b_cp[1])
                at(1, b_cp[1], b_cp[3])
                at(2, b_cp[2] + b_cp[3], [])
            if first:
                part(g, 1)
            else:
                pl.when(g < 3)(lambda: part(g, 1))
            return 0
        lax.fori_loop(0, 3 if first else 4, grp, 0)
        if first:
            part(3, 0)
        weave((out_proj(0, woa), 32), (a_attn(3, 1, 0), 130))
        loop(1, 4, lambda i: [(out_proj(i, woa), 32), (a_attn(3, 1, i), 130), (norm(i - 1), NORM)])
        loop(4, 8, lambda i: [(out_proj(i, woa), 32), (norm(i - 1), NORM)] + (
            [(prep_b(3, i - 4, n), 4) for n in range(2)] if first else []))

    def allred(f, x):
        out = []
        for a in range(2):
            r = _tree(f, [x[a * 64 + i * 8:a * 64 + i * 8 + 8] for i in range(8)])
            r = f(r, pltpu.roll(r, 4, 0))
            out.append(f(r, pltpu.roll(r, 2, 0)))
        return out

    def bc(r):
        return jnp.concatenate([r[0]] * 8 + [r[1]] * 8, axis=0)

    def feat(p, g, is_q):
        ep = jnp.exp(p - bc(allred(jnp.maximum, p)))
        en = jnp.exp(bc(allred(jnp.minimum, p)) - p)
        ip = [1.0 / t for t in allred(jnp.add, ep)]
        im = [1.0 / t for t in allred(jnp.add, en)]
        if is_q:
            dp = allred(jnp.add, ep * jnp.tile(zacc[g, :128], (1, 2)))
            dn = allred(jnp.add, en * jnp.tile(zacc[g, 128:], (1, 2)))
            r = [1.0 / (dp[a] * ip[a] + dn[a] * im[a] + 1e-6) for a in range(2)]
            ip = [ip[a] * r[a] for a in range(2)]
            im = [im[a] * r[a] for a in range(2)]
        ep, en = ep * bc(ip), en * bc(im)
        if not is_q:
            zacc[g, :128] += ep[:, :128] + ep[:, 128:]
            zacc[g, 128:] += en[:, :128] + en[:, 128:]
        return [jnp.concatenate([ep[a * 64:(a + 1) * 64], en[a * 64:(a + 1) * 64]], axis=0).astype(BF16)
                for a in range(2)]

    def b_kv(i):
        xin = rhs(xn, i)
        phis = []
        for g in range(9):
            if g < 8:
                pk = _mm(wrows(wb, 1, g), xin) if g == 0 else nxt
                if g < 7:
                    nxt = _mm(wrows(wb, 1, g + 1), xin)
                v = _mm(wrows(wb, 2, g), xin).astype(BF16)
            if g > 0:
                v1, ph = phis[g - 1]
                kvacc[g - 1] += jnp.concatenate(
                    [lax.dot_general(v1[a * 64:(a + 1) * 64], ph[a], NT, preferred_element_type=F32)
                     for a in range(2)], axis=0)
            yield
            if g < 8:
                phis.append((v, feat(pk, g, False)))

    def b_fin(g):
        r_i = lax.broadcasted_iota(jnp.int32, (128, 128), 0)
        r_j = lax.broadcasted_iota(jnp.int32, (128, 128), 1)
        kv = jnp.concatenate([kvacc[g, pl.ds(a * 64 + p, DH, stride=2), :]
                              for a in range(2) for p in range(2)], axis=0)
        kvm[g] = _pk(jnp.where(r_i // 16 % 2 == r_j % 2, kv, 0.0))
        zacc[g] = jnp.broadcast_to(jnp.sum(zacc[g], axis=1, keepdims=True), (256, 128))

    def b_q(i, first=False):
        xin = rhs(xn, i)
        phis = []
        for g in range(9):
            if g < 8:
                pq = _mm(wrows(wb, 0, g), xin) if g == 0 else nxt
                if g < 7:
                    nxt = _mm(wrows(wb, 0, g + 1), xin)
            if g > 0:
                for a in range(2):
                    o = _pk(_mm(_up(kvm[g - 1, a * 32:(a + 1) * 32]), phis[g - 1][a]))
                    for p in range(2):
                        row = (g - 1) // 2 * 128 + p * 64 + ((g - 1) % 2 * 2 + a) * 16
                        for h in range(2):
                            ot[i, h, row:row + 16, :] = o[p * 16:(p + 1) * 16, h * 128:(h + 1) * 128]
            yield
            if g < 8:
                if first:
                    b_fin(g)
                phis.append(feat(pq, g, True))

    def layer_b(last):
        zacc[...] = jnp.zeros_like(zacc)
        kvacc[...] = jnp.zeros_like(kvacc)
        weave((b_kv(0), 9), (norm(7), NORM * 2))
        loop(1, 8, lambda i: [(b_kv(i), 9)], 1)
        weave((b_q(0, True), 9))
        if last:
            loop(1, 8, lambda i: [(b_q(i), 9)], 1)
            lax.fori_loop(0, 8, final, 0)
            return
        weave((out_proj(0, wob), 32), (b_q(1), 9))
        loop(2, 8, lambda i: [(norm(i - 2), NORM), (out_proj(i - 1, wob), 32), (b_q(i), 9)], 1)
        weave((out_proj(7, wob), 32), (norm(6), NORM))

    for cp in a_cp[0]:
        cp.wait()
    weave((chain(*[prep_a(0, c, t, t) for c in range(4) for t in range(3)]), 48))
    for c in range(8):
        x_cp[c].wait()
        if c + 3 < 8:
            x_cp[c + 3].start()
        if c == 5:
            for cp in a_cp[1] + ao_cp:
                cp.start()
        load_x(c)
    weave((norm(0), NORM))
    for jj in range(4):
        weave((a_proj(0, 0, jj), 24), (chain(*[norm(i) for i in ((1, 4), (2, 5), (3, 6), (7,))[jj]]), 2 * NORM))
    layer_a(True)
    layer_b(False)
    weave((a_proj(0, 0, 0), 24), (norm(7), NORM))
    loop(1, 4, lambda jj: [(a_proj(0, 0, jj), 24)])
    layer_a(False)
    layer_b(True)
    for c in range(8):
        o_cp(c).wait()


@jax.jit
def pallas_interleave_layers__sliding_local_dilated__linear_kernel_hedgehog__prompt_kernel(
        A_x, A_wqkv, A_wo, B_x, B_wqkv, B_w_phi, B_wo):
    del B_x
    vm = pl.BlockSpec(memory_space=pltpu.VMEM)
    hbm = pl.BlockSpec(memory_space=pl.ANY)
    V = pltpu.VMEM
    out = pl.pallas_call(
        _kernel,
        in_specs=[pl.BlockSpec(memory_space=pltpu.SMEM)] + [hbm] * 4 + [vm, hbm],
        out_specs=hbm,
        out_shape=jax.ShapeDtypeStruct((S, D), BF16),
        scratch_shapes=[
            V((8, S, 128), BF16), V((12, 2, D, 128), BF16), V((8, D, 128), BF16),
            V((24, D, 128), BF16), V((8, D, 128), BF16),
            pltpu.SemaphoreType.DMA((72,)), pltpu.SemaphoreType.DMA((8,)), V((8, 64, 128), U32),
            V((4, 8, 384, 128), U32), V((8, 8, 64, 128), U32),
            V((3, 8, D // 2, 128), U32), V((8, 8, 64, 128), U32),
            V((8, 2, D, 128), F32), V((8, 2, 8, 128), F32), V((8, 2, D // 2, 128), U32), V((8, 2, D // 2, 128), U32),
            V((8, 256, 128), F32), V((16, 256, 128), F32), V((16, 256, 128), F32),
            V((8, 256, 128), F32), V((16, 256, 128), F32), V((16, 256, 128), F32),
            V((5, 264, 128), U32), V((8, 128, 128), F32), V((8, 256, 128), F32), V((8, 64, 128), U32),
        ],
        compiler_params=pltpu.CompilerParams(vmem_limit_bytes=110 * 1024 * 1024),
    )(np.zeros((1,), np.int32), A_x.reshape(S, D), A_wqkv, A_wo, B_wqkv, B_w_phi.reshape(D, DH), B_wo)
    return out.reshape(1, S, D)
```

```python
import functools

import numpy as np
import jax
import jax.numpy as jnp
from jax import lax
import jax.experimental.pallas as pl
import jax.experimental.pallas.tpu as pltpu

S, D, H, DH = 2048, 1024, 32, 32
W = 8
NC = S // 128
F32, BF16, U32 = jnp.float32, jnp.bfloat16, jnp.uint32
NT = (((1,), (1,)), ((), ()))


def _mm(a, b):
    return jnp.dot(a, b, preferred_element_type=F32)


def _pk(x):
    return pltpu.bitcast(x.astype(BF16), U32)


def _up(x):
    return pltpu.bitcast(x, BF16)


def _half(w, p):
    return lax.bitcast_convert_type((w << 16) if p == 0 else (w & jnp.uint32(0xFFFF0000)), F32)


def _tree(f, xs):
    xs = list(xs)
    while len(xs) > 1:
        xs = [f(xs[i], xs[i + 1]) for i in range(0, len(xs), 2)]
    return xs[0]


def _weave(*gens):
    order = sorted(((k + (0.5 if gi else 0)) / n, gi) for gi, (_, n) in enumerate(gens) for k in range(n))
    for _, gi in order:
        next(gens[gi][0], None)
    for g, _ in gens:
        for _ in g:
            pass


NORM = 16
XW = 4


def _kernel(zero_ref, x_hbm, awqkv_hbm, awo_hbm, bwqkv_hbm, bphi, bwo_hbm, out_hbm,
            xio, awqkv, awo, bwqkv, bwo, sems, osems, bds,
            wa, woa, wb, wob, xt, xsum, xn, ot, q0, k0, v0, q1, k1, v1, tmp, kvacc, zacc, kvm):
    never = lax.broadcasted_iota(jnp.int32, (8, 128), 0) < zero_ref[0]
    pace = []

    def gate(xs, who):
        if not pace or who in pace[1]:
            return xs
        pace[1].append(who)
        return [jnp.where(never, lax.bitcast_convert_type(pace[0], x.dtype), x) for x in xs]

    def gate1(w):
        return jnp.concatenate(gate([w[:8]], 'prep') + [w[8:]], axis=0)

    def chunks(n, lhs, x_ref, i, finish):
        for r in range(n):
            for k in range(0, 8, 2):
                yield
                t = _mm(_up(jnp.concatenate([lhs(r, k), lhs(r, k + 1)], axis=1)),
                        _up(jnp.concatenate([x_ref[i, h, k * 64:(k + 2) * 64, :] for h in range(2)], axis=1)))
                acc = t if k == 0 else acc + t
                pace[:] = [t[:8, :128], []]
            for h in range(2):
                finish(r, h, acc[:, h * 128:(h + 1) * 128])

    qkv_buf = ((q0, k0, v0), (q1, k1, v1))

    def norm(i):
        ms = [jnp.broadcast_to(jnp.sum(xsum[i, h], axis=0, keepdims=True) * (1.0 / D), (8, 128))
              for h in range(2)]
        invs = []
        for h in range(2):
            acc = None
            for r in range(4):
                ms[h], = gate([ms[h]], 'norm')
                d = xt[i, h, r * 256:(r + 1) * 256, :] - jnp.tile(ms[h], (32, 1))
                d = d * d
                t = _tree(jnp.add, [d[k * 8:k * 8 + 8] for k in range(32)])
                acc = t if r == 0 else acc + t
                yield
            invs.append(lax.rsqrt(jnp.sum(acc, axis=0, keepdims=True) * (1.0 / D) + 1e-5))
        for h in range(2):
            for r in range(4):
                ms[h], = gate([ms[h]], 'norm')
                for p in range(2):
                    x = xt[i, h, pl.ds(r * 256 + p, 128, stride=2), :]
                    xn[i, h, r * 128 + p * 64:r * 128 + p * 64 + 64, :] = _pk((x - jnp.tile(ms[h], (16, 1))) * invs[h])
                yield

    def put_x(i, h, r, x):
        xt[i, h, r * 128:(r + 1) * 128, :] = x
        t = _tree(jnp.add, [x[k * 8:k * 8 + 8] for k in range(16)])
        xsum[i, h] = t if r == 0 else xsum[i, h] + t

    def ds(i, n):
        return pl.ds(pl.multiple_of(i * n, n), n)

    def wrows(ref, g, r):
        return _up(jnp.concatenate([ref[g, k, r * 64:(r + 1) * 64, :] for k in range(8)], axis=1))

    def rhs(ref, i):
        return _up(jnp.concatenate([ref[i, 0], ref[i, 1]], axis=1))

    def lanes(src, dst, first, n, sem0):
        return [pltpu.make_async_copy(src.at[:, ds(first + c, 128)], dst.at[c], sems.at[sem0 + c])
                for c in range(n)]

    x_cp = lanes(x_hbm, xio, 0, 8, 0)
    a_cp = [[cp for t in range(3) for cp in lanes(awqkv_hbm, awqkv.at[g * 3 + t], t * 8 + g * 2, 2, 8 + g * 6 + t * 2)]
            for g in range(4)]
    ao_cp = lanes(awo_hbm, awo, 0, 8, 32)
    bq_cp = lanes(bwqkv_hbm, bwqkv, 0, 24, 40)
    b_cp = [[bq_cp[t * 8 + 2 * g + n] for t in range(3) for n in range(2)] for g in range(4)]
    b_cp[0] += lanes(bwo_hbm, bwo, 0, 8, 64)
    for cp in a_cp[0][:2] + x_cp[:XW]:
        cp.start()

    awqkv32, awo32, bwqkv32, bwo32 = [r.bitcast(U32) for r in (awqkv, awo, bwqkv, bwo)]

    def prep_a(g, c, t, u):
        for n in range(2):
            w = gate1(awqkv32[g * 3 + t, n, ds(c, 128), :]).T
            for h in range(4):
                tmp[u, pl.ds((n * 4 + h) * (DH + 1), DH), :] = w[h * DH:(h + 1) * DH]
            yield
        for half in range(2):
            w = jnp.concatenate([tmp[u, pl.ds(half * 16 + d, 8, stride=DH + 1), :] for d in range(16)], axis=0)
            for p in range(2):
                wa[g, 2 * c + p, t * 128 + half * 64:t * 128 + half * 64 + 64, :] = _pk(_half(w, p))
            yield

    def prep_ao(g, c, u):
        w = awo32[c, ds(g, 128), :]
        for h in range(8):
            tmp[u, pl.ds(h * 17, 16), :] = w[h * 16:(h + 1) * 16]
        yield
        w = jnp.concatenate([tmp[u, pl.ds(d, 8, stride=17), :] for d in range(16)], axis=0)
        w = gate1(w).T
        for p in range(2):
            woa[c, 2 * g + p] = _pk(_half(w, p))
        yield

    def prep_b(g, c, n):
        w = gate1(bwo32[2 * c + n, ds(g, 128), :]).T
        for p in range(2):
            wob[2 * c + n, 2 * g + p] = _pk(_half(w, p))
        yield
        w = gate1(bwqkv32[16 + 2 * g + n, ds(c, 128), :]).T
        for p in range(2):
            wb[2, 2 * c + p, ds(2 * g + n, 64), :] = _pk(_half(w, p))
        yield
        for t in range(2):
            w = bwqkv32[t * 8 + 2 * g + n, ds(c, 128), :]
            for p in range(2):
                wb[t, 2 * c + p, ds(2 * g + n, 64), :] = _pk(lax.dot_general(
                    _up(bds[2 * g + n]), _half(w, p).astype(BF16), NT, preferred_element_type=F32))
            yield

    f_i = lax.broadcasted_iota(jnp.int32, (DH, 128), 0)
    f_j = lax.broadcasted_iota(jnp.int32, (DH, 128), 1)
    rep = _mm(bphi[...], jnp.where(f_i == f_j % 64 // 2, 1.0, 0.0).astype(BF16))
    e_i = lax.broadcasted_iota(jnp.int32, (128, 128), 0)
    e_j = lax.broadcasted_iota(jnp.int32, (128, 128), 1)
    for g in range(8):
        bds[g] = _pk(jnp.where(e_i // 64 * 2 + e_i % 2 == e_j // DH, rep[g * 128:(g + 1) * 128].T, 0.0))

    xio32 = xio.bitcast(U32)

    def load_x(c):
        for jj in range(4):
            for h in range(2):
                w = xio32[c, pl.ds(2 * jj + h, 128, stride=8), :].T
                for p in range(2):
                    put_x(p * 4 + jj, h, c, _half(w, p))

    def chain(*gens):
        for g in gens:
            yield from g

    def o_cp(c):
        return pltpu.make_async_copy(xio.at[c], out_hbm.at[:, ds(c, 128)], osems.at[c])

    def final(c, _):
        w = _up(jnp.concatenate([wob[c, k] for k in range(8)], axis=1))
        for jj in range(4):
            t = [_mm(w, rhs(ot, p * 4 + jj)) for p in range(2)]
            for h in range(2):
                e, o = [lax.bitcast_convert_type(
                    (xt[p * 4 + jj, h, ds(c, 128), :] + t[p][:, h * 128:(h + 1) * 128]).astype(BF16).astype(F32),
                    U32) for p in range(2)]
                xio32[c, pl.ds(2 * jj + h, 128, stride=8), :] = ((e >> 16) | o).T
        o_cp(c).start()
        return 0

    def out_proj(i, w_ref):
        def finish(r, h, t):
            put_x(i, h, r, xt[i, h, r * 128:(r + 1) * 128, :] + t)
        return chunks(8, lambda r, k: w_ref[r, k], ot, i, finish)

    def a_proj(g, p, jj, rot=2):
        qr, kr, vr = qkv_buf[p]
        j = 2 * jj

        def finish(r, i, ti):
            r = (r + rot) % 6
            sl = slice((r % 2) * 128, (r % 2 + 1) * 128)
            if r < 2:
                qr[j + i, sl, :] = ti
            else:
                dst = kr if r < 4 else vr
                dst[8 + j + i, sl, :] = ti
                dst[j + i, sl, :] = pltpu.roll(ti, 1, 1)

        def lhs(r, k):
            r = (r + rot) % 6
            return wa[g, k, r * 64:(r + 1) * 64, :]
        return chunks(6, lhs, xn, p * 4 + jj, finish)

    lane0 = lax.broadcasted_iota(jnp.int32, (8, 128), 1) == 0

    def a_attn(g, p, jj):
        qr, kr, vr = qkv_buf[p]
        for i in range(2):
            j = 2 * jj + i
            lg = [None] * W
            for d in range(DH):
                sl = slice(d * 8, d * 8 + 8)
                q, = gate([qr[j, sl, :]], 'attn')
                for w in range(W):
                    t = q * kr[8 + j - w, sl, :]
                    lg[w] = t if d == 0 else lg[w] + t
                yield
            l = [t * (DH ** -0.5) for t in lg]
            l = [l[0]] + [jnp.where(lane0 & (j < w), -1e9, l[w]) for w in range(1, W)]
            m = _tree(jnp.maximum, l)
            e = [jnp.exp(t - m) for t in l]
            inv = 1.0 / _tree(jnp.add, e)
            pr = [t * inv for t in e]
            yield
            for par in range(2):
                o = []
                for dd in range(DH // 2):
                    pr = gate(pr, 'attn')
                    sl = slice((2 * dd + par) * 8, (2 * dd + par) * 8 + 8)
                    o.append(_tree(jnp.add, [pr[w] * vr[8 + j - w, sl, :] for w in range(W)]))
                    if dd % 2:
                        ot[p * 4 + jj, i, ds(g * 16 + par * 8 + dd // 2, 8), :] = _pk(
                            jnp.concatenate(o[-2:], axis=0))
                    yield

    def weave(*gens):
        pace.clear()
        _weave(*gens)
        pace.clear()

    def loop(lo, hi, make, u=2):
        if (hi - lo) % u:
            u = hi - lo

        def body(k, _):
            parts = [make(lo + k * u + t) for t in range(u)]
            weave(*[(chain(*[take(*pt[a]) for pt in parts]), u * parts[0][a][1])
                    for a in range(len(parts[0]))])
            return 0
        lax.fori_loop(0, (hi - lo) // u, body, 0)

    def take(gen, n):
        for _ in range(n):
            next(gen, None)
            yield
        for _ in gen:
            pass

    def layer_a(first):
        def part(g, p):
            def make(jj):
                gens = [(a_proj(g + p, 1 - p, jj), 24), (a_attn(g, p, jj), 130)]
                if first:
                    if p == 1:
                        gens += [(prep_b(g, jj, n), 4) for n in range(2)]
                    else:
                        gens.append((chain(*[prep_ao(g, 2 * jj + n, 3 + n) for n in range(2)]), 4))
                        if not (isinstance(g, int) and g == 3):
                            gens.append((chain(*[prep_a(g + 1, jj, t, t) for t in range(3)]), 12))
                return gens
            loop(0, 4, make, 4)

        def grp(g, _):
            def at(g0, wait, start):
                @pl.when(g == g0)
                def _():
                    for cp in wait:
                        cp.wait()
                    for cp in start:
                        cp.start()
            if first:
                at(0, a_cp[1] + ao_cp, a_cp[2] + b_cp[0])
                at(1, a_cp[2], b_cp[2])
                at(2, a_cp[3], [])
            part(g, 0)
            if first:
                at(0, b_cp[0], a_cp[3] + b_cp[1])
                at(1, b_cp[1], b_cp[3])
                at(2, b_cp[2] + b_cp[3], [])
            if first:
                part(g, 1)
            else:
                pl.when(g < 3)(lambda: part(g, 1))
            return 0
        lax.fori_loop(0, 3 if first else 4, grp, 0)
        if first:
            part(3, 0)
        weave((out_proj(0, woa), 32), (a_attn(3, 1, 0), 130))
        loop(1, 4, lambda i: [(out_proj(i, woa), 32), (a_attn(3, 1, i), 130), (norm(i - 1), NORM)])
        loop(4, 8, lambda i: [(out_proj(i, woa), 32), (norm(i - 1), NORM)] + (
            [(prep_b(3, i - 4, n), 4) for n in range(2)] if first else []))

    def allred(f, x):
        out = []
        for a in range(2):
            r = _tree(f, [x[a * 64 + i * 8:a * 64 + i * 8 + 8] for i in range(8)])
            r = f(r, pltpu.roll(r, 4, 0))
            out.append(f(r, pltpu.roll(r, 2, 0)))
        return out

    def bc(r):
        return jnp.concatenate([r[0]] * 8 + [r[1]] * 8, axis=0)

    def feat(p, g, is_q):
        ep = jnp.exp(p - bc(allred(jnp.maximum, p)))
        en = jnp.exp(bc(allred(jnp.minimum, p)) - p)
        ip = [1.0 / t for t in allred(jnp.add, ep)]
        im = [1.0 / t for t in allred(jnp.add, en)]
        if is_q:
            dp = allred(jnp.add, ep * jnp.tile(zacc[g, :128], (1, 2)))
            dn = allred(jnp.add, en * jnp.tile(zacc[g, 128:], (1, 2)))
            r = [1.0 / (dp[a] * ip[a] + dn[a] * im[a] + 1e-6) for a in range(2)]
            ip = [ip[a] * r[a] for a in range(2)]
            im = [im[a] * r[a] for a in range(2)]
        ep, en = ep * bc(ip), en * bc(im)
        if not is_q:
            zacc[g, :128] += ep[:, :128] + ep[:, 128:]
            zacc[g, 128:] += en[:, :128] + en[:, 128:]
        return [jnp.concatenate([ep[a * 64:(a + 1) * 64], en[a * 64:(a + 1) * 64]], axis=0).astype(BF16)
                for a in range(2)]

    def b_kv(i):
        xin = rhs(xn, i)
        phis = []
        for g in range(9):
            if g < 8:
                pk = _mm(wrows(wb, 1, g), xin) if g == 0 else nxt
                if g < 7:
                    nxt = _mm(wrows(wb, 1, g + 1), xin)
                v = _mm(wrows(wb, 2, g), xin).astype(BF16)
            if g > 0:
                v1, ph = phis[g - 1]
                kvacc[g - 1] += jnp.concatenate(
                    [lax.dot_general(v1[a * 64:(a + 1) * 64], ph[a], NT, preferred_element_type=F32)
                     for a in range(2)], axis=0)
            yield
            if g < 8:
                phis.append((v, feat(pk, g, False)))

    def b_fin(g):
        r_i = lax.broadcasted_iota(jnp.int32, (128, 128), 0)
        r_j = lax.broadcasted_iota(jnp.int32, (128, 128), 1)
        kv = jnp.concatenate([kvacc[g, pl.ds(a * 64 + p, DH, stride=2), :]
                              for a in range(2) for p in range(2)], axis=0)
        kvm[g] = _pk(jnp.where(r_i // 16 % 2 == r_j % 2, kv, 0.0))
        zacc[g] = jnp.broadcast_to(jnp.sum(zacc[g], axis=1, keepdims=True), (256, 128))

    def b_q(i, first=False):
        xin = rhs(xn, i)
        phis = []
        for g in range(9):
            if g < 8:
                pq = _mm(wrows(wb, 0, g), xin) if g == 0 else nxt
                if g < 7:
                    nxt = _mm(wrows(wb, 0, g + 1), xin)
            if g > 0:
                for a in range(2):
                    o = _pk(_mm(_up(kvm[g - 1, a * 32:(a + 1) * 32]), phis[g - 1][a]))
                    for p in range(2):
                        row = (g - 1) // 2 * 128 + p * 64 + ((g - 1) % 2 * 2 + a) * 16
                        for h in range(2):
                            ot[i, h, row:row + 16, :] = o[p * 16:(p + 1) * 16, h * 128:(h + 1) * 128]
            yield
            if g < 8:
                if first:
                    b_fin(g)
                phis.append(feat(pq, g, True))

    def layer_b(last):
        zacc[...] = jnp.zeros_like(zacc)
        kvacc[...] = jnp.zeros_like(kvacc)
        weave((b_kv(0), 9), (norm(7), NORM * 2))
        weave((b_kv(1), 9))
        loop(2, 8, lambda i: [(b_kv(i), 9)])
        weave((b_q(0, True), 9))
        if last:
            weave((b_q(1), 9))
            loop(2, 8, lambda i: [(b_q(i), 9)])
            lax.fori_loop(0, 8, final, 0)
            return
        weave((out_proj(0, wob), 32), (b_q(1), 9))
        loop(2, 8, lambda i: [(norm(i - 2), NORM), (out_proj(i - 1, wob), 32), (b_q(i), 9)], 1)
        weave((out_proj(7, wob), 32), (norm(6), NORM))

    def first_prep(ts):
        return chain(*[prep_a(0, c, t, t) for t in ts for c in range(4)])

    for cp in a_cp[0][:2]:
        cp.wait()
    weave((first_prep((0,)), 16))
    for c in range(8):
        x_cp[c].wait()
        if c + XW < 8:
            x_cp[c + XW].start()
        if c == 8 - XW:
            for cp in a_cp[0][2:]:
                cp.start()
        if c == 7:
            for cp in a_cp[1] + ao_cp:
                cp.start()
        load_x(c)
    weave((norm(0), NORM))
    for cp in a_cp[0][2:]:
        cp.wait()
    weave((a_proj(0, 0, 0, 0), 24), (chain(first_prep((1, 2)), iter(range(8)), norm(1)), 56))
    for jj, pair in ((1, (2, 4)), (2, (3, 5)), (3, (6, 7))):
        weave((a_proj(0, 0, jj), 24), (chain(*[norm(i) for i in pair]), 2 * NORM))
    layer_a(True)
    layer_b(False)
    weave((a_proj(0, 0, 0), 24), (norm(7), NORM))
    loop(1, 4, lambda jj: [(a_proj(0, 0, jj), 24)])
    layer_a(False)
    layer_b(True)
    for c in range(8):
        o_cp(c).wait()


@jax.jit
def pallas_interleave_layers__sliding_local_dilated__linear_kernel_hedgehog__prompt_kernel(
        A_x, A_wqkv, A_wo, B_x, B_wqkv, B_w_phi, B_wo):
    del B_x
    vm = pl.BlockSpec(memory_space=pltpu.VMEM)
    hbm = pl.BlockSpec(memory_space=pl.ANY)
    V = pltpu.VMEM
    out = pl.pallas_call(
        _kernel,
        in_specs=[pl.BlockSpec(memory_space=pltpu.SMEM)] + [hbm] * 4 + [vm, hbm],
        out_specs=hbm,
        out_shape=jax.ShapeDtypeStruct((S, D), BF16),
        scratch_shapes=[
            V((8, S, 128), BF16), V((12, 2, D, 128), BF16), V((8, D, 128), BF16),
            V((24, D, 128), BF16), V((8, D, 128), BF16),
            pltpu.SemaphoreType.DMA((72,)), pltpu.SemaphoreType.DMA((8,)), V((8, 64, 128), U32),
            V((4, 8, 384, 128), U32), V((8, 8, 64, 128), U32),
            V((3, 8, D // 2, 128), U32), V((8, 8, 64, 128), U32),
            V((8, 2, D, 128), F32), V((8, 2, 8, 128), F32), V((8, 2, D // 2, 128), U32), V((8, 2, D // 2, 128), U32),
            V((8, 256, 128), F32), V((16, 256, 128), F32), V((16, 256, 128), F32),
            V((8, 256, 128), F32), V((16, 256, 128), F32), V((16, 256, 128), F32),
            V((5, 264, 128), U32), V((8, 128, 128), F32), V((8, 256, 128), F32), V((8, 64, 128), U32),
        ],
        compiler_params=pltpu.CompilerParams(vmem_limit_bytes=110 * 1024 * 1024),
    )(np.zeros((1,), np.int32), A_x.reshape(S, D), A_wqkv, A_wo, B_wqkv, B_w_phi.reshape(D, DH), B_wo)
    return out.reshape(1, S, D)
```

```python
import numpy as np
import jax
import jax.numpy as jnp
from jax import lax
import jax.experimental.pallas as pl
import jax.experimental.pallas.tpu as pltpu

S, D, DH = 2048, 1024, 32
W = 8
F32, BF16, U32 = jnp.float32, jnp.bfloat16, jnp.uint32
NT = (((1,), (1,)), ((), ()))


def _mm(a, b):
    return jnp.dot(a, b, preferred_element_type=F32)


def _pk(x):
    return pltpu.bitcast(x.astype(BF16), U32)


def _up(x):
    return pltpu.bitcast(x, BF16)


def _half(w, p):
    return lax.bitcast_convert_type((w << 16) if p == 0 else (w & jnp.uint32(0xFFFF0000)), F32)


def _tree(f, xs):
    xs = list(xs)
    while len(xs) > 1:
        xs = [f(xs[i], xs[i + 1]) for i in range(0, len(xs), 2)]
    return xs[0]


def _weave(*gens):
    order = sorted(((k + (0.5 if gi else 0)) / n, gi) for gi, (_, n) in enumerate(gens) for k in range(n))
    for _, gi in order:
        next(gens[gi][0], None)
    for g, _ in gens:
        for _ in g:
            pass


NORM = 16
XW = 4


def _kernel(zero_ref, x_hbm, awqkv_hbm, awo_hbm, bwqkv_hbm, bphi, bwo_hbm, out_hbm,
            xio, awqkv, awo, bwqkv, bwo, sems, osems, bds,
            wa, woa, wb, wob, xt, xsum, xn, ot, q0, k0, v0, q1, k1, v1, tmp, kvacc, zacc, kvm):
    never = lax.broadcasted_iota(jnp.int32, (8, 128), 0) < zero_ref[0]
    pace = []

    def gate(xs, who):
        if not pace or who in pace[1]:
            return xs
        pace[1].append(who)
        return [jnp.where(never, lax.bitcast_convert_type(pace[0], x.dtype), x) for x in xs]

    def gate1(w):
        return jnp.concatenate(gate([w[:8]], 'prep') + [w[8:]], axis=0)

    def chunks(n, lhs, x_ref, i, finish):
        for r in range(n):
            for k in range(0, 8, 2):
                yield
                t = _mm(_up(jnp.concatenate([lhs(r, k), lhs(r, k + 1)], axis=1)),
                        _up(jnp.concatenate([x_ref[i, h, k * 64:(k + 2) * 64, :] for h in range(2)], axis=1)))
                acc = t if k == 0 else acc + t
                pace[:] = [t[:8, :128], []]
            for h in range(2):
                finish(r, h, acc[:, h * 128:(h + 1) * 128])

    qkv_buf = ((q0, k0, v0), (q1, k1, v1))

    def norm(i):
        ms = [jnp.broadcast_to(jnp.sum(xsum[i, h], axis=0, keepdims=True) * (1.0 / D), (8, 128))
              for h in range(2)]
        invs = []
        for h in range(2):
            acc = None
            for r in range(4):
                ms[h], = gate([ms[h]], 'norm')
                d = xt[i, h, r * 256:(r + 1) * 256, :] - jnp.tile(ms[h], (32, 1))
                d = d * d
                t = _tree(jnp.add, [d[k * 8:k * 8 + 8] for k in range(32)])
                acc = t if r == 0 else acc + t
                yield
            invs.append(lax.rsqrt(jnp.sum(acc, axis=0, keepdims=True) * (1.0 / D) + 1e-5))
        for h in range(2):
            for r in range(4):
                ms[h], = gate([ms[h]], 'norm')
                for p in range(2):
                    x = xt[i, h, pl.ds(r * 256 + p, 128, stride=2), :]
                    xn[i, h, r * 128 + p * 64:r * 128 + p * 64 + 64, :] = _pk((x - jnp.tile(ms[h], (16, 1))) * invs[h])
                yield

    def put_x(i, h, r, x):
        xt[i, h, r * 128:(r + 1) * 128, :] = x
        t = _tree(jnp.add, [x[k * 8:k * 8 + 8] for k in range(16)])
        xsum[i, h] = t if r == 0 else xsum[i, h] + t

    def ds(i, n):
        return pl.ds(pl.multiple_of(i * n, n), n)

    def wrows(ref, g, r):
        return _up(jnp.concatenate([ref[g, k, r * 64:(r + 1) * 64, :] for k in range(8)], axis=1))

    def rhs(ref, i):
        return _up(jnp.concatenate([ref[i, 0], ref[i, 1]], axis=1))

    def lanes(src, dst, first, n, sem0):
        return [pltpu.make_async_copy(src.at[:, ds(first + c, 128)], dst.at[c], sems.at[sem0 + c])
                for c in range(n)]

    x_cp = lanes(x_hbm, xio, 0, 8, 0)
    a_cp = [[cp for t in range(3) for cp in lanes(awqkv_hbm, awqkv.at[g * 3 + t], t * 8 + g * 2, 2, 8 + g * 6 + t * 2)]
            for g in range(4)]
    ao_cp = lanes(awo_hbm, awo, 0, 8, 32)
    bq_cp = lanes(bwqkv_hbm, bwqkv, 0, 24, 40)
    b_cp = [[bq_cp[t * 8 + 2 * g + n] for t in range(3) for n in range(2)] for g in range(4)]
    b_cp[0] += lanes(bwo_hbm, bwo, 0, 8, 64)
    for cp in a_cp[0][:2] + x_cp[:XW]:
        cp.start()

    awqkv32, awo32, bwqkv32, bwo32 = [r.bitcast(U32) for r in (awqkv, awo, bwqkv, bwo)]

    def prep_a(g, c, t, u):
        for n in range(2):
            w = gate1(awqkv32[g * 3 + t, n, ds(c, 128), :]).T
            for h in range(4):
                tmp[u, pl.ds((n * 4 + h) * (DH + 1), DH), :] = w[h * DH:(h + 1) * DH]
            yield
        for half in range(2):
            w = jnp.concatenate([tmp[u, pl.ds(half * 16 + d, 8, stride=DH + 1), :] for d in range(16)], axis=0)
            for p in range(2):
                wa[g, 2 * c + p, t * 128 + half * 64:t * 128 + half * 64 + 64, :] = _pk(_half(w, p))
            yield

    def prep_ao(g, c, u):
        w = awo32[c, ds(g, 128), :]
        for h in range(8):
            tmp[u, pl.ds(h * 17, 16), :] = w[h * 16:(h + 1) * 16]
        yield
        w = jnp.concatenate([tmp[u, pl.ds(d, 8, stride=17), :] for d in range(16)], axis=0)
        w = gate1(w).T
        for p in range(2):
            woa[c, 2 * g + p] = _pk(_half(w, p))
        yield

    def prep_b(g, c, n):
        w = gate1(bwo32[2 * c + n, ds(g, 128), :]).T
        for p in range(2):
            wob[2 * c + n, 2 * g + p] = _pk(_half(w, p))
        yield
        w = gate1(bwqkv32[16 + 2 * g + n, ds(c, 128), :]).T
        for p in range(2):
            wb[2, 2 * c + p, ds(2 * g + n, 64), :] = _pk(_half(w, p))
        yield
        for t in range(2):
            w = bwqkv32[t * 8 + 2 * g + n, ds(c, 128), :]
            for p in range(2):
                wb[t, 2 * c + p, ds(2 * g + n, 64), :] = _pk(lax.dot_general(
                    _up(bds[2 * g + n]), _half(w, p).astype(BF16), NT, preferred_element_type=F32))
            yield

    f_i = lax.broadcasted_iota(jnp.int32, (DH, 128), 0)
    f_j = lax.broadcasted_iota(jnp.int32, (DH, 128), 1)
    rep = _mm(bphi[...], jnp.where(f_i == f_j % 64 // 2, 1.0, 0.0).astype(BF16))
    e_i = lax.broadcasted_iota(jnp.int32, (128, 128), 0)
    e_j = lax.broadcasted_iota(jnp.int32, (128, 128), 1)
    for g in range(8):
        bds[g] = _pk(jnp.where(e_i // 64 * 2 + e_i % 2 == e_j // DH, rep[g * 128:(g + 1) * 128].T, 0.0))

    xio32 = xio.bitcast(U32)

    def load_x(c):
        for jj in range(4):
            for h in range(2):
                w = xio32[c, pl.ds(2 * jj + h, 128, stride=8), :].T
                for p in range(2):
                    put_x(p * 4 + jj, h, c, _half(w, p))

    def chain(*gens):
        for g in gens:
            yield from g

    def o_cp(c):
        return pltpu.make_async_copy(xio.at[c], out_hbm.at[:, ds(c, 128)], osems.at[c])

    def final(c, _):
        w = _up(jnp.concatenate([wob[c, k] for k in range(8)], axis=1))
        for jj in range(4):
            t = [_mm(w, rhs(ot, p * 4 + jj)) for p in range(2)]
            for h in range(2):
                e, o = [lax.bitcast_convert_type(
                    (xt[p * 4 + jj, h, ds(c, 128), :] + t[p][:, h * 128:(h + 1) * 128]).astype(BF16).astype(F32),
                    U32) for p in range(2)]
                xio32[c, pl.ds(2 * jj + h, 128, stride=8), :] = ((e >> 16) | o).T
        o_cp(c).start()
        return 0

    def out_proj(i, w_ref):
        def finish(r, h, t):
            put_x(i, h, r, xt[i, h, r * 128:(r + 1) * 128, :] + t)
        return chunks(8, lambda r, k: w_ref[r, k], ot, i, finish)

    def a_proj(g, p, jj, rot=2):
        qr, kr, vr = qkv_buf[p]
        j = 2 * jj

        def finish(r, i, ti):
            r = (r + rot) % 6
            sl = slice((r % 2) * 128, (r % 2 + 1) * 128)
            if r < 2:
                qr[j + i, sl, :] = ti
            else:
                dst = kr if r < 4 else vr
                dst[8 + j + i, sl, :] = ti
                dst[j + i, sl, :] = pltpu.roll(ti, 1, 1)

        def lhs(r, k):
            r = (r + rot) % 6
            return wa[g, k, r * 64:(r + 1) * 64, :]
        return chunks(6, lhs, xn, p * 4 + jj, finish)

    lane0 = lax.broadcasted_iota(jnp.int32, (8, 128), 1) == 0

    def a_attn(g, p, jj):
        qr, kr, vr = qkv_buf[p]
        for i in range(2):
            j = 2 * jj + i
            lg = [None] * W
            for d in range(DH):
                sl = slice(d * 8, d * 8 + 8)
                q, = gate([qr[j, sl, :]], 'attn')
                for w in range(W):
                    t = q * kr[8 + j - w, sl, :]
                    lg[w] = t if d == 0 else lg[w] + t
                yield
            l = [t * (DH ** -0.5) for t in lg]
            l = [l[0]] + [jnp.where(lane0 & (j < w), -1e9, l[w]) for w in range(1, W)]
            m = _tree(jnp.maximum, l)
            e = [jnp.exp(t - m) for t in l]
            inv = 1.0 / _tree(jnp.add, e)
            pr = [t * inv for t in e]
            yield
            for par in range(2):
                o = []
                for dd in range(DH // 2):
                    pr = gate(pr, 'attn')
                    sl = slice((2 * dd + par) * 8, (2 * dd + par) * 8 + 8)
                    o.append(_tree(jnp.add, [pr[w] * vr[8 + j - w, sl, :] for w in range(W)]))
                    if dd % 2:
                        ot[p * 4 + jj, i, ds(g * 16 + par * 8 + dd // 2, 8), :] = _pk(
                            jnp.concatenate(o[-2:], axis=0))
                    yield

    def weave(*gens):
        pace.clear()
        _weave(*gens)
        pace.clear()

    def loop(lo, hi, make, u=2):
        if (hi - lo) % u:
            u = hi - lo

        def body(k, _):
            parts = [make(lo + k * u + t) for t in range(u)]
            weave(*[(chain(*[take(*pt[a]) for pt in parts]), u * parts[0][a][1])
                    for a in range(len(parts[0]))])
            return 0
        lax.fori_loop(0, (hi - lo) // u, body, 0)

    def take(gen, n):
        for _ in range(n):
            next(gen, None)
            yield
        for _ in gen:
            pass

    def layer_a(first):
        def part(g, p):
            def make(jj):
                gens = [(a_proj(g + p, 1 - p, jj), 24), (a_attn(g, p, jj), 130)]
                if first:
                    if p == 1:
                        gens += [(prep_b(g, jj, n), 4) for n in range(2)]
                    else:
                        gens.append((chain(*[prep_ao(g, 2 * jj + n, 3 + n) for n in range(2)]), 4))
                        if not (isinstance(g, int) and g == 3):
                            gens.append((chain(*[prep_a(g + 1, jj, t, t) for t in range(3)]), 12))
                return gens
            loop(0, 4, make, 4)

        def grp(g, _):
            def at(g0, wait, start):
                @pl.when(g == g0)
                def _():
                    for cp in wait:
                        cp.wait()
                    for cp in start:
                        cp.start()
            if first:
                at(0, a_cp[1] + ao_cp, a_cp[2] + b_cp[0])
                at(1, a_cp[2], b_cp[2])
                at(2, a_cp[3], [])
            part(g, 0)
            if first:
                at(0, b_cp[0], a_cp[3] + b_cp[1])
                at(1, b_cp[1], b_cp[3])
                at(2, b_cp[2] + b_cp[3], [])
            if first:
                part(g, 1)
            else:
                pl.when(g < 3)(lambda: part(g, 1))
            return 0
        lax.fori_loop(0, 3 if first else 4, grp, 0)
        if first:
            part(3, 0)
        weave((out_proj(0, woa), 32), (a_attn(3, 1, 0), 130))
        loop(1, 4, lambda i: [(out_proj(i, woa), 32), (a_attn(3, 1, i), 130), (norm(i - 1), NORM)])
        loop(4, 8, lambda i: [(out_proj(i, woa), 32), (norm(i - 1), NORM)] + (
            [(prep_b(3, i - 4, n), 4) for n in range(2)] if first else []))

    def allred(f, x):
        out = []
        for a in range(2):
            r = _tree(f, [x[a * 64 + i * 8:a * 64 + i * 8 + 8] for i in range(8)])
            r = f(r, pltpu.roll(r, 4, 0))
            out.append(f(r, pltpu.roll(r, 2, 0)))
        return out

    def bc(r):
        return jnp.concatenate([r[0]] * 8 + [r[1]] * 8, axis=0)

    def feat(p, g, is_q, first=False):
        ep = jnp.exp(p - bc(allred(jnp.maximum, p)))
        en = jnp.exp(bc(allred(jnp.minimum, p)) - p)
        ip = [1.0 / t for t in allred(jnp.add, ep)]
        im = [1.0 / t for t in allred(jnp.add, en)]
        if is_q:
            dp = allred(jnp.add, ep * jnp.tile(zacc[g, :128], (1, 2)))
            dn = allred(jnp.add, en * jnp.tile(zacc[g, 128:], (1, 2)))
            r = [1.0 / (dp[a] * ip[a] + dn[a] * im[a] + 1e-6) for a in range(2)]
            ip = [ip[a] * r[a] for a in range(2)]
            im = [im[a] * r[a] for a in range(2)]
        ep, en = ep * bc(ip), en * bc(im)
        if not is_q:
            for e, sl in ((ep, slice(0, 128)), (en, slice(128, 256))):
                z = e[:, :128] + e[:, 128:]
                zacc[g, sl] = z if first else zacc[g, sl] + z
        return [jnp.concatenate([ep[a * 64:(a + 1) * 64], en[a * 64:(a + 1) * 64]], axis=0).astype(BF16)
                for a in range(2)]

    def b_kv(i, first=False):
        xin = rhs(xn, i)
        phis = []
        for g in range(9):
            if g < 8:
                pk = _mm(wrows(wb, 1, g), xin) if g == 0 else nxt
                if g < 7:
                    nxt = _mm(wrows(wb, 1, g + 1), xin)
                v = _mm(wrows(wb, 2, g), xin).astype(BF16)
            if g > 0:
                v1, ph = phis[g - 1]
                kv = jnp.concatenate(
                    [lax.dot_general(v1[a * 64:(a + 1) * 64], ph[a], NT, preferred_element_type=F32)
                     for a in range(2)], axis=0)
                kvacc[g - 1] = kv if first else kvacc[g - 1] + kv
            yield
            if g < 8:
                phis.append((v, feat(pk, g, False, first)))

    def b_fin(g):
        r_i = lax.broadcasted_iota(jnp.int32, (128, 128), 0)
        r_j = lax.broadcasted_iota(jnp.int32, (128, 128), 1)
        kv = jnp.concatenate([kvacc[g, pl.ds(a * 64 + p, DH, stride=2), :]
                              for a in range(2) for p in range(2)], axis=0)
        kvm[g] = _pk(jnp.where(r_i // 16 % 2 == r_j % 2, kv, 0.0))
        zacc[g] = jnp.broadcast_to(jnp.sum(zacc[g], axis=1, keepdims=True), (256, 128))

    def b_q(i, first=False):
        xin = rhs(xn, i)
        phis = []
        for g in range(9):
            if g < 8:
                pq = _mm(wrows(wb, 0, g), xin) if g == 0 else nxt
                if g < 7:
                    nxt = _mm(wrows(wb, 0, g + 1), xin)
            if g > 0:
                for a in range(2):
                    o = _pk(_mm(_up(kvm[g - 1, a * 32:(a + 1) * 32]), phis[g - 1][a]))
                    for p in range(2):
                        row = (g - 1) // 2 * 128 + p * 64 + ((g - 1) % 2 * 2 + a) * 16
                        for h in range(2):
                            ot[i, h, row:row + 16, :] = o[p * 16:(p + 1) * 16, h * 128:(h + 1) * 128]
            yield
            if g < 8:
                if first:
                    b_fin(g)
                phis.append(feat(pq, g, True))

    def layer_b(last):
        weave((b_kv(0, True), 9), (norm(7), NORM * 2))
        weave((b_kv(1), 9))
        loop(2, 8, lambda i: [(b_kv(i), 9)])
        weave((b_q(0, True), 9))
        if last:
            weave((b_q(1), 9))
            loop(2, 8, lambda i: [(b_q(i), 9)])
            lax.fori_loop(0, 8, final, 0)
            return
        weave((out_proj(0, wob), 32), (b_q(1), 9))
        loop(2, 8, lambda i: [(norm(i - 2), NORM), (out_proj(i - 1, wob), 32), (b_q(i), 9)], 1)
        weave((out_proj(7, wob), 32), (norm(6), NORM))

    def first_prep(ts):
        return chain(*[prep_a(0, c, t, t) for t in ts for c in range(4)])

    for cp in a_cp[0][:2]:
        cp.wait()
    weave((first_prep((0,)), 16))
    for c in range(8):
        x_cp[c].wait()
        if c + XW < 8:
            x_cp[c + XW].start()
        if c == 8 - XW:
            for cp in a_cp[0][2:]:
                cp.start()
        if c == 7:
            for cp in a_cp[1] + ao_cp:
                cp.start()
        load_x(c)
    weave((norm(0), NORM))
    for cp in a_cp[0][2:]:
        cp.wait()
    weave((a_proj(0, 0, 0, 0), 24), (chain(first_prep((1, 2)), iter(range(8)), norm(1)), 56))
    for jj, pair in ((1, (2, 4)), (2, (3, 5)), (3, (6, 7))):
        weave((a_proj(0, 0, jj), 24), (chain(*[norm(i) for i in pair]), 2 * NORM))
    layer_a(True)
    layer_b(False)
    weave((a_proj(0, 0, 0), 24), (norm(7), NORM))
    loop(1, 4, lambda jj: [(a_proj(0, 0, jj), 24)])
    layer_a(False)
    layer_b(True)
    for c in range(8):
        o_cp(c).wait()


@jax.jit
def pallas_interleave_layers__sliding_local_dilated__linear_kernel_hedgehog__prompt_kernel(
        A_x, A_wqkv, A_wo, B_x, B_wqkv, B_w_phi, B_wo):
    del B_x
    vm = pl.BlockSpec(memory_space=pltpu.VMEM)
    hbm = pl.BlockSpec(memory_space=pl.ANY)
    V = pltpu.VMEM
    out = pl.pallas_call(
        _kernel,
        in_specs=[pl.BlockSpec(memory_space=pltpu.SMEM)] + [hbm] * 4 + [vm, hbm],
        out_specs=hbm,
        out_shape=jax.ShapeDtypeStruct((S, D), BF16),
        scratch_shapes=[
            V((8, S, 128), BF16), V((12, 2, D, 128), BF16), V((8, D, 128), BF16),
            V((24, D, 128), BF16), V((8, D, 128), BF16),
            pltpu.SemaphoreType.DMA((72,)), pltpu.SemaphoreType.DMA((8,)), V((8, 64, 128), U32),
            V((4, 8, 384, 128), U32), V((8, 8, 64, 128), U32),
            V((3, 8, D // 2, 128), U32), V((8, 8, 64, 128), U32),
            V((8, 2, D, 128), F32), V((8, 2, 8, 128), F32), V((8, 2, D // 2, 128), U32), V((8, 2, D // 2, 128), U32),
            V((8, 256, 128), F32), V((16, 256, 128), F32), V((16, 256, 128), F32),
            V((8, 256, 128), F32), V((16, 256, 128), F32), V((16, 256, 128), F32),
            V((5, 264, 128), U32), V((8, 128, 128), F32), V((8, 256, 128), F32), V((8, 64, 128), U32),
        ],
        compiler_params=pltpu.CompilerParams(vmem_limit_bytes=110 * 1024 * 1024),
    )(np.zeros((1,), np.int32), A_x.reshape(S, D), A_wqkv, A_wo, B_wqkv, B_w_phi.reshape(D, DH), B_wo)
    return out.reshape(1, S, D)
```
